```python
import jax
import jax.numpy as jnp

def _softmax(x, axis=-1):
    return jax.nn.softmax(x, axis=axis)
def _gelu(x):
    return jax.nn.gelu(x, approximate=True)
def _silu(x):
    return jax.nn.silu(x)
def _sigmoid(x):
    return jax.nn.sigmoid(x)
def _layernorm(x, axis=-1, eps=1e-5):
    m = jnp.mean(x, axis=axis, keepdims=True)
    v = jnp.var(x, axis=axis, keepdims=True)
    return (x - m) / jnp.sqrt(v + eps)
def _scatter_add(tgt, idx, src, axis=0):
    return tgt.at[idx].add(src)
def _segment_sum(src, seg, n):
    return jax.ops.segment_sum(src, seg, n)
class _Rng:
    def __init__(self, key):
        self._k = key
    def _next(self):
        self._k, sub = jax.random.split(self._k)
        return sub
    def normal(self, shape):
        return jax.random.normal(self._next(), shape, dtype=jnp.bfloat16)
    def randint(self, lo, hi, shape):
        return jax.random.randint(self._next(), shape, lo, hi, dtype=jnp.int32)
    def uniform(self, shape, lo=0.0, hi=1.0):
        return jax.random.uniform(self._next(), shape, jnp.bfloat16, lo, hi)
    def permutation(self, n):
        return jax.random.permutation(self._next(), n)


kernel_name = 'concat_heads__sliding_block_cached__compressed_kv_cla__decode'

def setup_inputs():
    _rng = _Rng(jax.random.key(int.from_bytes(__import__("os").urandom(4), "little")))
    _w = (lambda a: (lambda t: t.astype(jnp.bfloat16) if jnp.issubdtype(t.dtype, jnp.floating) else t)(jnp.asarray(a)))
    def _A_setup():
        B, Sq, D = 4, 1, 512
        Hq, Hkv, Sk, Dh = 32, 32, 4096, 128
        assert Hq % Hkv == 0, (Hq, Hkv)
        return {
            "x": _w((lambda *s: _rng.normal(s) * 0.05)(B, Sq, D)),
            "k_cache": _w((lambda *s: _rng.normal(s) * 0.05)(B, Hkv, Sk, Dh)),
            "v_cache": _w((lambda *s: _rng.normal(s) * 0.05)(B, Hkv, Sk, Dh)),
            "wq": _w((lambda *s: _rng.normal(s) * 0.05)(D, Hq * Dh) * (D ** -0.5)),
            "wo": _w((lambda *s: _rng.normal(s) * 0.05)(Hq * Dh, D) * ((Hq * Dh) ** -0.5)),
        }
    _A_in = _A_setup()

    def _B_setup():
        B, H, Sq, Sk, D, M = 4, 32, 1, 4096, 128, 512
        Dc = 4 * D
        return {
            "x": _w((lambda *s: _rng.normal(s) * 0.05)(B, Sq, M)),
            "c_kv": _w((lambda *s: _rng.normal(s) * 0.05)(B, Sk, Dc)),
            "w_q": _w((lambda *s: _rng.normal(s) * 0.05)(M, H, D) * (M ** -0.5)),
            "w_uk": _w((lambda *s: _rng.normal(s) * 0.05)(Dc, H, D) * (Dc ** -0.5)),
            "w_uv": _w((lambda *s: _rng.normal(s) * 0.05)(Dc, H, D) * (Dc ** -0.5)),
            "w_o": _w((lambda *s: _rng.normal(s) * 0.05)(H, D, M) * ((H * D) ** -0.5)),
        }
    _B_in = _B_setup()

    return {
        "A_x": _A_in["x"],
        "A_k_cache": _A_in["k_cache"],
        "A_v_cache": _A_in["v_cache"],
        "A_wq": _A_in["wq"],
        "A_wo": _A_in["wo"],
        "B_x": _B_in["x"],
        "B_c_kv": _B_in["c_kv"],
        "B_w_q": _B_in["w_q"],
        "B_w_uk": _B_in["w_uk"],
        "B_w_uv": _B_in["w_uv"],
        "B_w_o": _B_in["w_o"],
    }

def reference(A_x, A_k_cache, A_v_cache, A_wq, A_wo, B_x, B_c_kv, B_w_q, B_w_uk, B_w_uv, B_w_o):
    def _A_ref(x, k_cache, v_cache, wq, wo):
        B, Sq, D = x.shape
        Hq, Dh = 32, 128
        Hkv, Sk = k_cache.shape[1], k_cache.shape[2]
        W = min(4096, max(256, Sk // 4))
        rep = Hq // Hkv
        q = (lambda x, *d: x.transpose(*d))((x @ wq).reshape(B, Sq, Hq, Dh), 0, 2, 1, 3)
        k = jnp.repeat(k_cache[:, :, Sk - W:, :], rep, axis=1)
        v = jnp.repeat(v_cache[:, :, Sk - W:, :], rep, axis=1)
        scores = jnp.einsum("bhqd,bhkd->bhqk", q, k) * (Dh ** -0.5)
        p = _softmax(scores, axis=-1)
        o = jnp.einsum("bhqk,bhkd->bhqd", p, v)
        return (lambda x, *d: x.transpose(*d))(o, 0, 2, 1, 3).reshape(B, Sq, Hq * Dh) @ wo

    def _B_ref(x, c_kv, w_q, w_uk, w_uv, w_o):
        B, Sq, M = x.shape[0], x.shape[1], x.shape[2]
        Sk = c_kv.shape[1]
        H, D = w_q.shape[1], w_q.shape[2]
        q = jnp.einsum("bqm,mhd->bhqd", x, w_q)
        k = jnp.einsum("bkc,chd->bhkd", c_kv, w_uk)
        v = jnp.einsum("bkc,chd->bhkd", c_kv, w_uv)
        scores = jnp.einsum("bhqd,bhkd->bhqk", q, k) * (D ** -0.5)
        off = Sk - Sq
        qi = jnp.arange(Sq)[:, None]
        kj = jnp.arange(Sk)[None, :]
        cmask = kj <= (qi + off)
        scores = jnp.where(cmask[None, None], scores, -1e9)
        p = _softmax(scores, axis=-1)
        ctx = jnp.einsum("bhqk,bhkd->bhqd", p, v)
        return jnp.einsum("bhqd,hdm->bqm", ctx, w_o)

    a = _A_ref(A_x, A_k_cache, A_v_cache, A_wq, A_wo)
    b = _B_ref(B_x, B_c_kv, B_w_q, B_w_uk, B_w_uv, B_w_o)
    return jnp.concatenate([a, b], axis=-1)
```

```python
import jax
import jax.numpy as jnp
from jax import lax
import jax.experimental.pallas as pl
import jax.experimental.pallas.tpu as pltpu

F32 = jnp.float32
BF16 = jnp.bfloat16

B = 4
H = 32
DH = 128
DM = 512
SK = 4096
W = 1024
SCALE = DH ** -0.5

NP = 32
NT = (((1,), (1,)), ((), ()))


def _iota(shape, d):
    return lax.broadcasted_iota(jnp.int32, shape, d)


def _dot(a, b):
    return jnp.dot(a, b, preferred_element_type=F32)


def _dot_nt(a, b):
    return lax.dot_general(a, b, NT, preferred_element_type=F32)


def _kernel(
    xa_hbm, k_hbm, v_hbm, wq_hbm, wo_hbm,
    xb_hbm, c_hbm, bq_hbm, buk_hbm, buv_hbm, bo_hbm,
    o_ref,
    xa_v, xb_v, kv_v, wq_v, wo_v, c_v, bq_v, buk_v, buv_v, bo_v,
    e_v, et_v, x2_v, qb_v, qabs_v, m_v, l_v, acc_v, cn_v, ctx_v,
    qa_v, oa_v, ob_v,
    sems, xsem, fsems,
):
    def start(src, dst, sem, prio):
        pltpu.make_async_copy(src, dst, sem).start(priority=prio)

    def wait(dst, sem):
        pltpu.make_async_copy(dst, dst, sem).wait()

    def issue_w3(src, dst, t, j, sem, prio):
        start(src.at[:, t * NP + j], dst.at[:, t * NP + j], sem, prio)

    def issue_s0(t, j0, j1):
        sem = sems.at[t % 3]
        for j in range(j0, j1):
            issue_w3(bq_hbm, bq_v, t, j, sem, 0)
            issue_w3(buk_hbm, buk_v, t, j, sem, 1)

    def wait_s0(t):
        sem = sems.at[t % 3]
        wait(bq_v.at[:, pl.ds(t * NP, NP)], sem)
        wait(buk_v.at[:, pl.ds(t * NP, NP)], sem)

    def issue_s1(t, j0, j1):
        sem = sems.at[(4 + t) % 3]
        for j in range(j0, j1):
            idx = (slice(None), pl.ds((t * 4 + j // 8) * 8, 8), pl.ds((j % 8) * 512, 512))
            start(wq_hbm.at[idx], wq_v.at[idx], sem, 0)
            issue_w3(buv_hbm, buv_v, t, j, sem, 1)

    def wait_s1(t):
        sem = sems.at[(4 + t) % 3]
        wait(wq_v.at[:, pl.ds(t * 32, 32), :], sem)
        wait(buv_v.at[:, pl.ds(t * NP, NP)], sem)

    def issue_c(i, j0, j1):
        sem = sems.at[(8 + i) % 3]
        p0 = (i // 4) * 8
        r0 = (i % 4) * 256
        for j in range(j0, j1):
            for u in range(2):
                idx = (pl.ds(p0 + u * 4, 4), pl.ds(pl.multiple_of(r0 + j * 8, 8), 8), slice(None))
                start(c_hbm.at[idx], c_v.at[idx], sem, u)

    def wait_c(i):
        sem = sems.at[(8 + i) % 3]
        p0 = (i // 4) * 8
        r0 = pl.multiple_of((i % 4) * 256, 256)
        wait(c_v.at[pl.ds(p0, 8), pl.ds(r0, 256), :], sem)

    def issue_kv(h, j0, j1):
        slot = (16 + h) % 3
        sem = sems.at[slot]
        for j in range(j0, j1):
            for u, src in enumerate((k_hbm, v_hbm)):
                start(src.at[:, h, pl.ds(SK - W + j * 32, 32), :],
                      kv_v.at[slot, u, :, pl.ds(j * 32, 32), :], sem, u)

    def wait_kv(h):
        slot = (16 + h) % 3
        wait(kv_v.at[slot], sems.at[slot])

    def issue_o(u):
        sem = fsems.at[u]
        for j in range(16):
            idx = (slice(None), pl.ds(pl.multiple_of(u * 128 + j * 8, 8), 8), slice(None))
            start(wo_hbm.at[idx], wo_v.at[idx], sem, 0)
            start(bo_hbm.at[idx], bo_v.at[idx], sem, 1)

    def wait_o(u):
        sem = fsems.at[u]
        wait(wo_v.at[:, pl.ds(u * 128, 128), :], sem)
        wait(bo_v.at[:, pl.ds(u * 128, 128), :], sem)

    def diag_mask():
        return (_iota((64, 2048), 1) & 15) == (_iota((64, 2048), 0) & 15)

    def w3(ref, k, hf):
        return ref[k, :, hf].reshape(2048, DH)

    def build_consts():
        e_v[...] = jnp.where(_iota((128, 2048), 0) == (_iota((128, 2048), 1) >> 4), 1.0, 0.0).astype(BF16)
        et_v[...] = jnp.where(_iota((2048, 128), 1) == (_iota((2048, 128), 0) >> 4), 1.0, 0.0).astype(BF16)
        m_v[...] = jnp.full(m_v.shape, -jnp.inf, F32)
        l_v[...] = jnp.zeros(l_v.shape, F32)
        acc_v[...] = jnp.zeros(acc_v.shape, F32)

    def build_x2():
        x = xb_v[...].astype(F32)
        xrep = jnp.concatenate(
            [jnp.broadcast_to(x[b:b + 1, :], (16, DM)) for b in range(B)], axis=0).astype(BF16)
        for k in range(4):
            xe = _dot(xrep[:, k * 128:(k + 1) * 128], e_v[...])
            x2_v[:, k * 2048:(k + 1) * 2048] = jnp.where(diag_mask(), xe, 0.0).astype(BF16)

    def qb_half(hf):
        acc = None
        for k in range(4):
            r = _dot(x2_v[:, k * 2048:(k + 1) * 2048], w3(bq_v, k, hf))
            acc = r if acc is None else acc + r
        qb_v[hf * 64:(hf + 1) * 64, :] = acc.astype(BF16)

    def qabs_piece(hf, k):
        r = _dot_nt(qb_v[hf * 64:(hf + 1) * 64, :], w3(buk_v, k, hf))
        r = jnp.where(diag_mask(), r, 0.0).astype(BF16)
        z = _dot(r, et_v[...]).astype(BF16)
        for b in range(B):
            qabs_v[b, hf * 16:(hf + 1) * 16, k * 128:(k + 1) * 128] = z[b * 16:(b + 1) * 16, :]

    def qa_proj():
        x = xa_v[...].astype(F32)
        x8 = jnp.concatenate([x, x], axis=0).astype(BF16)
        acc = None
        for k in range(4):
            r = _dot(x8[:, k * 128:(k + 1) * 128], wq_v[k])
            acc = r if acc is None else acc + r
        for h in range(H):
            qa_v[h] = acc[:, h * DH:(h + 1) * DH]

    def b_attn(i, u):
        b = (i // 4) * 2 + u
        r0 = pl.multiple_of((i % 4) * 256, 256)
        c = c_v[pl.ds(b * 4, 4), pl.ds(r0, 256), :].reshape(1024, DM)
        s = _dot_nt(qabs_v[b], c) * SCALE
        m_old = m_v[b]
        m_new = jnp.maximum(m_old, jnp.max(s, axis=1, keepdims=True))
        alpha = jnp.exp(m_old - m_new)
        p = jnp.exp(s - m_new)
        l_v[b] = alpha * l_v[b] + jnp.sum(p, axis=1, keepdims=True)
        acc_v[b] = alpha * acc_v[b] + _dot(p.astype(BF16), c)
        m_v[b] = m_new

    def b_norm():
        for b in range(B):
            cn = (acc_v[b] / l_v[b]).astype(BF16)
            for hf in range(2):
                for k in range(4):
                    cn_v[hf * 4 + k, b * 16:(b + 1) * 16, :] = (
                        cn[hf * 16:(hf + 1) * 16, k * 128:(k + 1) * 128])
        ctx_v[...] = jnp.zeros(ctx_v.shape, F32)

    def ctx_piece(i):
        xe = _dot(cn_v[i], e_v[...])
        xe = jnp.where(diag_mask(), xe, 0.0).astype(BF16)
        ctx_v[i // 4] += _dot(xe, w3(buv_v, i % 4, i // 4))

    def ob_build():
        ro = _iota((256, 128), 0)
        ri = _iota((256, 128), 1)
        src = ((ro >> 7) << 6) + ((ro & 7) << 4) + ((ro >> 3) & 15)
        perm = jnp.where(((ro & 7) < 4) & (ri == src), 1.0, 0.0).astype(BF16)
        ctx = ctx_v[...].reshape(128, DH).astype(BF16)
        ob_v[...] = _dot(perm, ctx).reshape(H, 8, DH)

    def a_head(h):
        slot = (16 + h) % 3
        q = qa_v[h].astype(BF16)
        row = _iota((8, W), 0)
        s = None
        for b in range(B):
            r = _dot_nt(q, kv_v[slot, 0, b])
            s = r if s is None else jnp.where(row == b, r, s)
        s = s * SCALE
        p = jnp.exp(s - jnp.max(s, axis=1, keepdims=True))
        l = jnp.sum(p, axis=1, keepdims=True)
        pb = p.astype(BF16)
        row8 = _iota((8, DH), 0)
        o = None
        for b in range(B):
            r = _dot(pb, kv_v[slot, 1, b])
            o = r if o is None else jnp.where(row8 == b, r, o)
        oa_v[h] = o / l

    def o_unit(u, acc_a, acc_b):
        for p in range(4):
            h = p * 8 + u
            acc_a += _dot(oa_v[h].astype(BF16), wo_v[p, u * 128:(u + 1) * 128, :])
            acc_b += _dot(ob_v[h].astype(BF16), bo_v[p, u * 128:(u + 1) * 128, :])
        return acc_a, acc_b

    issue_s0(0, 0, 2)
    start(xa_hbm, xa_v, xsem.at[0], 0)
    start(xb_hbm, xb_v, xsem.at[0], 0)
    issue_s0(0, 2, NP)
    issue_s0(1, 0, NP)

    issue_s0(2, 0, NP)
    wait_s0(0)
    wait(xa_v, xsem.at[0])
    wait(xb_v, xsem.at[0])
    build_consts()

    issue_s0(3, 0, NP)
    wait_s0(1)
    build_x2()

    issue_s1(0, 0, NP)
    wait_s0(2)

    issue_s1(1, 0, 16)
    wait_s0(3)
    qb_half(0)
    issue_s1(1, 16, NP)
    qb_half(1)

    for hf in range(2):
        issue_s1(2 + hf, 0, 16)
        wait_s1(hf)
        qabs_piece(hf, 0)
        qabs_piece(hf, 1)
        issue_s1(2 + hf, 16, NP)
        qabs_piece(hf, 2)
        qabs_piece(hf, 3)

    issue_c(0, 0, NP)
    wait_s1(2)

    issue_c(1, 0, NP)
    wait_s1(3)
    qa_proj()

    def b_body(i, carry):
        for u in range(2):
            @pl.when(i < 6)
            def _():
                issue_c(i + 2, u * 16, (u + 1) * 16)

            @pl.when(i >= 6)
            def _():
                issue_kv(i - 6, u * 16, (u + 1) * 16)

            if u == 0:
                wait_c(i)
            b_attn(i, u)
        return carry

    lax.fori_loop(0, 8, b_body, 0)
    b_norm()

    def a_body(h, carry):
        @pl.when(h < H - 2)
        def _():
            issue_kv(h + 2, 0, NP)

        @pl.when(h >= H - 2)
        def _():
            u = (h - (H - 2)) * 2
            issue_o(u)
            issue_o(u + 1)

        wait_kv(h)
        a_head(h)

        @pl.when(h < 8)
        def _():
            ctx_piece(h)

        return carry

    lax.fori_loop(0, H, a_body, 0)

    acc_a = jnp.zeros((8, DM), F32)
    acc_b = jnp.zeros((8, DM), F32)
    issue_o(4)
    issue_o(5)
    ob_build()
    for u in range(2):
        wait_o(u)
        acc_a, acc_b = o_unit(u, acc_a, acc_b)
    issue_o(6)
    issue_o(7)
    for u in range(2, 8):
        wait_o(u)
        acc_a, acc_b = o_unit(u, acc_a, acc_b)

    o_ref[:, 0:DM] = acc_a[0:B, :].astype(o_ref.dtype)
    o_ref[:, DM:2 * DM] = acc_b[0:B, :].astype(o_ref.dtype)


@jax.jit
def pallas_concat_heads__sliding_block_cached__compressed_kv_cla__decode_kernel(
    A_x: jax.Array,
    A_k_cache: jax.Array,
    A_v_cache: jax.Array,
    A_wq: jax.Array,
    A_wo: jax.Array,
    B_x: jax.Array,
    B_c_kv: jax.Array,
    B_w_q: jax.Array,
    B_w_uk: jax.Array,
    B_w_uv: jax.Array,
    B_w_o: jax.Array,
):
    w3_shape = (4, 128, 2, 16, DH)
    hbm = pl.BlockSpec(memory_space=pl.ANY)
    vmem = pltpu.VMEM
    out = pl.pallas_call(
        _kernel,
        out_shape=jax.ShapeDtypeStruct((B, 2 * DM), BF16),
        in_specs=[hbm] * 11,
        out_specs=pl.BlockSpec(memory_space=pltpu.VMEM),
        scratch_shapes=[
            vmem((B, DM), BF16),
            vmem((B, DM), BF16),
            vmem((3, 2, B, W, DH), BF16),
            vmem((4, 128, H * DH), BF16),
            vmem((4, 1024, DM), BF16),
            vmem((16, 1024, DM), BF16),
            vmem(w3_shape, BF16),
            vmem(w3_shape, BF16),
            vmem(w3_shape, BF16),
            vmem((4, 1024, DM), BF16),
            vmem((128, 2048), BF16),
            vmem((2048, 128), BF16),
            vmem((64, 8192), BF16),
            vmem((128, DH), BF16),
            vmem((B, H, DM), BF16),
            vmem((B, H, 1), F32),
            vmem((B, H, 1), F32),
            vmem((B, H, DM), F32),
            vmem((8, 64, 128), BF16),
            vmem((2, 64, DH), F32),
            vmem((H, 8, DH), F32),
            vmem((H, 8, DH), F32),
            vmem((H, 8, DH), F32),
            pltpu.SemaphoreType.DMA((3,)),
            pltpu.SemaphoreType.DMA((1,)),
            pltpu.SemaphoreType.DMA((8,)),
        ],
        compiler_params=pltpu.CompilerParams(vmem_limit_bytes=100 * 1024 * 1024),
        name="fused_decode",
    )(
        A_x.reshape(B, DM),
        A_k_cache,
        A_v_cache,
        A_wq.reshape(4, 128, H * DH),
        A_wo.reshape(4, 1024, DM),
        B_x.reshape(B, DM),
        B_c_kv.reshape(16, 1024, DM),
        B_w_q.reshape(w3_shape),
        B_w_uk.reshape(w3_shape),
        B_w_uv.reshape(w3_shape),
        B_w_o.reshape(4, 1024, DM),
    )
    return out.reshape(B, 1, 2 * DM)
```

```python
import jax
import jax.numpy as jnp
from jax import lax
import jax.experimental.pallas as pl
import jax.experimental.pallas.tpu as pltpu

F32 = jnp.float32
BF16 = jnp.bfloat16

B = 4
H = 32
DH = 128
DM = 512
SK = 4096
W = 1024
SCALE = DH ** -0.5

NP = 32
NT = (((1,), (1,)), ((), ()))


def _iota(shape, d):
    return lax.broadcasted_iota(jnp.int32, shape, d)


def _dot(a, b):
    return jnp.dot(a, b, preferred_element_type=F32)


def _dot_nt(a, b):
    return lax.dot_general(a, b, NT, preferred_element_type=F32)


def _kernel(
    xa_hbm, k_hbm, v_hbm, wq_hbm, wo_hbm,
    xb_hbm, c_hbm, bq_hbm, buk_hbm, buv_hbm, bo_hbm,
    o_ref,
    xa_v, xb_v, kv_v, wq_v, wo_v, c_v, bq_v, buk_v, buv_v, bo_v,
    e_v, et_v, x2_v, qb_v, qabs_v, m_v, l_v, acc_v, cn_v, ctx_v,
    qa_v, oa_v, ob_v,
    sems, xsem, fsems,
):
    def start(src, dst, sem, prio):
        pltpu.make_async_copy(src, dst, sem).start(priority=prio)

    def wait(dst, sem):
        pltpu.make_async_copy(dst, dst, sem).wait()

    def issue_w3(src, dst, t, j, sem, prio):
        start(src.at[:, t * NP + j], dst.at[:, t * NP + j], sem, prio)

    def issue_s0(t, j0, j1):
        sem = sems.at[t % 3]
        for j in range(j0, j1):
            issue_w3(bq_hbm, bq_v, t, j, sem, 0)
            issue_w3(buk_hbm, buk_v, t, j, sem, 1)

    def wait_s0(t):
        sem = sems.at[t % 3]
        wait(bq_v.at[:, pl.ds(t * NP, NP)], sem)
        wait(buk_v.at[:, pl.ds(t * NP, NP)], sem)

    def issue_s1(t, j0, j1):
        sem = sems.at[(4 + t) % 3]
        for j in range(j0, j1):
            idx = (slice(None), pl.ds((t * 4 + j // 8) * 8, 8), pl.ds((j % 8) * 512, 512))
            start(wq_hbm.at[idx], wq_v.at[idx], sem, 0)
            issue_w3(buv_hbm, buv_v, t, j, sem, 1)

    def wait_s1(t):
        sem = sems.at[(4 + t) % 3]
        wait(wq_v.at[:, pl.ds(t * 32, 32), :], sem)
        wait(buv_v.at[:, pl.ds(t * NP, NP)], sem)

    def issue_c(i, j0, j1):
        sem = sems.at[(8 + i) % 3]
        p0 = (i // 4) * 8
        r0 = (i % 4) * 256
        for j in range(j0, j1):
            for u in range(2):
                idx = (pl.ds(p0 + u * 4, 4), pl.ds(pl.multiple_of(r0 + j * 8, 8), 8), slice(None))
                start(c_hbm.at[idx], c_v.at[idx], sem, u)

    def wait_c(i):
        sem = sems.at[(8 + i) % 3]
        p0 = (i // 4) * 8
        r0 = pl.multiple_of((i % 4) * 256, 256)
        wait(c_v.at[pl.ds(p0, 8), pl.ds(r0, 256), :], sem)

    def issue_kv(g, j0, j1):
        slot = (16 + g) % 3
        sem = sems.at[slot]
        for j in range(j0, j1):
            for u, src in enumerate((k_hbm, v_hbm)):
                start(src.at[g // 8, pl.ds((g % 8) * 4, 4), pl.ds(SK - W + j * 32, 32), :],
                      kv_v.at[slot, u, :, pl.ds(j * 32, 32), :], sem, u)

    def wait_kv(g):
        slot = (16 + g) % 3
        wait(kv_v.at[slot], sems.at[slot])

    def issue_o(u):
        sem = fsems.at[u]
        for j in range(16):
            idx = (slice(None), pl.ds(pl.multiple_of(u * 128 + j * 8, 8), 8), slice(None))
            start(wo_hbm.at[idx], wo_v.at[idx], sem, 0)
            start(bo_hbm.at[idx], bo_v.at[idx], sem, 1)

    def wait_o(u):
        sem = fsems.at[u]
        wait(wo_v.at[:, pl.ds(u * 128, 128), :], sem)
        wait(bo_v.at[:, pl.ds(u * 128, 128), :], sem)

    def diag_mask():
        return (_iota((64, 2048), 1) & 15) == (_iota((64, 2048), 0) & 15)

    def w3(ref, k, hf):
        return ref[k, :, hf].reshape(2048, DH)

    def build_consts():
        e_v[...] = jnp.where(_iota((128, 2048), 0) == (_iota((128, 2048), 1) >> 4), 1.0, 0.0).astype(BF16)
        et_v[...] = jnp.where(_iota((2048, 128), 1) == (_iota((2048, 128), 0) >> 4), 1.0, 0.0).astype(BF16)
        m_v[...] = jnp.full(m_v.shape, -jnp.inf, F32)
        l_v[...] = jnp.zeros(l_v.shape, F32)
        acc_v[...] = jnp.zeros(acc_v.shape, F32)
        oa_v[...] = jnp.zeros(oa_v.shape, F32)

    def build_x2():
        x = xb_v[...].astype(F32)
        xrep = jnp.concatenate(
            [jnp.broadcast_to(x[b:b + 1, :], (16, DM)) for b in range(B)], axis=0).astype(BF16)
        for k in range(4):
            xe = _dot(xrep[:, k * 128:(k + 1) * 128], e_v[...])
            x2_v[:, k * 2048:(k + 1) * 2048] = jnp.where(diag_mask(), xe, 0.0).astype(BF16)

    def qb_half(hf):
        acc = None
        for k in range(4):
            r = _dot(x2_v[:, k * 2048:(k + 1) * 2048], w3(bq_v, k, hf))
            acc = r if acc is None else acc + r
        qb_v[hf * 64:(hf + 1) * 64, :] = acc.astype(BF16)

    def qabs_piece(hf, k):
        r = _dot_nt(qb_v[hf * 64:(hf + 1) * 64, :], w3(buk_v, k, hf))
        r = jnp.where(diag_mask(), r, 0.0).astype(BF16)
        z = _dot(r, et_v[...]).astype(BF16)
        for b in range(B):
            qabs_v[b, hf * 16:(hf + 1) * 16, k * 128:(k + 1) * 128] = z[b * 16:(b + 1) * 16, :]

    def qa_proj():
        x = xa_v[...].astype(F32)
        x8 = jnp.concatenate([x, x], axis=0).astype(BF16)
        acc = None
        for k in range(4):
            r = _dot(x8[:, k * 128:(k + 1) * 128], wq_v[k])
            acc = r if acc is None else acc + r
        for h in range(H):
            qa_v[h] = acc[:, h * DH:(h + 1) * DH]

    def b_attn(i, u):
        b = (i // 4) * 2 + u
        r0 = pl.multiple_of((i % 4) * 256, 256)
        c = c_v[pl.ds(b * 4, 4), pl.ds(r0, 256), :].reshape(1024, DM)
        s = _dot_nt(qabs_v[b], c) * SCALE
        m_old = m_v[b]
        m_new = jnp.maximum(m_old, jnp.max(s, axis=1, keepdims=True))
        alpha = jnp.exp(m_old - m_new)
        p = jnp.exp(s - m_new)
        l_v[b] = alpha * l_v[b] + jnp.sum(p, axis=1, keepdims=True)
        acc_v[b] = alpha * acc_v[b] + _dot(p.astype(BF16), c)
        m_v[b] = m_new

    def b_norm():
        for b in range(B):
            cn = (acc_v[b] / l_v[b]).astype(BF16)
            for hf in range(2):
                for k in range(4):
                    cn_v[hf * 4 + k, b * 16:(b + 1) * 16, :] = (
                        cn[hf * 16:(hf + 1) * 16, k * 128:(k + 1) * 128])
        ctx_v[...] = jnp.zeros(ctx_v.shape, F32)

    def ctx_piece(i):
        xe = _dot(cn_v[i], e_v[...])
        xe = jnp.where(diag_mask(), xe, 0.0).astype(BF16)
        ctx_v[i // 4] += _dot(xe, w3(buv_v, i % 4, i // 4))

    def ob_build():
        ro = _iota((256, 128), 0)
        ri = _iota((256, 128), 1)
        src = ((ro >> 7) << 6) + ((ro & 7) << 4) + ((ro >> 3) & 15)
        perm = jnp.where(((ro & 7) < 4) & (ri == src), 1.0, 0.0).astype(BF16)
        ctx = ctx_v[...].reshape(128, DH).astype(BF16)
        ob_v[...] = _dot(perm, ctx).reshape(H, 8, DH)

    def a_group(g):
        slot = (16 + g) % 3
        keep = _iota((8, DH), 0) == g // 8
        for j in range(4):
            h = (g % 8) * 4 + j
            s = _dot_nt(qa_v[h].astype(BF16), kv_v[slot, 0, j]) * SCALE
            p = jnp.exp(s - jnp.max(s, axis=1, keepdims=True))
            l = jnp.sum(p, axis=1, keepdims=True)
            o = _dot(p.astype(BF16), kv_v[slot, 1, j]) / l
            oa_v[h] = jnp.where(keep, o, oa_v[h])

    def o_unit(u, acc_a, acc_b):
        for p in range(4):
            h = p * 8 + u
            acc_a += _dot(oa_v[h].astype(BF16), wo_v[p, u * 128:(u + 1) * 128, :])
            acc_b += _dot(ob_v[h].astype(BF16), bo_v[p, u * 128:(u + 1) * 128, :])
        return acc_a, acc_b

    issue_s0(0, 0, 2)
    start(xa_hbm, xa_v, xsem.at[0], 0)
    start(xb_hbm, xb_v, xsem.at[0], 0)
    issue_s0(0, 2, NP)
    issue_s0(1, 0, NP)

    issue_s0(2, 0, NP)
    wait_s0(0)
    wait(xa_v, xsem.at[0])
    wait(xb_v, xsem.at[0])
    build_consts()

    issue_s0(3, 0, NP)
    wait_s0(1)
    build_x2()

    issue_s1(0, 0, NP)
    wait_s0(2)

    issue_s1(1, 0, 16)
    wait_s0(3)
    qb_half(0)
    issue_s1(1, 16, NP)
    qb_half(1)

    for hf in range(2):
        issue_s1(2 + hf, 0, 16)
        wait_s1(hf)
        qabs_piece(hf, 0)
        qabs_piece(hf, 1)
        issue_s1(2 + hf, 16, NP)
        qabs_piece(hf, 2)
        qabs_piece(hf, 3)

    issue_c(0, 0, NP)
    wait_s1(2)

    issue_c(1, 0, NP)
    wait_s1(3)
    qa_proj()

    def b_body(i, carry):
        for u in range(2):
            @pl.when(i < 6)
            def _():
                issue_c(i + 2, u * 16, (u + 1) * 16)

            @pl.when(i >= 6)
            def _():
                issue_kv(i - 6, u * 16, (u + 1) * 16)

            if u == 0:
                wait_c(i)
            b_attn(i, u)
        return carry

    lax.fori_loop(0, 8, b_body, 0)
    b_norm()

    def a_body(h, carry):
        @pl.when(h < H - 2)
        def _():
            issue_kv(h + 2, 0, NP)

        @pl.when(h >= H - 2)
        def _():
            u = (h - (H - 2)) * 2
            issue_o(u)
            issue_o(u + 1)

        wait_kv(h)
        a_group(h)

        @pl.when(h < 8)
        def _():
            ctx_piece(h)

        return carry

    lax.fori_loop(0, H, a_body, 0)

    acc_a = jnp.zeros((8, DM), F32)
    acc_b = jnp.zeros((8, DM), F32)
    issue_o(4)
    issue_o(5)
    ob_build()
    for u in range(2):
        wait_o(u)
        acc_a, acc_b = o_unit(u, acc_a, acc_b)
    issue_o(6)
    issue_o(7)
    for u in range(2, 8):
        wait_o(u)
        acc_a, acc_b = o_unit(u, acc_a, acc_b)

    o_ref[:, 0:DM] = acc_a[0:B, :].astype(o_ref.dtype)
    o_ref[:, DM:2 * DM] = acc_b[0:B, :].astype(o_ref.dtype)


@jax.jit
def pallas_concat_heads__sliding_block_cached__compressed_kv_cla__decode_kernel(
    A_x: jax.Array,
    A_k_cache: jax.Array,
    A_v_cache: jax.Array,
    A_wq: jax.Array,
    A_wo: jax.Array,
    B_x: jax.Array,
    B_c_kv: jax.Array,
    B_w_q: jax.Array,
    B_w_uk: jax.Array,
    B_w_uv: jax.Array,
    B_w_o: jax.Array,
):
    w3_shape = (4, 128, 2, 16, DH)
    hbm = pl.BlockSpec(memory_space=pl.ANY)
    vmem = pltpu.VMEM
    out = pl.pallas_call(
        _kernel,
        out_shape=jax.ShapeDtypeStruct((B, 2 * DM), BF16),
        in_specs=[hbm] * 11,
        out_specs=pl.BlockSpec(memory_space=pltpu.VMEM),
        scratch_shapes=[
            vmem((B, DM), BF16),
            vmem((B, DM), BF16),
            vmem((3, 2, B, W, DH), BF16),
            vmem((4, 128, H * DH), BF16),
            vmem((4, 1024, DM), BF16),
            vmem((16, 1024, DM), BF16),
            vmem(w3_shape, BF16),
            vmem(w3_shape, BF16),
            vmem(w3_shape, BF16),
            vmem((4, 1024, DM), BF16),
            vmem((128, 2048), BF16),
            vmem((2048, 128), BF16),
            vmem((64, 8192), BF16),
            vmem((128, DH), BF16),
            vmem((B, H, DM), BF16),
            vmem((B, H, 1), F32),
            vmem((B, H, 1), F32),
            vmem((B, H, DM), F32),
            vmem((8, 64, 128), BF16),
            vmem((2, 64, DH), F32),
            vmem((H, 8, DH), F32),
            vmem((H, 8, DH), F32),
            vmem((H, 8, DH), F32),
            pltpu.SemaphoreType.DMA((3,)),
            pltpu.SemaphoreType.DMA((1,)),
            pltpu.SemaphoreType.DMA((8,)),
        ],
        compiler_params=pltpu.CompilerParams(vmem_limit_bytes=100 * 1024 * 1024),
        name="fused_decode",
    )(
        A_x.reshape(B, DM),
        A_k_cache,
        A_v_cache,
        A_wq.reshape(4, 128, H * DH),
        A_wo.reshape(4, 1024, DM),
        B_x.reshape(B, DM),
        B_c_kv.reshape(16, 1024, DM),
        B_w_q.reshape(w3_shape),
        B_w_uk.reshape(w3_shape),
        B_w_uv.reshape(w3_shape),
        B_w_o.reshape(4, 1024, DM),
    )
    return out.reshape(B, 1, 2 * DM)
```

```python
import jax
import jax.numpy as jnp
from jax import lax
import jax.experimental.pallas as pl
import jax.experimental.pallas.tpu as pltpu

F32 = jnp.float32
BF16 = jnp.bfloat16

B = 4
H = 32
DH = 128
DM = 512
SK = 4096
W = 1024
SCALE = DH ** -0.5

NP = 32
NT = (((1,), (1,)), ((), ()))


def _iota(shape, d):
    return lax.broadcasted_iota(jnp.int32, shape, d)


def _dot(a, b):
    return jnp.dot(a, b, preferred_element_type=F32)


def _dot_nt(a, b):
    return lax.dot_general(a, b, NT, preferred_element_type=F32)


def _kernel(
    xa_hbm, k_hbm, v_hbm, wq_hbm, wo_hbm,
    xb_hbm, c_hbm, bq_hbm, buk_hbm, buv_hbm, bo_hbm,
    o_ref,
    xa_v, xb_v, kv_v, wq_v, wo_v, c_v, bq_v, buk_v, buv_v, bo_v,
    e_v, et_v, x2_v, qb_v, qabs_v, m_v, l_v, acc_v, cn_v, ctx_v,
    qa_v, oa_v, ob_v,
    sems, xsem, fsems,
):
    def start(src, dst, sem, prio):
        pltpu.make_async_copy(src, dst, sem).start(priority=prio)

    def wait(dst, sem):
        pltpu.make_async_copy(dst, dst, sem).wait()

    def issue_w3(src, dst, t, j, sem, prio):
        start(src.at[:, t * NP + j], dst.at[:, t * NP + j], sem, prio)

    def issue_s0(t, j0, j1):
        sem = sems.at[t % 3]
        for j in range(j0, j1):
            issue_w3(bq_hbm, bq_v, t, j, sem, 1 if (t == 0 and j < 16) else 0)
            issue_w3(buk_hbm, buk_v, t, j, sem, 1)

    def wait_s0(t):
        sem = sems.at[t % 3]
        wait(bq_v.at[:, pl.ds(t * NP, NP)], sem)
        wait(buk_v.at[:, pl.ds(t * NP, NP)], sem)

    def issue_s1(t, j0, j1):
        sem = sems.at[(4 + t) % 3]
        for j in range(j0, j1):
            idx = (slice(None), pl.ds((t * 4 + j // 8) * 8, 8), pl.ds((j % 8) * 512, 512))
            start(wq_hbm.at[idx], wq_v.at[idx], sem, 0)
            issue_w3(buv_hbm, buv_v, t, j, sem, 1)

    def wait_s1(t):
        sem = sems.at[(4 + t) % 3]
        wait(wq_v.at[:, pl.ds(t * 32, 32), :], sem)
        wait(buv_v.at[:, pl.ds(t * NP, NP)], sem)

    def issue_c(i, lo, j0, j1):
        sem = sems.at[(8 + i) % 3]
        r0 = (i % 4) * 256
        for j in range(j0, j1):
            rows8 = pl.ds(pl.multiple_of(r0 + j * 8, 8), 8)
            idx = (pl.ds(2 if lo else 10, 4), rows8, slice(None))
            start(c_hbm.at[idx], c_v.at[idx], sem, 0)
            if lo:
                idx = (pl.ds(6, 4), rows8, slice(None))
            else:
                idx = (pl.ds(14 if j % 2 == 0 else 0, 2),
                       pl.ds(pl.multiple_of(r0 + (j // 2) * 16, 16), 16), slice(None))
            start(c_hbm.at[idx], c_v.at[idx], sem, 1)

    def c_parts(i):
        ph = (i // 4) * 8
        return ((2 + ph, 2), (4 + ph, 4), ((8 + ph) % 16, 2))

    def wait_c(i):
        sem = sems.at[(8 + i) % 3]
        r0 = pl.multiple_of((i % 4) * 256, 256)
        for p0, n in c_parts(i):
            wait(c_v.at[pl.ds(p0, n), pl.ds(r0, 256), :], sem)

    def issue_kv(g, j0, j1):
        slot = (16 + g) % 3
        sem = sems.at[slot]
        for j in range(j0, j1):
            for u, src in enumerate((k_hbm, v_hbm)):
                if isinstance(g, int) and g == 0:
                    hh, r = j % 2, (j // 2) * 64
                    start(src.at[pl.ds(126 if hh == 0 else 0, 2), pl.ds(SK - W + r, 64), :],
                          kv_v.at[slot, u, pl.ds(hh * 2, 2), pl.ds(r, 64), :], sem, u)
                else:
                    start(src.at[pl.ds(g * 4 - 2, 4), pl.ds(SK - W + j * 32, 32), :],
                          kv_v.at[slot, u, :, pl.ds(j * 32, 32), :], sem, u)

    def wait_kv(g):
        slot = (16 + g) % 3
        wait(kv_v.at[slot], sems.at[slot])

    def issue_o(t):
        for j in range(NP):
            idx = (pl.ds((j % 2) * 4, 4), pl.ds(pl.multiple_of(t * 128 + (j // 2) * 8, 8), 8), slice(None))
            start(wo_hbm.at[idx], wo_v.at[idx], fsems.at[2 * t], 0)
            start(bo_hbm.at[idx], bo_v.at[idx], fsems.at[2 * t + 1], 1)

    TAIL = ((0, 4), (4, 2), (6, 1), (7, 1))

    def issue_o_last():
        lo = []
        for n, (p0, k) in enumerate(TAIL):
            rows = 32 // k
            lo += [(n, (pl.ds(p0, k), pl.ds(384 + r, rows), slice(None))) for r in range(0, 128, rows)]
        for j in range(NP):
            idx = (pl.ds((j % 2) * 4, 4), pl.ds(384 + (j // 2) * 8, 8), slice(None))
            start(wo_hbm.at[idx], wo_v.at[idx], fsems.at[6], 0)
            n, idx = lo[j]
            start(bo_hbm.at[idx], bo_v.at[idx], fsems.at[7 + n], 1)

    def diag_mask():
        return (_iota((64, 2048), 1) & 15) == (_iota((64, 2048), 0) & 15)

    def w3(ref, k, hf):
        return ref[k, :, hf].reshape(2048, DH)

    def build_consts():
        e_v[...] = jnp.where(_iota((128, 2048), 0) == (_iota((128, 2048), 1) >> 4), 1.0, 0.0).astype(BF16)
        et_v[...] = jnp.where(_iota((2048, 128), 1) == (_iota((2048, 128), 0) >> 4), 1.0, 0.0).astype(BF16)
        m_v[...] = jnp.full(m_v.shape, -jnp.inf, F32)
        l_v[...] = jnp.zeros(l_v.shape, F32)
        acc_v[...] = jnp.zeros(acc_v.shape, F32)
        oa_v[...] = jnp.zeros(oa_v.shape, F32)

    def build_x2():
        x = xb_v[...].astype(F32)
        xrep = jnp.concatenate(
            [jnp.broadcast_to(x[b:b + 1, :], (16, DM)) for b in range(B)], axis=0).astype(BF16)
        for k in range(4):
            xe = _dot(xrep[:, k * 128:(k + 1) * 128], e_v[...])
            x2_v[:, k * 2048:(k + 1) * 2048] = jnp.where(diag_mask(), xe, 0.0).astype(BF16)

    def qb_half(hf):
        acc = None
        for k in range(4):
            r = _dot(x2_v[:, k * 2048:(k + 1) * 2048], w3(bq_v, k, hf))
            acc = r if acc is None else acc + r
        qb_v[hf * 64:(hf + 1) * 64, :] = acc.astype(BF16)

    def qabs_piece(hf, k):
        r = _dot_nt(qb_v[hf * 64:(hf + 1) * 64, :], w3(buk_v, k, hf))
        r = jnp.where(diag_mask(), r, 0.0).astype(BF16)
        z = _dot(r, et_v[...]).astype(BF16)
        for b in range(B):
            qabs_v[b, hf * 16:(hf + 1) * 16, k * 128:(k + 1) * 128] = z[b * 16:(b + 1) * 16, :]

    def qa_proj():
        x = xa_v[...].astype(F32)
        x8 = jnp.concatenate([x, x], axis=0).astype(BF16)
        acc = None
        for k in range(4):
            r = _dot(x8[:, k * 128:(k + 1) * 128], wq_v[k])
            acc = r if acc is None else acc + r
        for h in range(H):
            qa_v[h] = acc[:, h * DH:(h + 1) * DH]

    def b_attn(i, part):
        p0, n = c_parts(i)[part]
        b = p0 // 4
        r0 = pl.multiple_of((i % 4) * 256, 256)
        c = c_v[pl.ds(p0, n), pl.ds(r0, 256), :].reshape(n * 256, DM)
        s = _dot_nt(qabs_v[b], c) * SCALE
        m_old = m_v[b]
        m_new = jnp.maximum(m_old, jnp.max(s, axis=1, keepdims=True))
        alpha = jnp.exp(m_old - m_new)
        p = jnp.exp(s - m_new)
        l_v[b] = alpha * l_v[b] + jnp.sum(p, axis=1, keepdims=True)
        acc_v[b] = alpha * acc_v[b] + _dot(p.astype(BF16), c)
        m_v[b] = m_new

    def b_norm():
        for b in range(B):
            cn = (acc_v[b] / l_v[b]).astype(BF16)
            for hf in range(2):
                for k in range(4):
                    cn_v[hf * 4 + k, b * 16:(b + 1) * 16, :] = (
                        cn[hf * 16:(hf + 1) * 16, k * 128:(k + 1) * 128])
        ctx_v[...] = jnp.zeros(ctx_v.shape, F32)

    def ctx_piece(i):
        xe = _dot(cn_v[i], e_v[...])
        xe = jnp.where(diag_mask(), xe, 0.0).astype(BF16)
        ctx_v[i // 4] += _dot(xe, w3(buv_v, i % 4, i // 4))

    def ob_build():
        ro = _iota((256, 128), 0)
        ri = _iota((256, 128), 1)
        src = ((ro >> 7) << 6) + ((ro & 7) << 4) + ((ro >> 3) & 15)
        perm = jnp.where(((ro & 7) < 4) & (ri == src), 1.0, 0.0).astype(BF16)
        ctx = ctx_v[...].reshape(128, DH).astype(BF16)
        ob_v[...] = _dot(perm, ctx).reshape(H, 8, DH)

    def a_group(g):
        slot = (16 + g) % 3
        for j in range(4):
            f = (g * 4 + (126 + j)) & 127
            h = f & 31
            s = _dot_nt(qa_v[h].astype(BF16), kv_v[slot, 0, j]) * SCALE
            p = jnp.exp(s - jnp.max(s, axis=1, keepdims=True))
            l = jnp.sum(p, axis=1, keepdims=True)
            o = _dot(p.astype(BF16), kv_v[slot, 1, j]) / l
            oa_v[h] = jnp.where(_iota((8, DH), 0) == (f >> 5), o, oa_v[h])

    def o_proj(acc, o_v, w_v, sem, t, p0, n):
        wait(w_v.at[pl.ds(p0, n), pl.ds(t * 128, 128), :], sem)
        for p in range(p0, p0 + n):
            acc += _dot(o_v[p * 4 + t].astype(BF16), w_v[p, t * 128:(t + 1) * 128, :])
        return acc

    issue_s0(0, 0, 2)
    start(xa_hbm, xa_v, xsem.at[0], 0)
    start(xb_hbm, xb_v, xsem.at[0], 0)
    issue_s0(0, 2, NP)
    issue_s0(1, 0, NP)

    issue_s0(2, 0, NP)
    wait_s0(0)
    wait(xa_v, xsem.at[0])
    wait(xb_v, xsem.at[0])
    build_consts()

    issue_s0(3, 0, NP)
    wait_s0(1)
    build_x2()

    issue_s1(0, 0, NP)
    wait_s0(2)

    issue_s1(1, 0, 16)
    wait_s0(3)
    qb_half(0)
    issue_s1(1, 16, NP)
    qb_half(1)

    for hf in range(2):
        issue_s1(2 + hf, 0, 16)
        wait_s1(hf)
        qabs_piece(hf, 0)
        qabs_piece(hf, 1)
        issue_s1(2 + hf, 16, NP)
        qabs_piece(hf, 2)
        qabs_piece(hf, 3)

    issue_c(0, True, 0, NP)
    wait_s1(2)

    issue_c(1, True, 0, NP)
    wait_s1(3)
    qa_proj()

    def b_body(i, carry):
        for u in range(2):
            j0, j1 = u * 16, (u + 1) * 16
            pl.when(i < 2)(lambda: issue_c(i + 2, True, j0, j1))
            pl.when((i >= 2) & (i < 6))(lambda: issue_c(i + 2, False, j0, j1))
            pl.when(i == 6)(lambda: issue_kv(0, j0, j1))
            pl.when(i == 7)(lambda: issue_kv(1, j0, j1))
            if u == 0:
                wait_c(i)
                b_attn(i, 0)
                b_attn(i, 2)
            else:
                b_attn(i, 1)
        return carry

    lax.fori_loop(0, 8, b_body, 0)
    b_norm()

    def a_body(g, carry):
        pl.when(g < H - 2)(lambda: issue_kv(g + 2, 0, NP))
        pl.when(g >= H - 2)(lambda: issue_o(g - (H - 2)))
        wait_kv(g)
        a_group(g)
        pl.when(g < 8)(lambda: ctx_piece(g))
        return carry

    lax.fori_loop(0, H, a_body, 0)

    acc_a = jnp.zeros((8, DM), F32)
    acc_b = jnp.zeros((8, DM), F32)
    issue_o(2)
    ob_build()
    acc_a = o_proj(acc_a, oa_v, wo_v, fsems.at[0], 0, 0, 8)
    acc_b = o_proj(acc_b, ob_v, bo_v, fsems.at[1], 0, 0, 8)
    issue_o_last()
    for t in (1, 2):
        acc_a = o_proj(acc_a, oa_v, wo_v, fsems.at[2 * t], t, 0, 8)
        acc_b = o_proj(acc_b, ob_v, bo_v, fsems.at[2 * t + 1], t, 0, 8)
    acc_a = o_proj(acc_a, oa_v, wo_v, fsems.at[6], 3, 0, 8)
    o_ref[:, 0:DM] = acc_a[0:B, :].astype(o_ref.dtype)
    for n, (p0, k) in enumerate(TAIL):
        acc_b = o_proj(acc_b, ob_v, bo_v, fsems.at[7 + n], 3, p0, k)
    o_ref[:, DM:2 * DM] = acc_b[0:B, :].astype(o_ref.dtype)


@jax.jit
def pallas_concat_heads__sliding_block_cached__compressed_kv_cla__decode_kernel(
    A_x: jax.Array,
    A_k_cache: jax.Array,
    A_v_cache: jax.Array,
    A_wq: jax.Array,
    A_wo: jax.Array,
    B_x: jax.Array,
    B_c_kv: jax.Array,
    B_w_q: jax.Array,
    B_w_uk: jax.Array,
    B_w_uv: jax.Array,
    B_w_o: jax.Array,
):
    w3_shape = (4, 128, 2, 16, DH)
    hbm = pl.BlockSpec(memory_space=pl.ANY)
    vmem = pltpu.VMEM
    out = pl.pallas_call(
        _kernel,
        out_shape=jax.ShapeDtypeStruct((B, 2 * DM), BF16),
        in_specs=[hbm] * 11,
        out_specs=pl.BlockSpec(memory_space=pltpu.VMEM),
        scratch_shapes=[
            vmem((B, DM), BF16),
            vmem((B, DM), BF16),
            vmem((3, 2, B, W, DH), BF16),
            vmem((4, 128, H * DH), BF16),
            vmem((8, 512, DM), BF16),
            vmem((16, 1024, DM), BF16),
            vmem(w3_shape, BF16),
            vmem(w3_shape, BF16),
            vmem(w3_shape, BF16),
            vmem((8, 512, DM), BF16),
            vmem((128, 2048), BF16),
            vmem((2048, 128), BF16),
            vmem((64, 8192), BF16),
            vmem((128, DH), BF16),
            vmem((B, H, DM), BF16),
            vmem((B, H, 1), F32),
            vmem((B, H, 1), F32),
            vmem((B, H, DM), F32),
            vmem((8, 64, 128), BF16),
            vmem((2, 64, DH), F32),
            vmem((H, 8, DH), F32),
            vmem((H, 8, DH), F32),
            vmem((H, 8, DH), F32),
            pltpu.SemaphoreType.DMA((3,)),
            pltpu.SemaphoreType.DMA((1,)),
            pltpu.SemaphoreType.DMA((11,)),
        ],
        compiler_params=pltpu.CompilerParams(
            vmem_limit_bytes=100 * 1024 * 1024, disable_semaphore_checks=True),
        name="fused_decode",
    )(
        A_x.reshape(B, DM),
        A_k_cache.reshape(B * H, SK, DH),
        A_v_cache.reshape(B * H, SK, DH),
        A_wq.reshape(4, 128, H * DH),
        A_wo.reshape(8, 512, DM),
        B_x.reshape(B, DM),
        B_c_kv.reshape(16, 1024, DM),
        B_w_q.reshape(w3_shape),
        B_w_uk.reshape(w3_shape),
        B_w_uv.reshape(w3_shape),
        B_w_o.reshape(8, 512, DM),
    )
    return out.reshape(B, 1, 2 * DM)
```

```python
import jax
import jax.numpy as jnp
from jax import lax
import jax.experimental.pallas as pl
import jax.experimental.pallas.tpu as pltpu

F32 = jnp.float32
BF16 = jnp.bfloat16

B = 4
H = 32
DH = 128
DM = 512
SK = 4096
W = 1024
SCALE = DH ** -0.5

NP = 32
NT = (((1,), (1,)), ((), ()))


def _iota(shape, d):
    return lax.broadcasted_iota(jnp.int32, shape, d)


def _dot(a, b):
    return jnp.dot(a, b, preferred_element_type=F32)


def _dot_nt(a, b):
    return lax.dot_general(a, b, NT, preferred_element_type=F32)


def _kernel(
    xa_hbm, k_hbm, v_hbm, wq_hbm, wo_hbm,
    xb_hbm, c_hbm, bq_hbm, buk_hbm, buv_hbm, bo_hbm,
    o_ref,
    xa_v, xb_v, kv_v, wq_v, wo_v, c_v, bq_v, buk_v, buv_v, bo_v,
    e_v, et_v, x2_v, qb_v, qabs_v, m_v, l_v, acc_v, cn_v, ctx_v,
    qa_v, oa_v, ob_v,
    sems, xsem, fsems,
):
    def start(src, dst, sem, prio):
        pltpu.make_async_copy(src, dst, sem).start(priority=prio)

    def wait(dst, sem):
        pltpu.make_async_copy(dst, dst, sem).wait()

    def issue_w3(src, dst, t, j, sem, prio):
        start(src.at[:, t * NP + j], dst.at[:, t * NP + j], sem, prio)

    def issue_s0(t, j0, j1):
        sem = sems.at[t % 3]
        for j in range(j0, j1):
            issue_w3(bq_hbm, bq_v, t, j, sem, 1 if (t == 0 and j < 16) else 0)
            issue_w3(buk_hbm, buk_v, t, j, sem, 1)

    def wait_s0(t):
        sem = sems.at[t % 3]
        wait(bq_v.at[:, pl.ds(t * NP, NP)], sem)
        wait(buk_v.at[:, pl.ds(t * NP, NP)], sem)

    def issue_s1(t, j0, j1):
        sem = sems.at[(4 + t) % 3]
        for j in range(j0, j1):
            idx = (slice(None), pl.ds((t * 4 + j // 8) * 8, 8), pl.ds((j % 8) * 512, 512))
            start(wq_hbm.at[idx], wq_v.at[idx], sem, 0)
            issue_w3(buv_hbm, buv_v, t, j, sem, 1)

    def wait_s1(t):
        sem = sems.at[(4 + t) % 3]
        wait(wq_v.at[:, pl.ds(t * 32, 32), :], sem)
        wait(buv_v.at[:, pl.ds(t * NP, NP)], sem)

    def issue_c(i, lo, j0, j1):
        sem = sems.at[(8 + i) % 3]
        r0 = (i % 4) * 256
        for j in range(j0, j1):
            rows8 = pl.ds(pl.multiple_of(r0 + j * 8, 8), 8)
            idx = (pl.ds(2 if lo else 10, 4), rows8, slice(None))
            start(c_hbm.at[idx], c_v.at[idx], sem, 0)
            if lo:
                idx = (pl.ds(6, 4), rows8, slice(None))
            else:
                idx = (pl.ds(14 if j % 2 == 0 else 0, 2),
                       pl.ds(pl.multiple_of(r0 + (j // 2) * 16, 16), 16), slice(None))
            start(c_hbm.at[idx], c_v.at[idx], sem, 1)

    def c_parts(i):
        ph = (i // 4) * 8
        return ((2 + ph, 2), (4 + ph, 4), ((8 + ph) % 16, 2))

    def wait_c(i):
        sem = sems.at[(8 + i) % 3]
        r0 = pl.multiple_of((i % 4) * 256, 256)
        for p0, n in c_parts(i):
            wait(c_v.at[pl.ds(p0, n), pl.ds(r0, 256), :], sem)

    def issue_kv(g, j0, j1):
        slot = (16 + g) % 3
        sem = sems.at[slot]
        for j in range(j0, j1):
            for u, src in enumerate((k_hbm, v_hbm)):
                if isinstance(g, int) and g == 0:
                    hh, r = j % 2, (j // 2) * 64
                    start(src.at[pl.ds(126 if hh == 0 else 0, 2), pl.ds(SK - W + r, 64), :],
                          kv_v.at[slot, u, pl.ds(hh * 2, 2), pl.ds(r, 64), :], sem, u)
                else:
                    start(src.at[pl.ds(g * 4 - 2, 4), pl.ds(SK - W + j * 32, 32), :],
                          kv_v.at[slot, u, :, pl.ds(j * 32, 32), :], sem, u)

    def wait_kv(g):
        slot = (16 + g) % 3
        wait(kv_v.at[slot], sems.at[slot])

    def issue_o(t):
        for j in range(NP):
            idx = (pl.ds((j % 2) * 4, 4), pl.ds(pl.multiple_of(t * 128 + (j // 2) * 8, 8), 8), slice(None))
            start(wo_hbm.at[idx], wo_v.at[idx], fsems.at[2 * t], 0)
            start(bo_hbm.at[idx], bo_v.at[idx], fsems.at[2 * t + 1], 1)

    TAIL = ((0, 4), (4, 2), (6, 1), (7, 1))

    def issue_o_last():
        lo = []
        for n, (p0, k) in enumerate(TAIL):
            rows = 32 // k
            lo += [(n, (pl.ds(p0, k), pl.ds(384 + r, rows), slice(None))) for r in range(0, 128, rows)]
        for j in range(NP):
            idx = (pl.ds((j % 2) * 4, 4), pl.ds(384 + (j // 2) * 8, 8), slice(None))
            start(wo_hbm.at[idx], wo_v.at[idx], fsems.at[6], 0)
            n, idx = lo[j]
            start(bo_hbm.at[idx], bo_v.at[idx], fsems.at[7 + n], 1)

    def diag_mask():
        return (_iota((64, 2048), 1) & 15) == (_iota((64, 2048), 0) & 15)

    def w3(ref, k, hf):
        return ref[k, :, hf].reshape(2048, DH)

    def build_consts():
        e_v[...] = jnp.where(_iota((128, 2048), 0) == (_iota((128, 2048), 1) >> 4), 1.0, 0.0).astype(BF16)
        et_v[...] = jnp.where(_iota((2048, 128), 1) == (_iota((2048, 128), 0) >> 4), 1.0, 0.0).astype(BF16)
        m_v[...] = jnp.full(m_v.shape, -jnp.inf, F32)
        l_v[...] = jnp.zeros(l_v.shape, F32)
        acc_v[...] = jnp.zeros(acc_v.shape, F32)
        oa_v[...] = jnp.zeros(oa_v.shape, F32)

    def build_x2():
        x = xb_v[...].astype(F32)
        xrep = jnp.concatenate(
            [jnp.broadcast_to(x[b:b + 1, :], (16, DM)) for b in range(B)], axis=0).astype(BF16)
        for k in range(4):
            xe = _dot(xrep[:, k * 128:(k + 1) * 128], e_v[...])
            x2_v[:, k * 2048:(k + 1) * 2048] = jnp.where(diag_mask(), xe, 0.0).astype(BF16)

    def qb_half(hf):
        acc = None
        for k in range(4):
            r = _dot(x2_v[:, k * 2048:(k + 1) * 2048], w3(bq_v, k, hf))
            acc = r if acc is None else acc + r
        qb_v[hf * 64:(hf + 1) * 64, :] = acc.astype(BF16)

    def qabs_piece(hf, k):
        r = _dot_nt(qb_v[hf * 64:(hf + 1) * 64, :], w3(buk_v, k, hf))
        r = jnp.where(diag_mask(), r, 0.0).astype(BF16)
        z = _dot(r, et_v[...]).astype(BF16)
        for b in range(B):
            qabs_v[b, hf * 16:(hf + 1) * 16, k * 128:(k + 1) * 128] = z[b * 16:(b + 1) * 16, :]

    def qa_proj():
        x = xa_v[...].astype(F32)
        x8 = jnp.concatenate([x, x], axis=0).astype(BF16)
        acc = None
        for k in range(4):
            r = _dot(x8[:, k * 128:(k + 1) * 128], wq_v[k])
            acc = r if acc is None else acc + r
        for h in range(H):
            qa_v[h] = acc[:, h * DH:(h + 1) * DH]

    def b_attn(i, part):
        p0, n = c_parts(i)[part]
        b = p0 // 4
        r0 = pl.multiple_of((i % 4) * 256, 256)
        c = c_v[pl.ds(p0, n), pl.ds(r0, 256), :].reshape(n * 256, DM)
        s = _dot_nt(qabs_v[b], c) * SCALE
        m_old = m_v[b]
        m_new = jnp.maximum(m_old, jnp.max(s, axis=1, keepdims=True))
        alpha = jnp.exp(m_old - m_new)
        p = jnp.exp(s - m_new)
        l_v[b] = alpha * l_v[b] + jnp.sum(p, axis=1, keepdims=True)
        acc_v[b] = alpha * acc_v[b] + _dot(p.astype(BF16), c)
        m_v[b] = m_new

    def b_norm():
        for b in range(B):
            cn = (acc_v[b] / l_v[b]).astype(BF16)
            for hf in range(2):
                for k in range(4):
                    cn_v[hf * 4 + k, b * 16:(b + 1) * 16, :] = (
                        cn[hf * 16:(hf + 1) * 16, k * 128:(k + 1) * 128])
        ctx_v[...] = jnp.zeros(ctx_v.shape, F32)

    def ctx_piece(i):
        xe = _dot(cn_v[i], e_v[...])
        xe = jnp.where(diag_mask(), xe, 0.0).astype(BF16)
        ctx_v[i // 4] += _dot(xe, w3(buv_v, i % 4, i // 4))

    def ob_build():
        ro = _iota((256, 128), 0)
        ri = _iota((256, 128), 1)
        src = ((ro >> 7) << 6) + ((ro & 7) << 4) + ((ro >> 3) & 15)
        perm = jnp.where(((ro & 7) < 4) & (ri == src), 1.0, 0.0).astype(BF16)
        ctx = ctx_v[...].reshape(128, DH).astype(BF16)
        ob_v[...] = _dot(perm, ctx).reshape(H, 8, DH)

    def a_group(g):
        slot = (16 + g) % 3
        for j in range(4):
            f = (g * 4 + (126 + j)) & 127
            h = f & 31
            s = _dot_nt(qa_v[h].astype(BF16), kv_v[slot, 0, j]) * SCALE
            p = jnp.exp(s - jnp.max(s, axis=1, keepdims=True))
            l = jnp.sum(p, axis=1, keepdims=True)
            o = _dot(p.astype(BF16), kv_v[slot, 1, j]) / l
            oa_v[h] = jnp.where(_iota((8, DH), 0) == (f >> 5), o, oa_v[h])

    def o_proj(acc, o_v, w_v, sem, t, p0, n):
        wait(w_v.at[pl.ds(p0, n), pl.ds(t * 128, 128), :], sem)
        for p in range(p0, p0 + n):
            acc += _dot(o_v[p * 4 + t].astype(BF16), w_v[p, t * 128:(t + 1) * 128, :])
        return acc

    issue_s0(0, 0, 2)
    start(xa_hbm, xa_v, xsem.at[0], 0)
    start(xb_hbm, xb_v, xsem.at[0], 0)
    issue_s0(0, 2, NP)
    issue_s0(1, 0, NP)

    issue_s0(2, 0, NP)
    wait_s0(0)
    wait(xa_v, xsem.at[0])
    wait(xb_v, xsem.at[0])
    build_consts()

    issue_s0(3, 0, NP)
    wait_s0(1)
    build_x2()

    issue_s1(0, 0, NP)
    wait_s0(2)

    issue_s1(1, 0, 16)
    wait_s0(3)
    qb_half(0)
    issue_s1(1, 16, NP)
    qb_half(1)

    for hf in range(2):
        issue_s1(2 + hf, 0, 16)
        wait_s1(hf)
        qabs_piece(hf, 0)
        qabs_piece(hf, 1)
        issue_s1(2 + hf, 16, NP)
        qabs_piece(hf, 2)
        qabs_piece(hf, 3)

    issue_c(0, True, 0, NP)
    wait_s1(2)

    issue_c(1, True, 0, NP)
    wait_s1(3)
    qa_proj()

    def b_body(i, carry):
        for u in range(2):
            j0, j1 = u * 16, (u + 1) * 16
            pl.when(i < 2)(lambda: issue_c(i + 2, True, j0, j1))
            pl.when((i >= 2) & (i < 6))(lambda: issue_c(i + 2, False, j0, j1))
            pl.when(i == 6)(lambda: issue_kv(0, j0, j1))
            pl.when(i == 7)(lambda: issue_kv(1, j0, j1))
            if u == 0:
                wait_c(i)
                b_attn(i, 0)
                b_attn(i, 2)
            else:
                b_attn(i, 1)
        return carry

    lax.fori_loop(0, 8, b_body, 0)
    b_norm()

    def a_body(g, carry):
        pl.when(g < H - 2)(lambda: issue_kv(g + 2, 0, NP))
        pl.when(g >= H - 2)(lambda: issue_o(g - (H - 2)))
        wait_kv(g)
        a_group(g)
        pl.when(g < 8)(lambda: ctx_piece(g))
        return carry

    lax.fori_loop(0, H, a_body, 0)

    acc_a = jnp.zeros((8, DM), F32)
    acc_b = jnp.zeros((8, DM), F32)
    issue_o(2)
    ob_build()
    acc_a = o_proj(acc_a, oa_v, wo_v, fsems.at[0], 0, 0, 8)
    acc_b = o_proj(acc_b, ob_v, bo_v, fsems.at[1], 0, 0, 8)
    issue_o_last()
    for t in (1, 2):
        acc_a = o_proj(acc_a, oa_v, wo_v, fsems.at[2 * t], t, 0, 8)
        acc_b = o_proj(acc_b, ob_v, bo_v, fsems.at[2 * t + 1], t, 0, 8)
    acc_a = o_proj(acc_a, oa_v, wo_v, fsems.at[6], 3, 0, 8)
    o_ref[:, 0:DM] = acc_a[0:B, :].astype(o_ref.dtype)
    for n, (p0, k) in enumerate(TAIL):
        acc_b = o_proj(acc_b, ob_v, bo_v, fsems.at[7 + n], 3, p0, k)
    o_ref[:, DM:2 * DM] = acc_b[0:B, :].astype(o_ref.dtype)


@jax.jit
def pallas_concat_heads__sliding_block_cached__compressed_kv_cla__decode_kernel(
    A_x: jax.Array,
    A_k_cache: jax.Array,
    A_v_cache: jax.Array,
    A_wq: jax.Array,
    A_wo: jax.Array,
    B_x: jax.Array,
    B_c_kv: jax.Array,
    B_w_q: jax.Array,
    B_w_uk: jax.Array,
    B_w_uv: jax.Array,
    B_w_o: jax.Array,
):
    w3_shape = (4, 128, 2, 16, DH)
    hbm = pl.BlockSpec(memory_space=pl.ANY)
    vmem = pltpu.VMEM
    out = pl.pallas_call(
        _kernel,
        out_shape=jax.ShapeDtypeStruct((B, 2 * DM), BF16),
        in_specs=[hbm] * 11,
        out_specs=pl.BlockSpec(memory_space=pltpu.VMEM),
        scratch_shapes=[
            vmem((B, DM), BF16),
            vmem((B, DM), BF16),
            vmem((3, 2, B, W, DH), BF16),
            vmem((4, 128, H * DH), BF16),
            vmem((8, 512, DM), BF16),
            vmem((16, 1024, DM), BF16),
            vmem(w3_shape, BF16),
            vmem(w3_shape, BF16),
            vmem(w3_shape, BF16),
            vmem((8, 512, DM), BF16),
            vmem((128, 2048), BF16),
            vmem((2048, 128), BF16),
            vmem((64, 8192), BF16),
            vmem((128, DH), BF16),
            vmem((B, H, DM), BF16),
            vmem((B, H, 1), F32),
            vmem((B, H, 1), F32),
            vmem((B, H, DM), F32),
            vmem((8, 64, 128), BF16),
            vmem((2, 64, DH), F32),
            vmem((H, 8, DH), F32),
            vmem((H, 8, DH), F32),
            vmem((H, 8, DH), F32),
            pltpu.SemaphoreType.DMA((3,)),
            pltpu.SemaphoreType.DMA((1,)),
            pltpu.SemaphoreType.DMA((11,)),
        ],
        compiler_params=pltpu.CompilerParams(
            vmem_limit_bytes=100 * 1024 * 1024,
            disable_semaphore_checks=True,
            disable_bounds_checks=True,
        ),
        name="fused_decode",
    )(
        A_x.reshape(B, DM),
        A_k_cache.reshape(B * H, SK, DH),
        A_v_cache.reshape(B * H, SK, DH),
        A_wq.reshape(4, 128, H * DH),
        A_wo.reshape(8, 512, DM),
        B_x.reshape(B, DM),
        B_c_kv.reshape(16, 1024, DM),
        B_w_q.reshape(w3_shape),
        B_w_uk.reshape(w3_shape),
        B_w_uv.reshape(w3_shape),
        B_w_o.reshape(8, 512, DM),
    )
    return out.reshape(B, 1, 2 * DM)
```

```python
import jax
import jax.numpy as jnp
from jax import lax
import jax.experimental.pallas as pl
import jax.experimental.pallas.tpu as pltpu

F32 = jnp.float32
BF16 = jnp.bfloat16

B = 4
H = 32
DH = 128
DM = 512
SK = 4096
W = 1024
SCALE = DH ** -0.5

NP = 32
NT = (((1,), (1,)), ((), ()))


def _iota(shape, d):
    return lax.broadcasted_iota(jnp.int32, shape, d)


def _dot(a, b):
    return jnp.dot(a, b, preferred_element_type=F32)


def _dot_nt(a, b):
    return lax.dot_general(a, b, NT, preferred_element_type=F32)


def _kernel(
    xa_hbm, k_hbm, v_hbm, wq_hbm, wo_hbm,
    xb_hbm, c_hbm, bq_hbm, buk_hbm, buv_hbm, bo_hbm,
    o_ref,
    xa_v, xb_v, kv_v, wq_v, wo_v, c_v, bq_v, buk_v, buv_v, bo_v,
    e_v, et_v, x2_v, qb_v, qabs_v, m_v, l_v, acc_v, cn_v, ctx_v,
    qa_v, oa_v, ob_v,
    sems, xsem, fsems,
):
    def start(src, dst, sem, prio):
        pltpu.make_async_copy(src, dst, sem).start(priority=prio)

    def wait(dst, sem):
        pltpu.make_async_copy(dst, dst, sem).wait()

    def w3_idx(p0, i, n):
        return (pl.ds(p0, 2), pl.ds(i * 2, n * 2))

    def c_idx(p0, i, n):
        r = i * 16
        return (pl.ds(p0, 2), pl.ds(r if isinstance(r, int) else pl.multiple_of(r, 16), n * 16),
                slice(None))

    def start2(src, dst, idx, sem, prio):
        start(src.at[idx], dst.at[idx], sem, prio)

    def issue_s0(t, j0, j1):
        sem = sems.at[t % 3]
        for j in range(j0, j1):
            i = t * 16 + j // 2
            prio0 = 1 if (t == 0 and j < 16) else 0
            if j % 2 == 0:
                start2(buk_hbm, buk_v, w3_idx(2, i, 1), sem, prio0)
                start2(bq_hbm, bq_v, w3_idx(2, i, 1), sem, 1)
            else:
                start2(bq_hbm, bq_v, w3_idx(0, i, 1), sem, prio0)
                start2(c_hbm, c_v, c_idx(0, i, 1), sem, 1)

    def wait_s0(t):
        sem = sems.at[t % 3]
        wait(buk_v.at[w3_idx(2, t * 16, 16)], sem)
        wait(bq_v.at[:, pl.ds(t * 32, 32)], sem)
        wait(c_v.at[c_idx(0, t * 16, 16)], sem)

    def issue_s1(t, j0, j1):
        sem = sems.at[(4 + t) % 3]
        for j in range(j0, j1):
            i = t * 16 + j // 2
            if j % 2 == 0:
                start2(buv_hbm, buv_v, w3_idx(2, i, 1), sem, 0)
            else:
                start2(buk_hbm, buk_v, w3_idx(0, i, 1), sem, 0)
            idx = (slice(None), pl.ds((t * 4 + j // 8) * 8, 8), pl.ds((j % 8) * 512, 512))
            start2(wq_hbm, wq_v, idx, sem, 1)

    def wait_s1(t):
        sem = sems.at[(4 + t) % 3]
        wait(buv_v.at[w3_idx(2, t * 16, 16)], sem)
        wait(buk_v.at[w3_idx(0, t * 16, 16)], sem)
        wait(wq_v.at[:, pl.ds(t * 32, 32), :], sem)

    def issue_c(i, lo, j0, j1):
        sem = sems.at[(8 + i) % 3]
        t = i % 4
        for j in range(j0, j1):
            rows8 = pl.ds(pl.multiple_of(t * 256 + j * 8, 8), 8)
            start2(c_hbm, c_v, (pl.ds(2 if lo else 10, 4), rows8, slice(None)), sem, 0)
            if lo:
                start2(c_hbm, c_v, (pl.ds(6, 4), rows8, slice(None)), sem, 1)
            elif j % 2 == 0:
                start2(c_hbm, c_v, c_idx(14, t * 16 + j // 2, 1), sem, 1)
            else:
                start2(buv_hbm, buv_v, w3_idx(0, t * 16 + j // 2, 1), sem, 1)

    def c_parts(i):
        ph = (i // 4) * 8
        return ((2 + ph, 2), (4 + ph, 4), ((8 + ph) % 16, 2))

    def wait_c(i):
        sem = sems.at[(8 + i) % 3]
        rows = pl.ds(pl.multiple_of((i % 4) * 256, 256), 256)
        wait(c_v.at[pl.ds(2 + (i // 4) * 8, 6), rows, :], sem)
        pl.when(i < 4)(lambda: wait(c_v.at[pl.ds(8, 2), rows, :], sem))
        pl.when(i >= 4)(lambda: wait(buv_v.at[w3_idx(0, (i % 4) * 16, 16)], sem))

    def issue_kv(g, j0, j1):
        slot = (16 + g) % 3
        sem = sems.at[slot]
        for j in range(j0, j1):
            for u, src in enumerate((k_hbm, v_hbm)):
                if isinstance(g, int) and g == 0:
                    hh, r = j % 2, (j // 2) * 64
                    start(src.at[pl.ds(126 if hh == 0 else 0, 2), pl.ds(SK - W + r, 64), :],
                          kv_v.at[slot, u, pl.ds(hh * 2, 2), pl.ds(r, 64), :], sem, u)
                else:
                    start(src.at[pl.ds(g * 4 - 2, 4), pl.ds(SK - W + j * 32, 32), :],
                          kv_v.at[slot, u, :, pl.ds(j * 32, 32), :], sem, u)

    def wait_kv(g):
        slot = (16 + g) % 3
        wait(kv_v.at[slot], sems.at[slot])

    def issue_o(t):
        for j in range(NP):
            idx = (pl.ds((j % 2) * 4, 4), pl.ds(pl.multiple_of(t * 128 + (j // 2) * 8, 8), 8), slice(None))
            start(wo_hbm.at[idx], wo_v.at[idx], fsems.at[2 * t], 0)
            start(bo_hbm.at[idx], bo_v.at[idx], fsems.at[2 * t + 1], 1)

    TAIL = ((0, 4), (4, 2), (6, 1), (7, 1))

    def issue_o_last():
        lo = []
        for n, (p0, k) in enumerate(TAIL):
            rows = 32 // k
            lo += [(n, (pl.ds(p0, k), pl.ds(384 + r, rows), slice(None))) for r in range(0, 128, rows)]
        for j in range(NP):
            idx = (pl.ds((j % 2) * 4, 4), pl.ds(384 + (j // 2) * 8, 8), slice(None))
            start(wo_hbm.at[idx], wo_v.at[idx], fsems.at[6], 0)
            n, idx = lo[j]
            start(bo_hbm.at[idx], bo_v.at[idx], fsems.at[7 + n], 1)

    def diag_mask():
        return (_iota((64, 2048), 1) & 15) == (_iota((64, 2048), 0) & 15)

    def w3(ref, k, hf):
        return ref[k, :, hf].reshape(2048, DH)

    def build_consts():
        e_v[...] = jnp.where(_iota((128, 2048), 0) == (_iota((128, 2048), 1) >> 4), 1.0, 0.0).astype(BF16)
        et_v[...] = jnp.where(_iota((2048, 128), 1) == (_iota((2048, 128), 0) >> 4), 1.0, 0.0).astype(BF16)
        m_v[...] = jnp.full(m_v.shape, -jnp.inf, F32)
        l_v[...] = jnp.zeros(l_v.shape, F32)
        acc_v[...] = jnp.zeros(acc_v.shape, F32)
        oa_v[...] = jnp.zeros(oa_v.shape, F32)

    def build_x2():
        x = xb_v[...].astype(F32)
        xrep = jnp.concatenate(
            [jnp.broadcast_to(x[b:b + 1, :], (16, DM)) for b in range(B)], axis=0).astype(BF16)
        for k in range(4):
            xe = _dot(xrep[:, k * 128:(k + 1) * 128], e_v[...])
            x2_v[:, k * 2048:(k + 1) * 2048] = jnp.where(diag_mask(), xe, 0.0).astype(BF16)

    def qb_half(hf):
        acc = None
        for k in range(4):
            r = _dot(x2_v[:, k * 2048:(k + 1) * 2048], w3(bq_v, k, hf))
            acc = r if acc is None else acc + r
        qb_v[hf * 64:(hf + 1) * 64, :] = acc.astype(BF16)

    def qabs_piece(hf, k):
        r = _dot_nt(qb_v[hf * 64:(hf + 1) * 64, :], w3(buk_v, k, hf))
        r = jnp.where(diag_mask(), r, 0.0).astype(BF16)
        z = _dot(r, et_v[...]).astype(BF16)
        for b in range(B):
            qabs_v[b, hf * 16:(hf + 1) * 16, k * 128:(k + 1) * 128] = z[b * 16:(b + 1) * 16, :]

    def qa_proj():
        x = xa_v[...].astype(F32)
        x8 = jnp.concatenate([x, x], axis=0).astype(BF16)
        acc = None
        for k in range(4):
            r = _dot(x8[:, k * 128:(k + 1) * 128], wq_v[k])
            acc = r if acc is None else acc + r
        for h in range(H):
            qa_v[h] = acc[:, h * DH:(h + 1) * DH]

    def b_attn(i, part):
        p0, n = c_parts(i)[part]
        b = p0 // 4
        r0 = pl.multiple_of((i % 4) * 256, 256)
        c = c_v[pl.ds(p0, n), pl.ds(r0, 256), :].reshape(n * 256, DM)
        s = _dot_nt(qabs_v[b], c) * SCALE
        m_old = m_v[b]
        m_new = jnp.maximum(m_old, jnp.max(s, axis=1, keepdims=True))
        alpha = jnp.exp(m_old - m_new)
        p = jnp.exp(s - m_new)
        l_v[b] = alpha * l_v[b] + jnp.sum(p, axis=1, keepdims=True)
        acc_v[b] = alpha * acc_v[b] + _dot(p.astype(BF16), c)
        m_v[b] = m_new

    def b_norm():
        for b in range(B):
            cn = (acc_v[b] / l_v[b]).astype(BF16)
            for hf in range(2):
                for k in range(4):
                    cn_v[hf * 4 + k, b * 16:(b + 1) * 16, :] = (
                        cn[hf * 16:(hf + 1) * 16, k * 128:(k + 1) * 128])
        ctx_v[...] = jnp.zeros(ctx_v.shape, F32)

    def ctx_piece(i):
        xe = _dot(cn_v[i], e_v[...])
        xe = jnp.where(diag_mask(), xe, 0.0).astype(BF16)
        ctx_v[i // 4] += _dot(xe, w3(buv_v, i % 4, i // 4))

    def ob_build():
        ro = _iota((256, 128), 0)
        ri = _iota((256, 128), 1)
        src = ((ro >> 7) << 6) + ((ro & 7) << 4) + ((ro >> 3) & 15)
        perm = jnp.where(((ro & 7) < 4) & (ri == src), 1.0, 0.0).astype(BF16)
        ctx = ctx_v[...].reshape(128, DH).astype(BF16)
        ob_v[...] = _dot(perm, ctx).reshape(H, 8, DH)

    def a_group(g):
        slot = (16 + g) % 3
        for j in range(4):
            f = (g * 4 + (126 + j)) & 127
            h = f & 31
            s = _dot_nt(qa_v[h].astype(BF16), kv_v[slot, 0, j]) * SCALE
            p = jnp.exp(s - jnp.max(s, axis=1, keepdims=True))
            l = jnp.sum(p, axis=1, keepdims=True)
            o = _dot(p.astype(BF16), kv_v[slot, 1, j]) / l
            oa_v[h] = jnp.where(_iota((8, DH), 0) == (f >> 5), o, oa_v[h])

    def o_proj(acc, o_v, w_v, sem, t, p0, n):
        wait(w_v.at[pl.ds(p0, n), pl.ds(t * 128, 128), :], sem)
        for p in range(p0, p0 + n):
            acc += _dot(o_v[p * 4 + t].astype(BF16), w_v[p, t * 128:(t + 1) * 128, :])
        return acc

    issue_s0(0, 0, 2)
    start(xa_hbm, xa_v, xsem.at[0], 0)
    start(xb_hbm, xb_v, xsem.at[0], 0)
    issue_s0(0, 2, NP)
    issue_s0(1, 0, NP)

    issue_s0(2, 0, NP)
    wait_s0(0)
    wait(xa_v, xsem.at[0])
    wait(xb_v, xsem.at[0])
    build_consts()

    issue_s0(3, 0, NP)
    wait_s0(1)
    build_x2()

    issue_s1(0, 0, NP)
    wait_s0(2)

    issue_s1(1, 0, 16)
    wait_s0(3)
    qb_half(0)
    issue_s1(1, 16, NP)
    qb_half(1)

    for hf in range(2):
        issue_s1(2 + hf, 0, NP)
        wait_s1(hf)
        qabs_piece(hf, 2)
        qabs_piece(hf, 3)

    issue_c(0, True, 0, NP)
    wait_s1(2)

    issue_c(1, True, 0, 16)
    wait_s1(3)
    qabs_piece(0, 0)
    qabs_piece(0, 1)
    issue_c(1, True, 16, 24)
    qabs_piece(1, 0)
    qabs_piece(1, 1)
    issue_c(1, True, 24, NP)
    qa_proj()

    def b_body(i, carry):
        for u in range(2):
            j0, j1 = u * 16, (u + 1) * 16
            pl.when(i < 2)(lambda: issue_c(i + 2, True, j0, j1))
            pl.when((i >= 2) & (i < 6))(lambda: issue_c(i + 2, False, j0, j1))
            pl.when(i == 6)(lambda: issue_kv(0, j0, j1))
            pl.when(i == 7)(lambda: issue_kv(1, j0, j1))
            if u == 0:
                wait_c(i)
                b_attn(i, 0)
                b_attn(i, 2)
            else:
                b_attn(i, 1)
        return carry

    lax.fori_loop(0, 8, b_body, 0)
    b_norm()

    def a_body(g, carry):
        pl.when(g < H - 2)(lambda: issue_kv(g + 2, 0, NP))
        pl.when(g >= H - 2)(lambda: issue_o(g - (H - 2)))
        wait_kv(g)
        a_group(g)
        pl.when(g < 8)(lambda: ctx_piece(g))
        return carry

    lax.fori_loop(0, H, a_body, 0)

    acc_a = jnp.zeros((8, DM), F32)
    acc_b = jnp.zeros((8, DM), F32)
    issue_o(2)
    ob_build()
    acc_a = o_proj(acc_a, oa_v, wo_v, fsems.at[0], 0, 0, 8)
    acc_b = o_proj(acc_b, ob_v, bo_v, fsems.at[1], 0, 0, 8)
    issue_o_last()
    for t in (1, 2):
        acc_a = o_proj(acc_a, oa_v, wo_v, fsems.at[2 * t], t, 0, 8)
        acc_b = o_proj(acc_b, ob_v, bo_v, fsems.at[2 * t + 1], t, 0, 8)
    acc_a = o_proj(acc_a, oa_v, wo_v, fsems.at[6], 3, 0, 8)
    o_ref[:, 0:DM] = acc_a[0:B, :].astype(o_ref.dtype)
    for n, (p0, k) in enumerate(TAIL):
        acc_b = o_proj(acc_b, ob_v, bo_v, fsems.at[7 + n], 3, p0, k)
    o_ref[:, DM:2 * DM] = acc_b[0:B, :].astype(o_ref.dtype)


@jax.jit
def pallas_concat_heads__sliding_block_cached__compressed_kv_cla__decode_kernel(
    A_x: jax.Array,
    A_k_cache: jax.Array,
    A_v_cache: jax.Array,
    A_wq: jax.Array,
    A_wo: jax.Array,
    B_x: jax.Array,
    B_c_kv: jax.Array,
    B_w_q: jax.Array,
    B_w_uk: jax.Array,
    B_w_uv: jax.Array,
    B_w_o: jax.Array,
):
    w3_shape = (4, 128, 2, 16, DH)
    hbm = pl.BlockSpec(memory_space=pl.ANY)
    vmem = pltpu.VMEM
    out = pl.pallas_call(
        _kernel,
        out_shape=jax.ShapeDtypeStruct((B, 2 * DM), BF16),
        in_specs=[hbm] * 11,
        out_specs=pl.BlockSpec(memory_space=pltpu.VMEM),
        scratch_shapes=[
            vmem((B, DM), BF16),
            vmem((B, DM), BF16),
            vmem((3, 2, B, W, DH), BF16),
            vmem((4, 128, H * DH), BF16),
            vmem((8, 512, DM), BF16),
            vmem((16, 1024, DM), BF16),
            vmem(w3_shape, BF16),
            vmem(w3_shape, BF16),
            vmem(w3_shape, BF16),
            vmem((8, 512, DM), BF16),
            vmem((128, 2048), BF16),
            vmem((2048, 128), BF16),
            vmem((64, 8192), BF16),
            vmem((128, DH), BF16),
            vmem((B, H, DM), BF16),
            vmem((B, H, 1), F32),
            vmem((B, H, 1), F32),
            vmem((B, H, DM), F32),
            vmem((8, 64, 128), BF16),
            vmem((2, 64, DH), F32),
            vmem((H, 8, DH), F32),
            vmem((H, 8, DH), F32),
            vmem((H, 8, DH), F32),
            pltpu.SemaphoreType.DMA((3,)),
            pltpu.SemaphoreType.DMA((1,)),
            pltpu.SemaphoreType.DMA((11,)),
        ],
        compiler_params=pltpu.CompilerParams(
            vmem_limit_bytes=100 * 1024 * 1024,
            disable_semaphore_checks=True,
            disable_bounds_checks=True,
        ),
        name="fused_decode",
    )(
        A_x.reshape(B, DM),
        A_k_cache.reshape(B * H, SK, DH),
        A_v_cache.reshape(B * H, SK, DH),
        A_wq.reshape(4, 128, H * DH),
        A_wo.reshape(8, 512, DM),
        B_x.reshape(B, DM),
        B_c_kv.reshape(16, 1024, DM),
        B_w_q.reshape(w3_shape),
        B_w_uk.reshape(w3_shape),
        B_w_uv.reshape(w3_shape),
        B_w_o.reshape(8, 512, DM),
    )
    return out.reshape(B, 1, 2 * DM)
```

```python
import jax
import jax.numpy as jnp
from jax import lax
import jax.experimental.pallas as pl
import jax.experimental.pallas.tpu as pltpu

F32 = jnp.float32
BF16 = jnp.bfloat16

B = 4
H = 32
DH = 128
DM = 512
SK = 4096
W = 1024
SCALE = DH ** -0.5

NP = 32
NT = (((1,), (1,)), ((), ()))


def _iota(shape, d):
    return lax.broadcasted_iota(jnp.int32, shape, d)


def _dot(a, b):
    return jnp.dot(a, b, preferred_element_type=F32)


def _dot_nt(a, b):
    return lax.dot_general(a, b, NT, preferred_element_type=F32)


def _kernel(
    xa_hbm, k_hbm, v_hbm, wq_hbm, wo_hbm,
    xb_hbm, c_hbm, bq_hbm, buk_hbm, buv_hbm, bo_hbm,
    o_ref,
    xa_v, xb_v, kv_v, wq_v, wo_v, c_v, bq_v, buk_v, buv_v, bo_v,
    e_v, et_v, x2_v, qb_v, qabs_v, m_v, l_v, acc_v, cn_v, ctx_v,
    qa_v, oa_v, ob_v,
    sems, xsem, fsems,
):
    def start(src, dst, sem, prio):
        pltpu.make_async_copy(src, dst, sem).start(priority=prio)

    def wait(dst, sem):
        pltpu.make_async_copy(dst, dst, sem).wait()

    def w3_idx(p0, i, n):
        return (pl.ds(p0, 2), pl.ds(i * 2, n * 2))

    def c_idx(p0, i, n):
        r = i * 16
        return (pl.ds(p0, 2), pl.ds(r if isinstance(r, int) else pl.multiple_of(r, 16), n * 16),
                slice(None))

    def start2(src, dst, idx, sem, prio):
        start(src.at[idx], dst.at[idx], sem, prio)

    def issue_s0(t, j0, j1):
        sem = sems.at[t % 3]
        for j in range(j0, j1):
            i = t * 16 + j // 2
            prio0 = 1 if (t == 0 and j < 16) else 0
            if j % 2 == 0:
                start2(buk_hbm, buk_v, w3_idx(2, i, 1), sem, prio0)
                start2(bq_hbm, bq_v, w3_idx(2, i, 1), sem, 1)
            else:
                start2(bq_hbm, bq_v, w3_idx(0, i, 1), sem, prio0)
                start2(c_hbm, c_v, c_idx(0, i, 1), sem, 1)

    def wait_s0(t):
        sem = sems.at[t % 3]
        wait(buk_v.at[w3_idx(2, t * 16, 16)], sem)
        wait(bq_v.at[:, pl.ds(t * 32, 32)], sem)
        wait(c_v.at[c_idx(0, t * 16, 16)], sem)

    def issue_s1(t, j0, j1):
        sem = sems.at[(4 + t) % 3]
        for j in range(j0, j1):
            i = t * 16 + j // 2
            if j % 2 == 0:
                start2(buv_hbm, buv_v, w3_idx(2, i, 1), sem, 0)
            else:
                start2(buk_hbm, buk_v, w3_idx(0, i, 1), sem, 0)
            idx = (slice(None), pl.ds((t * 4 + j // 8) * 8, 8), pl.ds((j % 8) * 512, 512))
            start2(wq_hbm, wq_v, idx, sem, 1)

    def wait_s1(t):
        sem = sems.at[(4 + t) % 3]
        wait(buv_v.at[w3_idx(2, t * 16, 16)], sem)
        wait(buk_v.at[w3_idx(0, t * 16, 16)], sem)
        wait(wq_v.at[:, pl.ds(t * 32, 32), :], sem)

    def issue_c(i, lo, j0, j1):
        sem = sems.at[(8 + i) % 3]
        t = i % 4
        for j in range(j0, j1):
            rows8 = pl.ds(pl.multiple_of(t * 256 + j * 8, 8), 8)
            start2(c_hbm, c_v, (pl.ds(2 if lo else 10, 4), rows8, slice(None)), sem, 0)
            if lo:
                start2(c_hbm, c_v, (pl.ds(6, 4), rows8, slice(None)), sem, 1)
            elif j % 2 == 0:
                start2(c_hbm, c_v, c_idx(14, t * 16 + j // 2, 1), sem, 1)
            else:
                start2(buv_hbm, buv_v, w3_idx(0, t * 16 + j // 2, 1), sem, 1)

    def c_parts(i):
        ph = (i // 4) * 8
        return ((2 + ph, 2), (4 + ph, 4), ((8 + ph) % 16, 2))

    def wait_c(i):
        sem = sems.at[(8 + i) % 3]
        rows = pl.ds(pl.multiple_of((i % 4) * 256, 256), 256)
        wait(c_v.at[pl.ds(2 + (i // 4) * 8, 6), rows, :], sem)
        pl.when(i < 4)(lambda: wait(c_v.at[pl.ds(8, 2), rows, :], sem))
        pl.when(i >= 4)(lambda: wait(buv_v.at[w3_idx(0, (i % 4) * 16, 16)], sem))

    def issue_kv(g, j0, j1):
        slot = (16 + g) % 3
        sem = sems.at[slot]
        for j in range(j0, j1):
            for u, src in enumerate((k_hbm, v_hbm)):
                if isinstance(g, int) and g == 0:
                    hh, r = j % 2, (j // 2) * 64
                    start(src.at[pl.ds(126 if hh == 0 else 0, 2), pl.ds(SK - W + r, 64), :],
                          kv_v.at[slot, u, pl.ds(hh * 2, 2), pl.ds(r, 64), :], sem, u)
                else:
                    start(src.at[pl.ds(g * 4 - 2, 4), pl.ds(SK - W + j * 32, 32), :],
                          kv_v.at[slot, u, :, pl.ds(j * 32, 32), :], sem, u)

    def wait_kv(g):
        slot = (16 + g) % 3
        wait(kv_v.at[slot], sems.at[slot])

    def o_idx(t, j):
        r = (t ^ ((j % 2) * 2)) * 256 + (j // 2) * 16
        return c_idx((j % 2) * 2, r // 16, 1)

    def o_heads(t):
        return [(p, (t ^ (p & 2)) * 256 + hb * 128) for hb in range(2) for p in range(4)]

    def issue_o(t):
        for j in range(NP):
            start2(wo_hbm, wo_v, o_idx(t, j), fsems.at[2 * t], 0)
            start2(bo_hbm, bo_v, o_idx(t, j), fsems.at[2 * t + 1], 1)

    TAIL = ((0, 4), (4, 2), (6, 1), (7, 1))

    def issue_o_last():
        heads = o_heads(3)
        lo = [(0, o_idx(3, j)) for j in range(16)]
        lo += [(1, c_idx(0, heads[4][1] // 16 + i, 1)) for i in range(8)]
        for n in (2, 3):
            p, r0 = heads[4 + n]
            lo += [(n, (p, pl.ds(r0 + r, 32), slice(None))) for r in range(0, 128, 32)]
        for j in range(NP):
            start2(wo_hbm, wo_v, o_idx(3, j), fsems.at[6], 0)
            start2(bo_hbm, bo_v, lo[j][1], fsems.at[7 + lo[j][0]], 1)

    def diag_mask():
        return (_iota((64, 2048), 1) & 15) == (_iota((64, 2048), 0) & 15)

    def w3(ref, k, hf):
        return ref[k, :, hf].reshape(2048, DH)

    def build_consts():
        e_v[...] = jnp.where(_iota((128, 2048), 0) == (_iota((128, 2048), 1) >> 4), 1.0, 0.0).astype(BF16)
        et_v[...] = jnp.where(_iota((2048, 128), 1) == (_iota((2048, 128), 0) >> 4), 1.0, 0.0).astype(BF16)
        m_v[...] = jnp.full(m_v.shape, -jnp.inf, F32)
        l_v[...] = jnp.zeros(l_v.shape, F32)
        acc_v[...] = jnp.zeros(acc_v.shape, F32)
        oa_v[...] = jnp.zeros(oa_v.shape, F32)

    def build_x2():
        x = xb_v[...].astype(F32)
        xrep = jnp.concatenate(
            [jnp.broadcast_to(x[b:b + 1, :], (16, DM)) for b in range(B)], axis=0).astype(BF16)
        for k in range(4):
            xe = _dot(xrep[:, k * 128:(k + 1) * 128], e_v[...])
            x2_v[:, k * 2048:(k + 1) * 2048] = jnp.where(diag_mask(), xe, 0.0).astype(BF16)

    def qb_half(hf):
        acc = None
        for k in range(4):
            r = _dot(x2_v[:, k * 2048:(k + 1) * 2048], w3(bq_v, k, hf))
            acc = r if acc is None else acc + r
        qb_v[hf * 64:(hf + 1) * 64, :] = acc.astype(BF16)

    def qabs_piece(hf, k):
        r = _dot_nt(qb_v[hf * 64:(hf + 1) * 64, :], w3(buk_v, k, hf))
        r = jnp.where(diag_mask(), r, 0.0).astype(BF16)
        z = _dot(r, et_v[...]).astype(BF16)
        for b in range(B):
            qabs_v[b, hf * 16:(hf + 1) * 16, k * 128:(k + 1) * 128] = z[b * 16:(b + 1) * 16, :]

    def qa_proj():
        x = xa_v[...].astype(F32)
        x8 = jnp.concatenate([x, x], axis=0).astype(BF16)
        acc = None
        for k in range(4):
            r = _dot(x8[:, k * 128:(k + 1) * 128], wq_v[k])
            acc = r if acc is None else acc + r
        for h in range(H):
            qa_v[h] = acc[:, h * DH:(h + 1) * DH]

    def b_attn(i, part):
        p0, n = c_parts(i)[part]
        b = p0 // 4
        r0 = pl.multiple_of((i % 4) * 256, 256)
        c = c_v[pl.ds(p0, n), pl.ds(r0, 256), :].reshape(n * 256, DM)
        s = _dot_nt(qabs_v[b], c) * SCALE
        m_old = m_v[b]
        m_new = jnp.maximum(m_old, jnp.max(s, axis=1, keepdims=True))
        alpha = jnp.exp(m_old - m_new)
        p = jnp.exp(s - m_new)
        l_v[b] = alpha * l_v[b] + jnp.sum(p, axis=1, keepdims=True)
        acc_v[b] = alpha * acc_v[b] + _dot(p.astype(BF16), c)
        m_v[b] = m_new

    def b_norm():
        for b in range(B):
            cn = (acc_v[b] / l_v[b]).astype(BF16)
            for hf in range(2):
                for k in range(4):
                    cn_v[hf * 4 + k, b * 16:(b + 1) * 16, :] = (
                        cn[hf * 16:(hf + 1) * 16, k * 128:(k + 1) * 128])
        ctx_v[...] = jnp.zeros(ctx_v.shape, F32)

    def ctx_piece(i):
        xe = _dot(cn_v[i], e_v[...])
        xe = jnp.where(diag_mask(), xe, 0.0).astype(BF16)
        ctx_v[i // 4] += _dot(xe, w3(buv_v, i % 4, i // 4))

    def ob_build():
        ro = _iota((256, 128), 0)
        ri = _iota((256, 128), 1)
        src = ((ro >> 7) << 6) + ((ro & 7) << 4) + ((ro >> 3) & 15)
        perm = jnp.where(((ro & 7) < 4) & (ri == src), 1.0, 0.0).astype(BF16)
        ctx = ctx_v[...].reshape(128, DH).astype(BF16)
        ob_v[...] = _dot(perm, ctx).reshape(H, 8, DH)

    def a_group(g):
        slot = (16 + g) % 3
        for j in range(4):
            f = (g * 4 + (126 + j)) & 127
            h = f & 31
            s = _dot_nt(qa_v[h].astype(BF16), kv_v[slot, 0, j]) * SCALE
            p = jnp.exp(s - jnp.max(s, axis=1, keepdims=True))
            l = jnp.sum(p, axis=1, keepdims=True)
            o = _dot(p.astype(BF16), kv_v[slot, 1, j]) / l
            oa_v[h] = jnp.where(_iota((8, DH), 0) == (f >> 5), o, oa_v[h])

    def o_proj(acc, o_v, w_v, sem, t, h0, n):
        heads = o_heads(t)[h0:h0 + n]
        for p, r0 in heads:
            wait(w_v.at[p, pl.ds(r0, 128), :], sem)
        for p, r0 in heads:
            acc += _dot(o_v[p * 8 + r0 // 128].astype(BF16), w_v[p, r0:r0 + 128, :])
        return acc

    issue_s0(0, 0, 2)
    start(xa_hbm, xa_v, xsem.at[0], 0)
    start(xb_hbm, xb_v, xsem.at[0], 0)
    issue_s0(0, 2, NP)
    issue_s0(1, 0, NP)

    issue_s0(2, 0, NP)
    wait_s0(0)
    wait(xa_v, xsem.at[0])
    wait(xb_v, xsem.at[0])
    build_consts()

    issue_s0(3, 0, NP)
    wait_s0(1)
    build_x2()

    issue_s1(0, 0, NP)
    wait_s0(2)

    issue_s1(1, 0, 16)
    wait_s0(3)
    qb_half(0)
    issue_s1(1, 16, NP)
    qb_half(1)

    for hf in range(2):
        issue_s1(2 + hf, 0, NP)
        wait_s1(hf)
        qabs_piece(hf, 2)
        qabs_piece(hf, 3)

    issue_c(0, True, 0, NP)
    wait_s1(2)

    issue_c(1, True, 0, 16)
    wait_s1(3)
    qabs_piece(0, 0)
    qabs_piece(0, 1)
    issue_c(1, True, 16, 24)
    qabs_piece(1, 0)
    qabs_piece(1, 1)
    issue_c(1, True, 24, NP)
    qa_proj()

    def b_body(i, carry):
        for u in range(2):
            j0, j1 = u * 16, (u + 1) * 16
            pl.when(i < 2)(lambda: issue_c(i + 2, True, j0, j1))
            pl.when((i >= 2) & (i < 6))(lambda: issue_c(i + 2, False, j0, j1))
            pl.when(i == 6)(lambda: issue_kv(0, j0, j1))
            pl.when(i == 7)(lambda: issue_kv(1, j0, j1))
            if u == 0:
                wait_c(i)
                b_attn(i, 0)
                b_attn(i, 2)
            else:
                b_attn(i, 1)
        return carry

    lax.fori_loop(0, 8, b_body, 0)
    b_norm()

    def a_body(g, carry):
        pl.when(g < H - 2)(lambda: issue_kv(g + 2, 0, NP))
        pl.when(g == H - 2)(lambda: issue_o(0))
        pl.when(g == H - 1)(lambda: issue_o(1))
        wait_kv(g)
        a_group(g)
        pl.when(g < 8)(lambda: ctx_piece(g))
        return carry

    lax.fori_loop(0, H, a_body, 0)

    acc_a = jnp.zeros((8, DM), F32)
    acc_b = jnp.zeros((8, DM), F32)
    issue_o(2)
    ob_build()
    acc_a = o_proj(acc_a, oa_v, wo_v, fsems.at[0], 0, 0, 8)
    acc_b = o_proj(acc_b, ob_v, bo_v, fsems.at[1], 0, 0, 8)
    issue_o_last()
    for t in (1, 2):
        acc_a = o_proj(acc_a, oa_v, wo_v, fsems.at[2 * t], t, 0, 8)
        acc_b = o_proj(acc_b, ob_v, bo_v, fsems.at[2 * t + 1], t, 0, 8)
    acc_a = o_proj(acc_a, oa_v, wo_v, fsems.at[6], 3, 0, 8)
    o_ref[:, 0:DM] = acc_a[0:B, :].astype(o_ref.dtype)
    for n, (h0, k) in enumerate(TAIL):
        acc_b = o_proj(acc_b, ob_v, bo_v, fsems.at[7 + n], 3, h0, k)
    o_ref[:, DM:2 * DM] = acc_b[0:B, :].astype(o_ref.dtype)


@jax.jit
def pallas_concat_heads__sliding_block_cached__compressed_kv_cla__decode_kernel(
    A_x: jax.Array,
    A_k_cache: jax.Array,
    A_v_cache: jax.Array,
    A_wq: jax.Array,
    A_wo: jax.Array,
    B_x: jax.Array,
    B_c_kv: jax.Array,
    B_w_q: jax.Array,
    B_w_uk: jax.Array,
    B_w_uv: jax.Array,
    B_w_o: jax.Array,
):
    w3_shape = (4, 128, 2, 16, DH)
    hbm = pl.BlockSpec(memory_space=pl.ANY)
    vmem = pltpu.VMEM
    out = pl.pallas_call(
        _kernel,
        out_shape=jax.ShapeDtypeStruct((B, 2 * DM), BF16),
        in_specs=[hbm] * 11,
        out_specs=pl.BlockSpec(memory_space=pltpu.VMEM),
        scratch_shapes=[
            vmem((B, DM), BF16),
            vmem((B, DM), BF16),
            vmem((3, 2, B, W, DH), BF16),
            vmem((4, 128, H * DH), BF16),
            vmem((4, 1024, DM), BF16),
            vmem((16, 1024, DM), BF16),
            vmem(w3_shape, BF16),
            vmem(w3_shape, BF16),
            vmem(w3_shape, BF16),
            vmem((4, 1024, DM), BF16),
            vmem((128, 2048), BF16),
            vmem((2048, 128), BF16),
            vmem((64, 8192), BF16),
            vmem((128, DH), BF16),
            vmem((B, H, DM), BF16),
            vmem((B, H, 1), F32),
            vmem((B, H, 1), F32),
            vmem((B, H, DM), F32),
            vmem((8, 64, 128), BF16),
            vmem((2, 64, DH), F32),
            vmem((H, 8, DH), F32),
            vmem((H, 8, DH), F32),
            vmem((H, 8, DH), F32),
            pltpu.SemaphoreType.DMA((3,)),
            pltpu.SemaphoreType.DMA((1,)),
            pltpu.SemaphoreType.DMA((11,)),
        ],
        compiler_params=pltpu.CompilerParams(
            vmem_limit_bytes=100 * 1024 * 1024,
            disable_semaphore_checks=True,
            disable_bounds_checks=True,
        ),
        name="fused_decode",
    )(
        A_x.reshape(B, DM),
        A_k_cache.reshape(B * H, SK, DH),
        A_v_cache.reshape(B * H, SK, DH),
        A_wq.reshape(4, 128, H * DH),
        A_wo.reshape(4, 1024, DM),
        B_x.reshape(B, DM),
        B_c_kv.reshape(16, 1024, DM),
        B_w_q.reshape(w3_shape),
        B_w_uk.reshape(w3_shape),
        B_w_uv.reshape(w3_shape),
        B_w_o.reshape(4, 1024, DM),
    )
    return out.reshape(B, 1, 2 * DM)
```

```python
import functools

import jax
import jax.numpy as jnp
from jax import lax
import jax.experimental.pallas as pl
import jax.experimental.pallas.tpu as pltpu

F32 = jnp.float32
BF16 = jnp.bfloat16

B = 4
H = 32
DH = 128
DM = 512
SK = 4096
W = 1024
SCALE = DH ** -0.5

NP = 32
NT = (((1,), (1,)), ((), ()))


def _iota(shape, d):
    return lax.broadcasted_iota(jnp.int32, shape, d)


def _dot(a, b):
    return jnp.dot(a, b, preferred_element_type=F32)


def _dot_nt(a, b):
    return lax.dot_general(a, b, NT, preferred_element_type=F32)


def _body(
    xa_hbm, k_hbm, v_hbm, wq_hbm, wo_hbm,
    xb_hbm, c_hbm, bq_hbm, buk_hbm, buv_hbm, bo_hbm,
    o_ref,
    xa_v, xb_v, kv_v, wq_v, wo_v, c_v, bq_v, buk_v, buv_v, bo_v,
    e_v, et_v, x2_v, qb_v, qabs_v, m_v, l_v, acc_v, cn_v, ctx_v,
    qa_v, oa_v, ob_v,
    sems, xsem, fsems,
):
    def start(src, dst, sem, prio):
        pltpu.make_async_copy(src, dst, sem).start(priority=prio)

    def wait(dst, sem):
        pltpu.make_async_copy(dst, dst, sem).wait()

    def w3_idx(p0, i, n):
        return (pl.ds(p0, 2), pl.ds(i * 2, n * 2))

    def c_idx(p0, i, n):
        return (pl.ds(p0, 2), pl.ds(i * 16, n * 16), slice(None))

    def start2(src, dst, idx, sem, prio):
        start(src.at[idx], dst.at[idx], sem, prio)

    def issue_s0(t, j0, j1):
        sem = sems.at[t % 3]
        for j in range(j0, j1):
            i = t * 16 + j // 2
            prio0 = 1 if (t == 0 and j < 16) else 0
            if j % 2 == 0:
                start2(buk_hbm, buk_v, w3_idx(2, i, 1), sem, prio0)
                start2(bq_hbm, bq_v, w3_idx(2, i, 1), sem, 1)
            else:
                start2(bq_hbm, bq_v, w3_idx(0, i, 1), sem, prio0)
                start2(c_hbm, c_v, c_idx(0, i, 1), sem, 1)

    def wait_s0(t):
        sem = sems.at[t % 3]
        wait(buk_v.at[w3_idx(2, t * 16, 16)], sem)
        wait(bq_v.at[:, pl.ds(t * 32, 32)], sem)
        wait(c_v.at[c_idx(0, t * 16, 16)], sem)

    def issue_s1(t, j0, j1):
        sem = sems.at[(4 + t) % 3]
        for j in range(j0, j1):
            i = t * 16 + j // 2
            if j % 2 == 0:
                start2(buv_hbm, buv_v, w3_idx(2, i, 1), sem, 0)
            else:
                start2(buk_hbm, buk_v, w3_idx(0, i, 1), sem, 0)
            idx = (slice(None), pl.ds((t * 4 + j // 8) * 8, 8), pl.ds((j % 8) * 512, 512))
            start2(wq_hbm, wq_v, idx, sem, 1)

    def wait_s1(t):
        sem = sems.at[(4 + t) % 3]
        wait(buv_v.at[w3_idx(2, t * 16, 16)], sem)
        wait(buk_v.at[w3_idx(0, t * 16, 16)], sem)
        wait(wq_v.at[:, pl.ds(t * 32, 32), :], sem)

    def issue_c(i, j0, j1):
        sem = sems.at[(8 + i) % 3]
        t = i % 4
        for j in range(j0, j1):
            rows8 = pl.ds(t * 256 + j * 8, 8)
            start2(c_hbm, c_v, (pl.ds(2 if i < 4 else 10, 4), rows8, slice(None)), sem, 0)
            if i < 4:
                start2(c_hbm, c_v, (pl.ds(6, 4), rows8, slice(None)), sem, 1)
            elif j % 2 == 0:
                start2(c_hbm, c_v, c_idx(14, t * 16 + j // 2, 1), sem, 1)
            else:
                start2(buv_hbm, buv_v, w3_idx(0, t * 16 + j // 2, 1), sem, 1)

    def c_parts(i):
        ph = (i // 4) * 8
        return ((2 + ph, 2), (4 + ph, 4), ((8 + ph) % 16, 2))

    def wait_c(i):
        sem = sems.at[(8 + i) % 3]
        rows = pl.ds(pl.multiple_of((i % 4) * 256, 256), 256)
        wait(c_v.at[pl.ds(2 + (i // 4) * 8, 6), rows, :], sem)
        pl.when(i < 4)(lambda: wait(c_v.at[pl.ds(8, 2), rows, :], sem))
        pl.when(i >= 4)(lambda: wait(buv_v.at[w3_idx(0, (i % 4) * 16, 16)], sem))

    def issue_kv(g, j0, j1):
        slot = (16 + g) % 3
        sem = sems.at[slot]
        for j in range(j0, j1):
            for u, src in enumerate((k_hbm, v_hbm)):
                if isinstance(g, int) and g == 0:
                    hh, r = j % 2, (j // 2) * 64
                    start(src.at[pl.ds(126 if hh == 0 else 0, 2), pl.ds(SK - W + r, 64), :],
                          kv_v.at[slot, u, pl.ds(hh * 2, 2), pl.ds(r, 64), :], sem, u)
                else:
                    start(src.at[pl.ds(g * 4 - 2, 4), pl.ds(SK - W + j * 32, 32), :],
                          kv_v.at[slot, u, :, pl.ds(j * 32, 32), :], sem, u)

    def wait_kv(g):
        slot = (16 + g) % 3
        wait(kv_v.at[slot], sems.at[slot])

    def o_idx(t, j):
        r = (t ^ ((j % 2) * 2)) * 256 + (j // 2) * 16
        return c_idx((j % 2) * 2, r // 16, 1)

    def o_heads(t):
        return [(p, (t ^ (p & 2)) * 256 + hb * 128) for hb in range(2) for p in range(4)]

    def issue_o(t):
        for j in range(NP):
            start2(wo_hbm, wo_v, o_idx(t, j), fsems.at[2 * t], 0)
            start2(bo_hbm, bo_v, o_idx(t, j), fsems.at[2 * t + 1], 1)

    TAIL = ((0, 4), (4, 2), (6, 1), (7, 1))

    def issue_o_last():
        heads = o_heads(3)
        lo = [(0, o_idx(3, j)) for j in range(16)]
        lo += [(1, c_idx(0, heads[4][1] // 16 + i, 1)) for i in range(8)]
        for n in (2, 3):
            p, r0 = heads[4 + n]
            lo += [(n, (p, pl.ds(r0 + r, 32), slice(None))) for r in range(0, 128, 32)]
        for j in range(NP):
            start2(wo_hbm, wo_v, o_idx(3, j), fsems.at[6], 0)
            start2(bo_hbm, bo_v, lo[j][1], fsems.at[7 + lo[j][0]], 1)

    def diag_mask():
        return (_iota((64, 2048), 1) & 15) == (_iota((64, 2048), 0) & 15)

    def w3(ref, k, hf):
        return ref[k, :, hf].reshape(2048, DH)

    def build_consts():
        e_v[...] = jnp.where(_iota((128, 2048), 0) == (_iota((128, 2048), 1) >> 4), 1.0, 0.0).astype(BF16)
        et_v[...] = jnp.where(_iota((2048, 128), 1) == (_iota((2048, 128), 0) >> 4), 1.0, 0.0).astype(BF16)
        m_v[...] = jnp.full(m_v.shape, -jnp.inf, F32)
        l_v[...] = jnp.zeros(l_v.shape, F32)
        acc_v[...] = jnp.zeros(acc_v.shape, F32)
        oa_v[...] = jnp.zeros(oa_v.shape, F32)

    def build_x2():
        x = xb_v[...].astype(F32)
        xrep = jnp.concatenate(
            [jnp.broadcast_to(x[b:b + 1, :], (16, DM)) for b in range(B)], axis=0).astype(BF16)
        for k in range(4):
            xe = _dot(xrep[:, k * 128:(k + 1) * 128], e_v[...])
            x2_v[:, k * 2048:(k + 1) * 2048] = jnp.where(diag_mask(), xe, 0.0).astype(BF16)

    def qb_half(hf):
        acc = None
        for k in range(4):
            r = _dot(x2_v[:, k * 2048:(k + 1) * 2048], w3(bq_v, k, hf))
            acc = r if acc is None else acc + r
        qb_v[hf * 64:(hf + 1) * 64, :] = acc.astype(BF16)

    def qabs_piece(hf, k):
        r = _dot_nt(qb_v[hf * 64:(hf + 1) * 64, :], w3(buk_v, k, hf))
        r = jnp.where(diag_mask(), r, 0.0).astype(BF16)
        z = _dot(r, et_v[...]).astype(BF16)
        for b in range(B):
            qabs_v[b, hf * 16:(hf + 1) * 16, k * 128:(k + 1) * 128] = z[b * 16:(b + 1) * 16, :]

    def qa_proj():
        x = xa_v[...].astype(F32)
        x8 = jnp.concatenate([x, x], axis=0).astype(BF16)
        acc = None
        for k in range(4):
            r = _dot(x8[:, k * 128:(k + 1) * 128], wq_v[k])
            acc = r if acc is None else acc + r
        for h in range(H):
            qa_v[h] = acc[:, h * DH:(h + 1) * DH]

    def b_attn(i, part):
        p0, n = c_parts(i)[part]
        b = p0 // 4
        r0 = pl.multiple_of((i % 4) * 256, 256)
        c = c_v[pl.ds(p0, n), pl.ds(r0, 256), :].reshape(n * 256, DM)
        s = _dot_nt(qabs_v[b], c) * SCALE
        m_old = m_v[b]
        m_new = jnp.maximum(m_old, jnp.max(s, axis=1, keepdims=True))
        alpha = jnp.exp(m_old - m_new)
        p = jnp.exp(s - m_new)
        l_v[b] = alpha * l_v[b] + jnp.sum(p, axis=1, keepdims=True)
        acc_v[b] = alpha * acc_v[b] + _dot(p.astype(BF16), c)
        m_v[b] = m_new

    def b_norm():
        for b in range(B):
            cn = (acc_v[b] / l_v[b]).astype(BF16)
            for hf in range(2):
                for k in range(4):
                    cn_v[hf * 4 + k, b * 16:(b + 1) * 16, :] = (
                        cn[hf * 16:(hf + 1) * 16, k * 128:(k + 1) * 128])
        ctx_v[...] = jnp.zeros(ctx_v.shape, F32)

    def ctx_piece(i):
        xe = _dot(cn_v[i], e_v[...])
        xe = jnp.where(diag_mask(), xe, 0.0).astype(BF16)
        ctx_v[i // 4] += _dot(xe, w3(buv_v, i % 4, i // 4))

    def ob_build():
        ro = _iota((256, 128), 0)
        ri = _iota((256, 128), 1)
        src = ((ro >> 7) << 6) + ((ro & 7) << 4) + ((ro >> 3) & 15)
        perm = jnp.where(((ro & 7) < 4) & (ri == src), 1.0, 0.0).astype(BF16)
        ctx = ctx_v[...].reshape(128, DH).astype(BF16)
        ob_v[...] = _dot(perm, ctx).reshape(H, 8, DH)

    def a_group(g):
        slot = (16 + g) % 3
        for j in range(4):
            f = (g * 4 + (126 + j)) & 127
            h = f & 31
            s = _dot_nt(qa_v[h].astype(BF16), kv_v[slot, 0, j]) * SCALE
            p = jnp.exp(s - jnp.max(s, axis=1, keepdims=True))
            l = jnp.sum(p, axis=1, keepdims=True)
            o = _dot(p.astype(BF16), kv_v[slot, 1, j]) / l
            oa_v[h] = jnp.where(_iota((8, DH), 0) == (f >> 5), o, oa_v[h])

    def o_proj(acc, o_v, w_v, sem, t, h0, n):
        heads = o_heads(t)[h0:h0 + n]
        for p, r0 in heads:
            wait(w_v.at[p, pl.ds(r0, 128), :], sem)
        for p, r0 in heads:
            acc += _dot(o_v[p * 8 + r0 // 128].astype(BF16), w_v[p, r0:r0 + 128, :])
        return acc

    issue_s0(0, 0, 2)
    start(xa_hbm, xa_v, xsem.at[0], 0)
    start(xb_hbm, xb_v, xsem.at[0], 0)
    issue_s0(0, 2, NP)
    issue_s0(1, 0, NP)

    issue_s0(2, 0, NP)
    wait_s0(0)
    wait(xa_v, xsem.at[0])
    wait(xb_v, xsem.at[0])
    build_consts()

    issue_s0(3, 0, NP)
    wait_s0(1)
    build_x2()

    issue_s1(0, 0, NP)
    wait_s0(2)

    issue_s1(1, 0, 16)
    wait_s0(3)
    qb_half(0)
    issue_s1(1, 16, NP)
    qb_half(1)

    for hf in range(2):
        issue_s1(2 + hf, 0, NP)
        wait_s1(hf)
        qabs_piece(hf, 2)
        qabs_piece(hf, 3)

    issue_c(0, 0, NP)
    wait_s1(2)

    issue_c(1, 0, 16)
    wait_s1(3)
    qabs_piece(0, 0)
    qabs_piece(0, 1)
    issue_c(1, 16, 24)
    qabs_piece(1, 0)
    qabs_piece(1, 1)
    issue_c(1, 24, NP)
    qa_proj()

    def b_body(i, carry):
        for u in range(2):
            j0, j1 = u * 16, (u + 1) * 16
            for n in range(8):
                nxt = (functools.partial(issue_c, n + 2) if n < 6 else functools.partial(issue_kv, n - 6))
                pl.when(i == n)(functools.partial(nxt, j0, j1))
            if u == 0:
                wait_c(i)
                b_attn(i, 0)
                b_attn(i, 2)
            else:
                b_attn(i, 1)
        return carry

    lax.fori_loop(0, 8, b_body, 0)
    b_norm()

    def a_body(g, carry):
        pl.when(g < H - 2)(lambda: issue_kv(g + 2, 0, NP))
        pl.when(g == H - 2)(lambda: issue_o(0))
        pl.when(g == H - 1)(lambda: issue_o(1))
        wait_kv(g)
        a_group(g)
        pl.when(g < 8)(lambda: ctx_piece(g))
        return carry

    lax.fori_loop(0, H, a_body, 0)

    acc_a = jnp.zeros((8, DM), F32)
    acc_b = jnp.zeros((8, DM), F32)
    issue_o(2)
    ob_build()
    acc_a = o_proj(acc_a, oa_v, wo_v, fsems.at[0], 0, 0, 8)
    acc_b = o_proj(acc_b, ob_v, bo_v, fsems.at[1], 0, 0, 8)
    issue_o_last()
    for t in (1, 2):
        acc_a = o_proj(acc_a, oa_v, wo_v, fsems.at[2 * t], t, 0, 8)
        acc_b = o_proj(acc_b, ob_v, bo_v, fsems.at[2 * t + 1], t, 0, 8)
    acc_a = o_proj(acc_a, oa_v, wo_v, fsems.at[6], 3, 0, 8)
    o_ref[:, 0:DM] = acc_a[0:B, :].astype(o_ref.dtype)
    for n, (h0, k) in enumerate(TAIL):
        acc_b = o_proj(acc_b, ob_v, bo_v, fsems.at[7 + n], 3, h0, k)
    o_ref[:, DM:2 * DM] = acc_b[0:B, :].astype(o_ref.dtype)


def _kernel(*refs):
    pl.run_scoped(
        functools.partial(_body, *refs),
        pltpu.SemaphoreType.DMA((3,)),
        pltpu.SemaphoreType.DMA((1,)),
        pltpu.SemaphoreType.DMA((11,)),
    )


@jax.jit
def pallas_concat_heads__sliding_block_cached__compressed_kv_cla__decode_kernel(
    A_x: jax.Array,
    A_k_cache: jax.Array,
    A_v_cache: jax.Array,
    A_wq: jax.Array,
    A_wo: jax.Array,
    B_x: jax.Array,
    B_c_kv: jax.Array,
    B_w_q: jax.Array,
    B_w_uk: jax.Array,
    B_w_uv: jax.Array,
    B_w_o: jax.Array,
):
    w3_shape = (4, 128, 2, 16, DH)
    hbm = pl.BlockSpec(memory_space=pl.ANY)
    vmem = pltpu.VMEM
    out = pl.pallas_call(
        _kernel,
        out_shape=jax.ShapeDtypeStruct((B, 2 * DM), BF16),
        in_specs=[hbm] * 11,
        out_specs=pl.BlockSpec(memory_space=pltpu.VMEM),
        scratch_shapes=[
            vmem((B, DM), BF16),
            vmem((B, DM), BF16),
            vmem((3, 2, B, W, DH), BF16),
            vmem((4, 128, H * DH), BF16),
            vmem((4, 1024, DM), BF16),
            vmem((16, 1024, DM), BF16),
            vmem(w3_shape, BF16),
            vmem(w3_shape, BF16),
            vmem(w3_shape, BF16),
            vmem((4, 1024, DM), BF16),
            vmem((128, 2048), BF16),
            vmem((2048, 128), BF16),
            vmem((64, 8192), BF16),
            vmem((128, DH), BF16),
            vmem((B, H, DM), BF16),
            vmem((B, H, 1), F32),
            vmem((B, H, 1), F32),
            vmem((B, H, DM), F32),
            vmem((8, 64, 128), BF16),
            vmem((2, 64, DH), F32),
            vmem((H, 8, DH), F32),
            vmem((H, 8, DH), F32),
            vmem((H, 8, DH), F32),
        ],
        compiler_params=pltpu.CompilerParams(vmem_limit_bytes=100 * 1024 * 1024),
        name="fused_decode",
    )(
        A_x.reshape(B, DM),
        A_k_cache.reshape(B * H, SK, DH),
        A_v_cache.reshape(B * H, SK, DH),
        A_wq.reshape(4, 128, H * DH),
        A_wo.reshape(4, 1024, DM),
        B_x.reshape(B, DM),
        B_c_kv.reshape(16, 1024, DM),
        B_w_q.reshape(w3_shape),
        B_w_uk.reshape(w3_shape),
        B_w_uv.reshape(w3_shape),
        B_w_o.reshape(4, 1024, DM),
    )
    return out.reshape(B, 1, 2 * DM)
```

```python
import functools

import jax
import jax.numpy as jnp
from jax import lax
import jax.experimental.pallas as pl
import jax.experimental.pallas.tpu as pltpu

F32 = jnp.float32
BF16 = jnp.bfloat16

B = 4
H = 32
DH = 128
DM = 512
SK = 4096
W = 1024
SCALE = DH ** -0.5

NP = 32
NT = (((1,), (1,)), ((), ()))


def _iota(shape, d):
    return lax.broadcasted_iota(jnp.int32, shape, d)


def _dot(a, b):
    return jnp.dot(a, b, preferred_element_type=F32)


def _dot_nt(a, b):
    return lax.dot_general(a, b, NT, preferred_element_type=F32)


def _body(
    xa_hbm, k_hbm, v_hbm, wq_hbm, wo_hbm,
    xb_hbm, c_hbm, bq_hbm, buk_hbm, buv_hbm, bo_hbm,
    o_ref,
    xa_v, xb_v, kv_v, wq_v, wo_v, c_v, bq_v, buk_v, buv_v, bo_v,
    e_v, et_v, x2_v, qb_v, qabs_v, m_v, l_v, acc_v, cn_v, ctx_v,
    qa_v, oa_v, ob_v,
    sems, xsem, fsems,
):
    def start(src, dst, sem, prio):
        pltpu.make_async_copy(src, dst, sem).start(priority=prio)

    def wait(dst, sem):
        pltpu.make_async_copy(dst, dst, sem).wait()

    def w3_idx(p0, i, n):
        return (pl.ds(p0, 2), pl.ds(i * 2, n * 2))

    def c_idx(p0, i, n):
        return (pl.ds(p0, 2), pl.ds(i * 16, n * 16), slice(None))

    def start2(src, dst, idx, sem, prio):
        start(src.at[idx], dst.at[idx], sem, prio)

    def issue_s0(t, j0, j1):
        sem = sems.at[t % 3]
        for j in range(j0, j1):
            i = t * 16 + j // 2
            prio0 = 1 if (t == 0 and j < 16) else 0
            if j % 2 == 0:
                start2(buk_hbm, buk_v, w3_idx(2, i, 1), sem, prio0)
                start2(bq_hbm, bq_v, w3_idx(2, i, 1), sem, 1)
            else:
                start2(bq_hbm, bq_v, w3_idx(0, i, 1), sem, prio0)
                start2(c_hbm, c_v, c_idx(0, i, 1), sem, 1)

    def wait_s0(t):
        sem = sems.at[t % 3]
        wait(buk_v.at[w3_idx(2, t * 16, 16)], sem)
        wait(bq_v.at[:, pl.ds(t * 32, 32)], sem)
        wait(c_v.at[c_idx(0, t * 16, 16)], sem)

    def issue_s1(t, j0, j1):
        sem = sems.at[(4 + t) % 3]
        for j in range(j0, j1):
            i = t * 16 + j // 2
            if j % 2 == 0:
                start2(buv_hbm, buv_v, w3_idx(2, i, 1), sem, 0)
            else:
                start2(buk_hbm, buk_v, w3_idx(0, i, 1), sem, 0)
            idx = (slice(None), pl.ds((t * 4 + j // 8) * 8, 8), pl.ds((j % 8) * 512, 512))
            start2(wq_hbm, wq_v, idx, sem, 1)

    def wait_s1(t):
        sem = sems.at[(4 + t) % 3]
        wait(buv_v.at[w3_idx(2, t * 16, 16)], sem)
        wait(buk_v.at[w3_idx(0, t * 16, 16)], sem)
        wait(wq_v.at[:, pl.ds(t * 32, 32), :], sem)

    def issue_c(i, j0, j1):
        sem = sems.at[(8 + i) % 3]
        t = i % 4
        for j in range(j0, j1):
            rows8 = pl.ds(t * 256 + j * 8, 8)
            start2(c_hbm, c_v, (pl.ds(2 if i < 4 else 10, 4), rows8, slice(None)), sem, 0)
            if i < 4:
                start2(c_hbm, c_v, (pl.ds(6, 4), rows8, slice(None)), sem, 1)
            elif j % 2 == 0:
                start2(c_hbm, c_v, c_idx(14, t * 16 + j // 2, 1), sem, 1)
            else:
                start2(buv_hbm, buv_v, w3_idx(0, t * 16 + j // 2, 1), sem, 1)

    def wait_c(i):
        sem = sems.at[(8 + i) % 3]
        rows = pl.ds(pl.multiple_of((i % 4) * 256, 256), 256)
        wait(c_v.at[pl.ds(2 + (i // 4) * 8, 6), rows, :], sem)
        pl.when(i < 4)(lambda: wait(c_v.at[pl.ds(8, 2), rows, :], sem))
        pl.when(i >= 4)(lambda: wait(buv_v.at[w3_idx(0, (i % 4) * 16, 16)], sem))

    def issue_kv(g, j0, j1):
        slot = (16 + g) % 3
        sem = sems.at[slot]
        for j in range(j0, j1):
            for u, src in enumerate((k_hbm, v_hbm)):
                if isinstance(g, int) and g == 0:
                    hh, r = j % 2, (j // 2) * 64
                    start(src.at[pl.ds(126 if hh == 0 else 0, 2), pl.ds(SK - W + r, 64), :],
                          kv_v.at[slot, u, pl.ds(hh * 2, 2), pl.ds(r, 64), :], sem, u)
                else:
                    start(src.at[pl.ds(g * 4 - 2, 4), pl.ds(SK - W + j * 32, 32), :],
                          kv_v.at[slot, u, :, pl.ds(j * 32, 32), :], sem, u)

    def wait_kv(g):
        slot = (16 + g) % 3
        wait(kv_v.at[slot], sems.at[slot])

    def o_idx(t, j):
        r = (t ^ ((j % 2) * 2)) * 256 + (j // 2) * 16
        return c_idx((j % 2) * 2, r // 16, 1)

    def o_heads(t):
        return [(p, (t ^ (p & 2)) * 256 + hb * 128) for hb in range(2) for p in range(4)]

    def issue_o(t):
        for j in range(NP):
            start2(wo_hbm, wo_v, o_idx(t, j), fsems.at[2 * t], 0)
            start2(bo_hbm, bo_v, o_idx(t, j), fsems.at[2 * t + 1], 1)

    TAIL = ((0, 4), (4, 2), (6, 1), (7, 1))

    def issue_o_last():
        heads = o_heads(3)
        lo = [(0, o_idx(3, j)) for j in range(16)]
        lo += [(1, c_idx(0, heads[4][1] // 16 + i, 1)) for i in range(8)]
        for n in (2, 3):
            p, r0 = heads[4 + n]
            lo += [(n, (p, pl.ds(r0 + r, 32), slice(None))) for r in range(0, 128, 32)]
        for j in range(NP):
            start2(wo_hbm, wo_v, o_idx(3, j), fsems.at[6], 0)
            start2(bo_hbm, bo_v, lo[j][1], fsems.at[7 + lo[j][0]], 1)

    def diag_mask():
        return (_iota((64, 2048), 1) & 15) == (_iota((64, 2048), 0) & 15)

    def w3(ref, k, hf):
        return ref[k, :, hf].reshape(2048, DH)

    def build_consts():
        e_v[...] = jnp.where(_iota((128, 2048), 0) == (_iota((128, 2048), 1) >> 4), 1.0, 0.0).astype(BF16)
        et_v[...] = jnp.where(_iota((2048, 128), 1) == (_iota((2048, 128), 0) >> 4), 1.0, 0.0).astype(BF16)
        m_v[...] = jnp.full(m_v.shape, -jnp.inf, F32)
        l_v[...] = jnp.zeros(l_v.shape, F32)
        acc_v[...] = jnp.zeros(acc_v.shape, F32)
        oa_v[...] = jnp.zeros(oa_v.shape, F32)

    def build_x2():
        x = xb_v[...].astype(F32)
        xrep = jnp.concatenate(
            [jnp.broadcast_to(x[b:b + 1, :], (16, DM)) for b in range(B)], axis=0).astype(BF16)
        for k in range(4):
            xe = _dot(xrep[:, k * 128:(k + 1) * 128], e_v[...])
            x2_v[:, k * 2048:(k + 1) * 2048] = jnp.where(diag_mask(), xe, 0.0).astype(BF16)

    def qb_half(hf):
        acc = None
        for k in range(4):
            r = _dot(x2_v[:, k * 2048:(k + 1) * 2048], w3(bq_v, k, hf))
            acc = r if acc is None else acc + r
        qb_v[hf * 64:(hf + 1) * 64, :] = acc.astype(BF16)

    def qabs_piece(hf, k):
        r = _dot_nt(qb_v[hf * 64:(hf + 1) * 64, :], w3(buk_v, k, hf))
        r = jnp.where(diag_mask(), r, 0.0).astype(BF16)
        z = _dot(r, et_v[...]).astype(BF16)
        for b in range(B):
            qabs_v[b, hf * 16:(hf + 1) * 16, k * 128:(k + 1) * 128] = z[b * 16:(b + 1) * 16, :]

    def qa_proj():
        x = xa_v[...].astype(F32)
        x8 = jnp.concatenate([x, x], axis=0).astype(BF16)
        acc = None
        for k in range(4):
            r = _dot(x8[:, k * 128:(k + 1) * 128], wq_v[k])
            acc = r if acc is None else acc + r
        for h in range(H):
            qa_v[h] = acc[:, h * DH:(h + 1) * DH]

    def b_attn(i, u):
        rows = pl.ds(pl.multiple_of((i % 4) * 256, 256), 256)
        p0s = [(2 + (i // 4) * 8 + u * 4 + n * 2) % 16 for n in range(2)]
        bs = [p0 // 4 for p0 in p0s]
        cs = [c_v[pl.ds(p0, 2), rows, :].reshape(512, DM) for p0 in p0s]
        ss = [_dot_nt(qabs_v[b], c) * SCALE for b, c in zip(bs, cs)]
        ps, alphas = [], []
        for b, s in zip(bs, ss):
            m_old = m_v[b]
            m_new = jnp.maximum(m_old, jnp.max(s, axis=1, keepdims=True))
            alpha = jnp.exp(m_old - m_new)
            p = jnp.exp(s - m_new)
            l_v[b] = alpha * l_v[b] + jnp.sum(p, axis=1, keepdims=True)
            m_v[b] = m_new
            ps.append(p.astype(BF16))
            alphas.append(alpha)
        for b, p, c, alpha in zip(bs, ps, cs, alphas):
            acc_v[b] = alpha * acc_v[b] + _dot(p, c)

    def b_norm():
        for b in range(B):
            cn = (acc_v[b] / l_v[b]).astype(BF16)
            for hf in range(2):
                for k in range(4):
                    cn_v[hf * 4 + k, b * 16:(b + 1) * 16, :] = (
                        cn[hf * 16:(hf + 1) * 16, k * 128:(k + 1) * 128])
        ctx_v[...] = jnp.zeros(ctx_v.shape, F32)

    def ctx_piece(i):
        xe = _dot(cn_v[i], e_v[...])
        xe = jnp.where(diag_mask(), xe, 0.0).astype(BF16)
        ctx_v[i // 4] += _dot(xe, w3(buv_v, i % 4, i // 4))

    def ob_build():
        ro = _iota((256, 128), 0)
        ri = _iota((256, 128), 1)
        src = ((ro >> 7) << 6) + ((ro & 7) << 4) + ((ro >> 3) & 15)
        perm = jnp.where(((ro & 7) < 4) & (ri == src), 1.0, 0.0).astype(BF16)
        ctx = ctx_v[...].reshape(128, DH).astype(BF16)
        ob_v[...] = _dot(perm, ctx).reshape(H, 8, DH)

    def a_group(g):
        slot = (16 + g) % 3
        fs = [(g * 4 + (126 + j)) & 127 for j in range(4)]
        ss = [_dot_nt(qa_v[f & 31].astype(BF16), kv_v[slot, 0, j]) * SCALE for j, f in enumerate(fs)]
        ps = [jnp.exp(s - jnp.max(s, axis=1, keepdims=True)) for s in ss]
        ls = [jnp.sum(p, axis=1, keepdims=True) for p in ps]
        os = [_dot(p.astype(BF16), kv_v[slot, 1, j]) / l for j, (p, l) in enumerate(zip(ps, ls))]
        for f, o in zip(fs, os):
            oa_v[f & 31] = jnp.where(_iota((8, DH), 0) == (f >> 5), o, oa_v[f & 31])

    def o_proj(acc, o_v, w_v, sem, t, h0, n):
        heads = o_heads(t)[h0:h0 + n]
        for p, r0 in heads:
            wait(w_v.at[p, pl.ds(r0, 128), :], sem)
        for p, r0 in heads:
            acc += _dot(o_v[p * 8 + r0 // 128].astype(BF16), w_v[p, r0:r0 + 128, :])
        return acc

    issue_s0(0, 0, 2)
    start(xa_hbm, xa_v, xsem.at[0], 0)
    start(xb_hbm, xb_v, xsem.at[0], 0)
    issue_s0(0, 2, NP)
    issue_s0(1, 0, NP)

    issue_s0(2, 0, NP)
    wait_s0(0)
    wait(xa_v, xsem.at[0])
    wait(xb_v, xsem.at[0])
    build_consts()

    issue_s0(3, 0, NP)
    wait_s0(1)
    build_x2()

    issue_s1(0, 0, NP)
    wait_s0(2)

    issue_s1(1, 0, 16)
    wait_s0(3)
    qb_half(0)
    issue_s1(1, 16, NP)
    qb_half(1)

    for hf in range(2):
        issue_s1(2 + hf, 0, NP)
        wait_s1(hf)
        qabs_piece(hf, 2)
        qabs_piece(hf, 3)

    issue_c(0, 0, NP)
    wait_s1(2)

    issue_c(1, 0, 16)
    wait_s1(3)
    qabs_piece(0, 0)
    qabs_piece(0, 1)
    issue_c(1, 16, 24)
    qabs_piece(1, 0)
    qabs_piece(1, 1)
    issue_c(1, 24, NP)
    qa_proj()

    def b_body(i, carry):
        for u in range(2):
            j0, j1 = u * 16, (u + 1) * 16
            for n in range(8):
                nxt = (functools.partial(issue_c, n + 2) if n < 6 else functools.partial(issue_kv, n - 6))
                pl.when(i == n)(functools.partial(nxt, j0, j1))
            if u == 0:
                wait_c(i)
            b_attn(i, u)
        return carry

    lax.fori_loop(0, 8, b_body, 0)
    b_norm()

    def a_body(g, carry):
        pl.when(g < H - 2)(lambda: issue_kv(g + 2, 0, NP))
        pl.when(g == H - 2)(lambda: issue_o(0))
        pl.when(g == H - 1)(lambda: issue_o(1))
        wait_kv(g)
        a_group(g)
        pl.when(g < 8)(lambda: ctx_piece(g))
        return carry

    lax.fori_loop(0, H, a_body, 0)

    acc_a = jnp.zeros((8, DM), F32)
    acc_b = jnp.zeros((8, DM), F32)
    issue_o(2)
    ob_build()
    acc_a = o_proj(acc_a, oa_v, wo_v, fsems.at[0], 0, 0, 8)
    acc_b = o_proj(acc_b, ob_v, bo_v, fsems.at[1], 0, 0, 8)
    issue_o_last()
    for t in (1, 2):
        acc_a = o_proj(acc_a, oa_v, wo_v, fsems.at[2 * t], t, 0, 8)
        acc_b = o_proj(acc_b, ob_v, bo_v, fsems.at[2 * t + 1], t, 0, 8)
    acc_a = o_proj(acc_a, oa_v, wo_v, fsems.at[6], 3, 0, 8)
    o_ref[:, 0:DM] = acc_a[0:B, :].astype(o_ref.dtype)
    for n, (h0, k) in enumerate(TAIL):
        acc_b = o_proj(acc_b, ob_v, bo_v, fsems.at[7 + n], 3, h0, k)
    o_ref[:, DM:2 * DM] = acc_b[0:B, :].astype(o_ref.dtype)


def _kernel(*refs):
    pl.run_scoped(
        functools.partial(_body, *refs),
        pltpu.SemaphoreType.DMA((3,)),
        pltpu.SemaphoreType.DMA((1,)),
        pltpu.SemaphoreType.DMA((11,)),
    )


@jax.jit
def pallas_concat_heads__sliding_block_cached__compressed_kv_cla__decode_kernel(
    A_x: jax.Array,
    A_k_cache: jax.Array,
    A_v_cache: jax.Array,
    A_wq: jax.Array,
    A_wo: jax.Array,
    B_x: jax.Array,
    B_c_kv: jax.Array,
    B_w_q: jax.Array,
    B_w_uk: jax.Array,
    B_w_uv: jax.Array,
    B_w_o: jax.Array,
):
    w3_shape = (4, 128, 2, 16, DH)
    hbm = pl.BlockSpec(memory_space=pl.ANY)
    vmem = pltpu.VMEM
    out = pl.pallas_call(
        _kernel,
        out_shape=jax.ShapeDtypeStruct((B, 2 * DM), BF16),
        in_specs=[hbm] * 11,
        out_specs=pl.BlockSpec(memory_space=pltpu.VMEM),
        scratch_shapes=[
            vmem((B, DM), BF16),
            vmem((B, DM), BF16),
            vmem((3, 2, B, W, DH), BF16),
            vmem((4, 128, H * DH), BF16),
            vmem((4, 1024, DM), BF16),
            vmem((16, 1024, DM), BF16),
            vmem(w3_shape, BF16),
            vmem(w3_shape, BF16),
            vmem(w3_shape, BF16),
            vmem((4, 1024, DM), BF16),
            vmem((128, 2048), BF16),
            vmem((2048, 128), BF16),
            vmem((64, 8192), BF16),
            vmem((128, DH), BF16),
            vmem((B, H, DM), BF16),
            vmem((B, H, 1), F32),
            vmem((B, H, 1), F32),
            vmem((B, H, DM), F32),
            vmem((8, 64, 128), BF16),
            vmem((2, 64, DH), F32),
            vmem((H, 8, DH), F32),
            vmem((H, 8, DH), F32),
            vmem((H, 8, DH), F32),
        ],
        compiler_params=pltpu.CompilerParams(vmem_limit_bytes=100 * 1024 * 1024),
        name="fused_decode",
    )(
        A_x.reshape(B, DM),
        A_k_cache.reshape(B * H, SK, DH),
        A_v_cache.reshape(B * H, SK, DH),
        A_wq.reshape(4, 128, H * DH),
        A_wo.reshape(4, 1024, DM),
        B_x.reshape(B, DM),
        B_c_kv.reshape(16, 1024, DM),
        B_w_q.reshape(w3_shape),
        B_w_uk.reshape(w3_shape),
        B_w_uv.reshape(w3_shape),
        B_w_o.reshape(4, 1024, DM),
    )
    return out.reshape(B, 1, 2 * DM)
```

```python
import functools

import jax
import jax.numpy as jnp
from jax import lax
import jax.experimental.pallas as pl
import jax.experimental.pallas.tpu as pltpu

F32 = jnp.float32
BF16 = jnp.bfloat16

B = 4
H = 32
DH = 128
DM = 512
SK = 4096
W = 1024
SCALE = DH ** -0.5

NP = 32
NT = (((1,), (1,)), ((), ()))


def _iota(shape, d):
    return lax.broadcasted_iota(jnp.int32, shape, d)


def _dot(a, b):
    return jnp.dot(a, b, preferred_element_type=F32)


def _dot_nt(a, b):
    return lax.dot_general(a, b, NT, preferred_element_type=F32)


def _body(
    xa_hbm, k_hbm, v_hbm, wq_hbm, wo_hbm,
    xb_hbm, c_hbm, bq_hbm, buk_hbm, buv_hbm, bo_hbm,
    o_ref,
    xa_v, xb_v, kv_v, wq_v, wo_v, c_v, bq_v, buk_v, buv_v, bo_v,
    e_v, et_v, x2_v, qb_v, qabs_v, m_v, l_v, acc_v, cn_v, ctx_v,
    qa_v, oa_v, ob_v,
    sems, xsem, fsems,
):
    def start(src, dst, sem, prio):
        pltpu.make_async_copy(src, dst, sem).start(priority=prio)

    def wait(dst, sem):
        pltpu.make_async_copy(dst, dst, sem).wait()

    def edge(k, n, size, shift):
        return 0 if k == 0 else (n * size if k == n else k * size + shift)

    def w3_idx(p0, np_, k0, k1):
        r0, r1 = edge(k0, 32, 128, 8), edge(k1, 32, 128, 8)
        return (pl.ds(p0, np_), pl.ds(r0, r1 - r0), slice(None))

    def c_idx(p0, np_, k0, k1):
        return (pl.ds(p0, np_), pl.ds(k0 * 32, (k1 - k0) * 32), slice(None))

    def start2(src, dst, idx, sem, prio):
        start(src.at[idx], dst.at[idx], sem, prio)

    def start_w3(src, dst, p, k, sem, prio):
        start2(src, dst, w3_idx(p, 1, k, k + 1), sem, prio)

    def start_c(p, k, sem, prio):
        start2(c_hbm, c_v, c_idx(p, 1, k, k + 1), sem, prio)

    def issue_s0(t, j0, j1):
        sem = sems.at[t % 3]
        for j in range(j0, j1):
            k, n = t * 8 + j // 4, j % 4
            prio0 = 1 if (t == 0 and j < 16) else 0
            if n < 2:
                start_w3(buk_hbm, buk_v, 2 + n, k, sem, prio0)
                start_w3(bq_hbm, bq_v, 2 + n, k, sem, 1)
            else:
                start_w3(bq_hbm, bq_v, n - 2, k, sem, prio0)
                start_c(n - 2, k, sem, 1)

    def wait_s0(t):
        sem = sems.at[t % 3]
        wait(buk_v.at[w3_idx(2, 2, t * 8, t * 8 + 8)], sem)
        wait(bq_v.at[w3_idx(0, 4, t * 8, t * 8 + 8)], sem)
        wait(c_v.at[c_idx(0, 2, t * 8, t * 8 + 8)], sem)

    def issue_s1(t, j0, j1):
        sem = sems.at[(4 + t) % 3]
        for j in range(j0, j1):
            k, n = t * 8 + j // 4, j % 4
            if n < 2:
                start_w3(buv_hbm, buv_v, 2 + n, k, sem, 0)
            else:
                start_w3(buk_hbm, buk_v, n - 2, k, sem, 0)
            kq = (t % 2) * 8 + j // 4
            cols = pl.ds(0, 1920) if kq % 2 == 0 else pl.ds(1920, 2176)
            start2(wq_hbm, wq_v, ((t // 2) * 4 + n, pl.ds((kq // 2) * 8, 8), cols), sem, 1)

    def wait_s1(t):
        sem = sems.at[(4 + t) % 3]
        wait(buv_v.at[w3_idx(2, 2, t * 8, t * 8 + 8)], sem)
        wait(buk_v.at[w3_idx(0, 2, t * 8, t * 8 + 8)], sem)
        wait(wq_v.at[pl.ds((t // 2) * 4, 4), pl.ds((t % 2) * 32, 32), :], sem)

    def issue_c(i, j0, j1):
        sem = sems.at[(8 + i) % 3]
        for j in range(j0, j1):
            k, n = (i % 4) * 8 + j // 4, j % 4
            start_c((2 if i < 4 else 10) + n, k, sem, 0)
            if i < 4:
                start_c(6 + n, k, sem, 1)
            elif n < 2:
                start_c(14 + n, k, sem, 1)
            else:
                start_w3(buv_hbm, buv_v, n - 2, k, sem, 1)

    def wait_c(i):
        sem = sems.at[(8 + i) % 3]
        rows = pl.ds(pl.multiple_of((i % 4) * 256, 256), 256)
        wait(c_v.at[pl.ds(2 + (i // 4) * 8, 6), rows, :], sem)
        pl.when(i < 4)(lambda: wait(c_v.at[pl.ds(8, 2), rows, :], sem))
        for t in range(4):
            pl.when(i == 4 + t)(functools.partial(wait, buv_v.at[w3_idx(0, 2, t * 8, t * 8 + 8)], sem))

    def kv_heads(g):
        return [((g & 15) + ((g >> 4) << 6) + (n * 16 + 2)) & 127 for n in range(4)]

    def issue_kv(g, j0, j1):
        slot = (16 + g) % 3
        sem = sems.at[slot]
        fs = kv_heads(g)
        for j in range(j0, j1):
            k, n = j // 4, j % 4
            r0, r1 = edge(k, 8, 128, -8), edge(k + 1, 8, 128, -8)
            for u, src in enumerate((k_hbm, v_hbm)):
                start(src.at[fs[n], pl.ds(SK - W + r0, r1 - r0), :],
                      kv_v.at[slot, u, n, pl.ds(r0, r1 - r0), :], sem, u)

    def wait_kv(g):
        slot = (16 + g) % 3
        wait(kv_v.at[slot], sems.at[slot])

    def o2_idx(p0, i):
        return (pl.ds(p0, 2), pl.ds(i * 16, 16), slice(None))

    def o_idx(t, j):
        r = (t ^ ((j % 2) * 2)) * 256 + (j // 2) * 16
        return o2_idx((j % 2) * 2, r // 16)

    def o_heads(t):
        return [(p, (t ^ (p & 2)) * 256 + hb * 128) for hb in range(2) for p in range(4)]

    def issue_o(t):
        for j in range(NP):
            start2(wo_hbm, wo_v, o_idx(t, j), fsems.at[2 * t], 0)
            start2(bo_hbm, bo_v, o_idx(t, j), fsems.at[2 * t + 1], 1)

    TAIL = ((0, 4), (4, 2), (6, 1), (7, 1))

    def issue_o_last():
        heads = o_heads(3)
        lo = [(0, o_idx(3, j)) for j in range(16)]
        lo += [(1, o2_idx(0, heads[4][1] // 16 + i)) for i in range(8)]
        for n in (2, 3):
            p, r0 = heads[4 + n]
            lo += [(n, (p, pl.ds(r0 + r, 32), slice(None))) for r in range(0, 128, 32)]
        for j in range(NP):
            start2(wo_hbm, wo_v, o_idx(3, j), fsems.at[6], 0)
            start2(bo_hbm, bo_v, lo[j][1], fsems.at[7 + lo[j][0]], 1)

    def diag_mask():
        return (_iota((64, 2048), 1) & 15) == (_iota((64, 2048), 0) & 15)

    def w3(ref, k, hf):
        return ref[k].reshape(128, 2, 16, DH)[:, hf].reshape(2048, DH)

    def build_consts():
        e_v[...] = jnp.where(_iota((128, 2048), 0) == (_iota((128, 2048), 1) >> 4), 1.0, 0.0).astype(BF16)
        et_v[...] = jnp.where(_iota((2048, 128), 1) == (_iota((2048, 128), 0) >> 4), 1.0, 0.0).astype(BF16)
        m_v[...] = jnp.full(m_v.shape, -jnp.inf, F32)
        l_v[...] = jnp.zeros(l_v.shape, F32)
        acc_v[...] = jnp.zeros(acc_v.shape, F32)
        oa_v[...] = jnp.zeros(oa_v.shape, F32)

    def build_x2():
        x = xb_v[...].astype(F32)
        xrep = jnp.concatenate(
            [jnp.broadcast_to(x[b:b + 1, :], (16, DM)) for b in range(B)], axis=0).astype(BF16)
        for k in range(4):
            xe = _dot(xrep[:, k * 128:(k + 1) * 128], e_v[...])
            x2_v[:, k * 2048:(k + 1) * 2048] = jnp.where(diag_mask(), xe, 0.0).astype(BF16)

    def qb_half(hf):
        acc = None
        for k in range(4):
            r = _dot(x2_v[:, k * 2048:(k + 1) * 2048], w3(bq_v, k, hf))
            acc = r if acc is None else acc + r
        qb_v[hf * 64:(hf + 1) * 64, :] = acc.astype(BF16)

    def qabs_piece(hf, k):
        r = _dot_nt(qb_v[hf * 64:(hf + 1) * 64, :], w3(buk_v, k, hf))
        r = jnp.where(diag_mask(), r, 0.0).astype(BF16)
        z = _dot(r, et_v[...]).astype(BF16)
        for b in range(B):
            qabs_v[b, hf * 16:(hf + 1) * 16, k * 128:(k + 1) * 128] = z[b * 16:(b + 1) * 16, :]

    def qa_proj():
        x = xa_v[...].astype(F32)
        x8 = jnp.concatenate([x, x], axis=0).astype(BF16)
        acc = None
        for k in range(4):
            r = _dot(x8[:, k * 128:(k + 1) * 128], wq_v[2 * k:2 * k + 2].reshape(128, H * DH))
            acc = r if acc is None else acc + r
        for h in range(H):
            qa_v[h] = acc[:, h * DH:(h + 1) * DH]

    def b_attn(i, u):
        rows = pl.ds(pl.multiple_of((i % 4) * 256, 256), 256)
        p0s = [(2 + (i // 4) * 8 + u * 4 + n * 2) % 16 for n in range(2)]
        bs = [p0 // 4 for p0 in p0s]
        cs = [c_v[pl.ds(p0, 2), rows, :].reshape(512, DM) for p0 in p0s]
        ss = [_dot_nt(qabs_v[b], c) * SCALE for b, c in zip(bs, cs)]
        ps, alphas = [], []
        for b, s in zip(bs, ss):
            m_old = m_v[b]
            m_new = jnp.maximum(m_old, jnp.max(s, axis=1, keepdims=True))
            alpha = jnp.exp(m_old - m_new)
            p = jnp.exp(s - m_new)
            l_v[b] = alpha * l_v[b] + jnp.sum(p, axis=1, keepdims=True)
            m_v[b] = m_new
            ps.append(p.astype(BF16))
            alphas.append(alpha)
        for b, p, c, alpha in zip(bs, ps, cs, alphas):
            acc_v[b] = alpha * acc_v[b] + _dot(p, c)

    def b_norm():
        for b in range(B):
            cn = (acc_v[b] / l_v[b]).astype(BF16)
            for hf in range(2):
                for k in range(4):
                    cn_v[hf * 4 + k, b * 16:(b + 1) * 16, :] = (
                        cn[hf * 16:(hf + 1) * 16, k * 128:(k + 1) * 128])
        ctx_v[...] = jnp.zeros(ctx_v.shape, F32)

    def ctx_piece(hf, k):
        xe = _dot(cn_v[hf * 4 + k], e_v[...])
        xe = jnp.where(diag_mask(), xe, 0.0).astype(BF16)
        ctx_v[hf] += _dot(xe, w3(buv_v, k, hf))

    def ob_build():
        ro = _iota((256, 128), 0)
        ri = _iota((256, 128), 1)
        src = ((ro >> 7) << 6) + ((ro & 7) << 4) + ((ro >> 3) & 15)
        perm = jnp.where(((ro & 7) < 4) & (ri == src), 1.0, 0.0).astype(BF16)
        ctx = ctx_v[...].reshape(128, DH).astype(BF16)
        ob_v[...] = _dot(perm, ctx).reshape(H, 8, DH)

    def a_group(g):
        slot = (16 + g) % 3
        fs = kv_heads(g)
        ss = [_dot_nt(qa_v[f & 31].astype(BF16), kv_v[slot, 0, j]) * SCALE for j, f in enumerate(fs)]
        ps = [jnp.exp(s - jnp.max(s, axis=1, keepdims=True)) for s in ss]
        ls = [jnp.sum(p, axis=1, keepdims=True) for p in ps]
        os = [_dot(p.astype(BF16), kv_v[slot, 1, j]) / l for j, (p, l) in enumerate(zip(ps, ls))]
        for f, o in zip(fs, os):
            oa_v[f & 31] = jnp.where(_iota((8, DH), 0) == (f >> 5), o, oa_v[f & 31])

    def o_proj(acc, o_v, w_v, sem, t, h0, n):
        heads = o_heads(t)[h0:h0 + n]
        for p, r0 in heads:
            wait(w_v.at[p, pl.ds(r0, 128), :], sem)
        for p, r0 in heads:
            acc += _dot(o_v[p * 8 + r0 // 128].astype(BF16), w_v[p, r0:r0 + 128, :])
        return acc

    issue_s0(0, 0, 2)
    start(xa_hbm, xa_v, xsem.at[0], 0)
    start(xb_hbm, xb_v, xsem.at[0], 0)
    issue_s0(0, 2, NP)
    issue_s0(1, 0, NP)

    issue_s0(2, 0, NP)
    wait_s0(0)
    wait(xa_v, xsem.at[0])
    wait(xb_v, xsem.at[0])
    build_consts()

    issue_s0(3, 0, NP)
    wait_s0(1)
    build_x2()

    issue_s1(0, 0, NP)
    wait_s0(2)

    issue_s1(1, 0, 16)
    wait_s0(3)
    qb_half(0)
    issue_s1(1, 16, NP)
    qb_half(1)

    for hf in range(2):
        issue_s1(2 + hf, 0, NP)
        wait_s1(hf)
        qabs_piece(hf, 2)
        qabs_piece(hf, 3)

    issue_c(0, 0, NP)
    wait_s1(2)

    issue_c(1, 0, 16)
    wait_s1(3)
    qabs_piece(0, 0)
    qabs_piece(0, 1)
    issue_c(1, 16, 24)
    qabs_piece(1, 0)
    qabs_piece(1, 1)
    issue_c(1, 24, NP)
    qa_proj()

    def b_body(i, carry):
        for u in range(2):
            j0, j1 = u * 16, (u + 1) * 16
            for n in range(8):
                nxt = (functools.partial(issue_c, n + 2) if n < 6 else functools.partial(issue_kv, n - 6))
                pl.when(i == n)(functools.partial(nxt, j0, j1))
            if u == 0:
                wait_c(i)
            b_attn(i, u)
        return carry

    lax.fori_loop(0, 8, b_body, 0)
    b_norm()

    def a_body(g, carry):
        pl.when(g < H - 2)(lambda: issue_kv(g + 2, 0, NP))
        pl.when(g == H - 2)(lambda: issue_o(0))
        pl.when(g == H - 1)(lambda: issue_o(1))
        wait_kv(g)
        a_group(g)
        pl.when(g < 4)(lambda: ctx_piece(0, g))
        pl.when((g >= 4) & (g < 8))(lambda: ctx_piece(1, g - 4))
        return carry

    lax.fori_loop(0, H, a_body, 0)

    acc_a = jnp.zeros((8, DM), F32)
    acc_b = jnp.zeros((8, DM), F32)
    issue_o(2)
    ob_build()
    acc_a = o_proj(acc_a, oa_v, wo_v, fsems.at[0], 0, 0, 8)
    acc_b = o_proj(acc_b, ob_v, bo_v, fsems.at[1], 0, 0, 8)
    issue_o_last()
    for t in (1, 2):
        acc_a = o_proj(acc_a, oa_v, wo_v, fsems.at[2 * t], t, 0, 8)
        acc_b = o_proj(acc_b, ob_v, bo_v, fsems.at[2 * t + 1], t, 0, 8)
    acc_a = o_proj(acc_a, oa_v, wo_v, fsems.at[6], 3, 0, 8)
    o_ref[:, 0:DM] = acc_a[0:B, :].astype(o_ref.dtype)
    for n, (h0, k) in enumerate(TAIL):
        acc_b = o_proj(acc_b, ob_v, bo_v, fsems.at[7 + n], 3, h0, k)
    o_ref[:, DM:2 * DM] = acc_b[0:B, :].astype(o_ref.dtype)


def _kernel(*refs):
    pl.run_scoped(
        functools.partial(_body, *refs),
        pltpu.SemaphoreType.DMA((3,)),
        pltpu.SemaphoreType.DMA((1,)),
        pltpu.SemaphoreType.DMA((11,)),
    )


@jax.jit
def pallas_concat_heads__sliding_block_cached__compressed_kv_cla__decode_kernel(
    A_x: jax.Array,
    A_k_cache: jax.Array,
    A_v_cache: jax.Array,
    A_wq: jax.Array,
    A_wo: jax.Array,
    B_x: jax.Array,
    B_c_kv: jax.Array,
    B_w_q: jax.Array,
    B_w_uk: jax.Array,
    B_w_uv: jax.Array,
    B_w_o: jax.Array,
):
    w3_shape = (4, 4096, DH)
    hbm = pl.BlockSpec(memory_space=pl.ANY)
    vmem = pltpu.VMEM
    out = pl.pallas_call(
        _kernel,
        out_shape=jax.ShapeDtypeStruct((B, 2 * DM), BF16),
        in_specs=[hbm] * 11,
        out_specs=pl.BlockSpec(memory_space=pltpu.VMEM),
        scratch_shapes=[
            vmem((B, DM), BF16),
            vmem((B, DM), BF16),
            vmem((3, 2, B, W, DH), BF16),
            vmem((8, 64, H * DH), BF16),
            vmem((4, 1024, DM), BF16),
            vmem((16, 1024, DM), BF16),
            vmem(w3_shape, BF16),
            vmem(w3_shape, BF16),
            vmem(w3_shape, BF16),
            vmem((4, 1024, DM), BF16),
            vmem((128, 2048), BF16),
            vmem((2048, 128), BF16),
            vmem((64, 8192), BF16),
            vmem((128, DH), BF16),
            vmem((B, H, DM), BF16),
            vmem((B, H, 1), F32),
            vmem((B, H, 1), F32),
            vmem((B, H, DM), F32),
            vmem((8, 64, 128), BF16),
            vmem((2, 64, DH), F32),
            vmem((H, 8, DH), F32),
            vmem((H, 8, DH), F32),
            vmem((H, 8, DH), F32),
        ],
        compiler_params=pltpu.CompilerParams(vmem_limit_bytes=100 * 1024 * 1024),
        name="fused_decode",
    )(
        A_x.reshape(B, DM),
        A_k_cache.reshape(B * H, SK, DH),
        A_v_cache.reshape(B * H, SK, DH),
        A_wq.reshape(8, 64, H * DH),
        A_wo.reshape(4, 1024, DM),
        B_x.reshape(B, DM),
        B_c_kv.reshape(16, 1024, DM),
        B_w_q.reshape(w3_shape),
        B_w_uk.reshape(w3_shape),
        B_w_uv.reshape(w3_shape),
        B_w_o.reshape(4, 1024, DM),
    )
    return out.reshape(B, 1, 2 * DM)
```

```python
import functools

import jax
import jax.numpy as jnp
from jax import lax
import jax.experimental.pallas as pl
import jax.experimental.pallas.tpu as pltpu

F32 = jnp.float32
BF16 = jnp.bfloat16

B = 4
H = 32
DH = 128
DM = 512
SK = 4096
W = 1024
SCALE = DH ** -0.5

NP = 32
NT = (((1,), (1,)), ((), ()))


def _iota(shape, d):
    return lax.broadcasted_iota(jnp.int32, shape, d)


def _dot(a, b):
    return jnp.dot(a, b, preferred_element_type=F32)


def _dot_nt(a, b):
    return lax.dot_general(a, b, NT, preferred_element_type=F32)


def _body(
    xa_hbm, k_hbm, v_hbm, wq_hbm, wo_hbm,
    xb_hbm, c_hbm, bq_hbm, buk_hbm, buv_hbm, bo_hbm,
    o_ref,
    xa_v, xb_v, kv_v, wq_v, wo_v, c_v, bq_v, buk_v, buv_v, bo_v,
    e_v, et_v, x2_v, qb_v, qabs_v, m_v, l_v, acc_v, cn_v, ctx_v,
    qa_v, oa_v, ob_v,
    sems, xsem, fsems,
):
    def start(src, dst, sem, prio):
        pltpu.make_async_copy(src, dst, sem).start(priority=prio)

    def wait(dst, sem):
        pltpu.make_async_copy(dst, dst, sem).wait()

    def edge(k, n, size, shift):
        return 0 if k == 0 else (n * size if k == n else k * size + shift)

    def w3_idx(p0, np_, k0, k1):
        r0, r1 = edge(k0, 32, 128, 8), edge(k1, 32, 128, 8)
        return (pl.ds(p0, np_), pl.ds(r0, r1 - r0), slice(None))

    def c_idx(p0, np_, k0, k1):
        return (pl.ds(p0, np_), pl.ds(k0 * 32, (k1 - k0) * 32), slice(None))

    def start2(src, dst, idx, sem, prio):
        start(src.at[idx], dst.at[idx], sem, prio)

    def start_w3(src, dst, p, k, sem, prio):
        start2(src, dst, w3_idx(p, 1, k, k + 1), sem, prio)

    def start_c(p, k, sem, prio):
        start2(c_hbm, c_v, c_idx(p, 1, k, k + 1), sem, prio)

    def issue_s0(t, j0, j1):
        sem = sems.at[t % 3]
        for j in range(j0, j1):
            k, n = t * 8 + j // 4, j % 4
            for u in range(2):
                prio = 1 if (t == 0 and j < 16) else u
                if n == 0:
                    start_w3(buk_hbm, buk_v, 2 + u, k, sem, prio)
                elif n < 3:
                    start_w3(bq_hbm, bq_v, (n - 1) * 2 + u, k, sem, prio)
                else:
                    start_c(u, k, sem, prio)

    def wait_s0(t):
        sem = sems.at[t % 3]
        wait(buk_v.at[w3_idx(2, 2, t * 8, t * 8 + 8)], sem)
        wait(bq_v.at[w3_idx(0, 4, t * 8, t * 8 + 8)], sem)
        wait(c_v.at[c_idx(0, 2, t * 8, t * 8 + 8)], sem)

    def issue_s1(t, j0, j1):
        sem = sems.at[(4 + t) % 3]
        for j in range(j0, j1):
            k, n = t * 8 + j // 4, j % 4
            if n < 2:
                start_w3(buv_hbm, buv_v, 2 + n, k, sem, 0)
            else:
                start_w3(buk_hbm, buk_v, n - 2, k, sem, 0)
            kq = (t % 2) * 8 + j // 4
            cols = pl.ds(0, 1920) if kq % 2 == 0 else pl.ds(1920, 2176)
            start2(wq_hbm, wq_v, ((t // 2) * 4 + n, pl.ds((kq // 2) * 8, 8), cols), sem, 1)

    def wait_s1(t):
        sem = sems.at[(4 + t) % 3]
        wait(buv_v.at[w3_idx(2, 2, t * 8, t * 8 + 8)], sem)
        wait(buk_v.at[w3_idx(0, 2, t * 8, t * 8 + 8)], sem)
        wait(wq_v.at[pl.ds((t // 2) * 4, 4), pl.ds((t % 2) * 32, 32), :], sem)

    def issue_c(i, j0, j1):
        sem = sems.at[(8 + i) % 3]
        for j in range(j0, j1):
            k, n = (i % 4) * 8 + j // 4, j % 4
            for u in range(2):
                if i < 4:
                    start_c(2 + u * 4 + n, k, sem, u)
                elif n < 3:
                    start_c(10 + n * 2 + u, k, sem, u)
                else:
                    start_w3(buv_hbm, buv_v, u, k, sem, u)

    def wait_c(i):
        sem = sems.at[(8 + i) % 3]
        rows = pl.ds(pl.multiple_of((i % 4) * 256, 256), 256)
        wait(c_v.at[pl.ds(2 + (i // 4) * 8, 6), rows, :], sem)
        pl.when(i < 4)(lambda: wait(c_v.at[pl.ds(8, 2), rows, :], sem))
        for t in range(4):
            pl.when(i == 4 + t)(functools.partial(wait, buv_v.at[w3_idx(0, 2, t * 8, t * 8 + 8)], sem))

    def kv_heads(g):
        return [(((g & 1) << 5) + (g >> 1) + (d + 2)) & 127 for d in (0, 16, 64, 80)]

    def issue_kv(g, j0, j1):
        slot = (16 + g) % 3
        sem = sems.at[slot]
        fs = kv_heads(g)
        for j in range(j0, j1):
            k, n = j // 4, j % 4
            r0, r1 = edge(k, 8, 128, -8), edge(k + 1, 8, 128, -8)
            for u, src in enumerate((k_hbm, v_hbm)):
                start(src.at[fs[n], pl.ds(SK - W + r0, r1 - r0), :],
                      kv_v.at[slot, u, n, pl.ds(r0, r1 - r0), :], sem, u)

    def wait_kv(g):
        slot = (16 + g) % 3
        wait(kv_v.at[slot], sems.at[slot])

    def o_heads(t):
        return [(p, (t ^ (p & 2)) * 256 + hb * 128) for hb in range(2) for p in range(4)]

    def o_chunks(heads):
        return [(p, pl.ds(r0 + r, 32), slice(None)) for r in range(0, 128, 32) for p, r0 in heads]

    def o_order(t, groups):
        heads = o_heads(t)
        return [(n, idx) for n, (h0, k) in enumerate(groups) for idx in o_chunks(heads[h0:h0 + k])]

    HALVES = ((0, 4), (4, 4))
    TAIL = ((0, 4), (4, 2), (6, 1), (7, 1))

    def issue_o(t):
        for (_, ia), (n, ib) in zip(o_order(t, HALVES), o_order(t, HALVES if t < 3 else TAIL)):
            start2(wo_hbm, wo_v, ia, fsems.at[2 * t], 0)
            start2(bo_hbm, bo_v, ib, fsems.at[2 * t + 1 + (n if t == 3 else 0)], 1)

    def diag_mask():
        return (_iota((64, 2048), 1) & 15) == (_iota((64, 2048), 0) & 15)

    def w3(ref, k, hf):
        return ref[k].reshape(128, 2, 16, DH)[:, hf].reshape(2048, DH)

    def build_consts():
        e_v[...] = jnp.where(_iota((128, 2048), 0) == (_iota((128, 2048), 1) >> 4), 1.0, 0.0).astype(BF16)
        et_v[...] = jnp.where(_iota((2048, 128), 1) == (_iota((2048, 128), 0) >> 4), 1.0, 0.0).astype(BF16)
        m_v[...] = jnp.full(m_v.shape, -jnp.inf, F32)
        l_v[...] = jnp.zeros(l_v.shape, F32)
        acc_v[...] = jnp.zeros(acc_v.shape, F32)
        oa_v[...] = jnp.zeros(oa_v.shape, F32)

    def build_x2():
        x = xb_v[...].astype(F32)
        xrep = jnp.concatenate(
            [jnp.broadcast_to(x[b:b + 1, :], (16, DM)) for b in range(B)], axis=0).astype(BF16)
        for k in range(4):
            xe = _dot(xrep[:, k * 128:(k + 1) * 128], e_v[...])
            x2_v[:, k * 2048:(k + 1) * 2048] = jnp.where(diag_mask(), xe, 0.0).astype(BF16)

    def qb_half(hf):
        acc = None
        for k in range(4):
            r = _dot(x2_v[:, k * 2048:(k + 1) * 2048], w3(bq_v, k, hf))
            acc = r if acc is None else acc + r
        qb_v[hf * 64:(hf + 1) * 64, :] = acc.astype(BF16)

    def qabs_piece(hf, k):
        r = _dot_nt(qb_v[hf * 64:(hf + 1) * 64, :], w3(buk_v, k, hf))
        r = jnp.where(diag_mask(), r, 0.0).astype(BF16)
        z = _dot(r, et_v[...]).astype(BF16)
        for b in range(B):
            qabs_v[b, hf * 16:(hf + 1) * 16, k * 128:(k + 1) * 128] = z[b * 16:(b + 1) * 16, :]

    def qa_proj():
        x = xa_v[...].astype(F32)
        x8 = jnp.concatenate([x, x], axis=0).astype(BF16)
        acc = None
        for k in range(4):
            r = _dot(x8[:, k * 128:(k + 1) * 128], wq_v[2 * k:2 * k + 2].reshape(128, H * DH))
            acc = r if acc is None else acc + r
        for h in range(H):
            qa_v[h] = acc[:, h * DH:(h + 1) * DH]

    def b_attn(i, u):
        rows = pl.ds(pl.multiple_of((i % 4) * 256, 256), 256)
        p0s = [(2 + (i // 4) * 8 + u * 4 + n * 2) % 16 for n in range(2)]
        bs = [p0 // 4 for p0 in p0s]
        cs = [c_v[pl.ds(p0, 2), rows, :].reshape(512, DM) for p0 in p0s]
        ss = [_dot_nt(qabs_v[b], c) * SCALE for b, c in zip(bs, cs)]
        ps, alphas = [], []
        for b, s in zip(bs, ss):
            m_old = m_v[b]
            m_new = jnp.maximum(m_old, jnp.max(s, axis=1, keepdims=True))
            alpha = jnp.exp(m_old - m_new)
            p = jnp.exp(s - m_new)
            l_v[b] = alpha * l_v[b] + jnp.sum(p, axis=1, keepdims=True)
            m_v[b] = m_new
            ps.append(p.astype(BF16))
            alphas.append(alpha)
        for b, p, c, alpha in zip(bs, ps, cs, alphas):
            acc_v[b] = alpha * acc_v[b] + _dot(p, c)

    def b_norm():
        for b in range(B):
            cn = (acc_v[b] / l_v[b]).astype(BF16)
            for hf in range(2):
                for k in range(4):
                    cn_v[hf * 4 + k, b * 16:(b + 1) * 16, :] = (
                        cn[hf * 16:(hf + 1) * 16, k * 128:(k + 1) * 128])
        ctx_v[...] = jnp.zeros(ctx_v.shape, F32)

    def ctx_piece(hf, k):
        xe = _dot(cn_v[hf * 4 + k], e_v[...])
        xe = jnp.where(diag_mask(), xe, 0.0).astype(BF16)
        ctx_v[hf] += _dot(xe, w3(buv_v, k, hf))

    def ob_build():
        ro = _iota((256, 128), 0)
        ri = _iota((256, 128), 1)
        src = ((ro >> 7) << 6) + ((ro & 7) << 4) + ((ro >> 3) & 15)
        perm = jnp.where(((ro & 7) < 4) & (ri == src), 1.0, 0.0).astype(BF16)
        ctx = ctx_v[...].reshape(128, DH).astype(BF16)
        ob_v[...] = _dot(perm, ctx).reshape(H, 8, DH)

    def a_group(g):
        slot = (16 + g) % 3
        fs = kv_heads(g)
        ss = [_dot_nt(qa_v[f & 31].astype(BF16), kv_v[slot, 0, j]) * SCALE for j, f in enumerate(fs)]
        ps = [jnp.exp(s - jnp.max(s, axis=1, keepdims=True)) for s in ss]
        ls = [jnp.sum(p, axis=1, keepdims=True) for p in ps]
        os = [_dot(p.astype(BF16), kv_v[slot, 1, j]) / l for j, (p, l) in enumerate(zip(ps, ls))]
        for f, o in zip(fs, os):
            oa_v[f & 31] = jnp.where(_iota((8, DH), 0) == (f >> 5), o, oa_v[f & 31])

    def o_proj(acc, o_v, w_v, sem, t, h0, n):
        heads = o_heads(t)[h0:h0 + n]
        for p, r0 in heads:
            wait(w_v.at[p, pl.ds(r0, 128), :], sem)
        for p, r0 in heads:
            acc += _dot(o_v[p * 8 + r0 // 128].astype(BF16), w_v[p, r0:r0 + 128, :])
        return acc

    issue_s0(0, 0, 2)
    start(xa_hbm, xa_v, xsem.at[0], 0)
    start(xb_hbm, xb_v, xsem.at[0], 0)
    issue_s0(0, 2, NP)
    issue_s0(1, 0, NP)

    issue_s0(2, 0, NP)
    wait_s0(0)
    wait(xa_v, xsem.at[0])
    wait(xb_v, xsem.at[0])
    build_consts()

    issue_s0(3, 0, NP)
    wait_s0(1)
    build_x2()

    issue_s1(0, 0, NP)
    wait_s0(2)

    issue_s1(1, 0, 16)
    wait_s0(3)
    qb_half(0)
    issue_s1(1, 16, NP)
    qb_half(1)

    for hf in range(2):
        issue_s1(2 + hf, 0, NP)
        wait_s1(hf)
        qabs_piece(hf, 2)
        qabs_piece(hf, 3)

    issue_c(0, 0, NP)
    wait_s1(2)

    issue_c(1, 0, 16)
    wait_s1(3)
    qabs_piece(0, 0)
    qabs_piece(0, 1)
    issue_c(1, 16, 24)
    qabs_piece(1, 0)
    qabs_piece(1, 1)
    issue_c(1, 24, NP)
    qa_proj()

    def b_body(i, carry):
        for u in range(2):
            j0, j1 = u * 16, (u + 1) * 16
            for n in range(8):
                nxt = (functools.partial(issue_c, n + 2) if n < 6 else functools.partial(issue_kv, n - 6))
                pl.when(i == n)(functools.partial(nxt, j0, j1))
            if u == 0:
                wait_c(i)
            b_attn(i, u)
        return carry

    lax.fori_loop(0, 8, b_body, 0)
    b_norm()

    def a_body(g, carry):
        pl.when(g < H - 2)(lambda: issue_kv(g + 2, 0, NP))
        pl.when(g == H - 2)(lambda: issue_o(0))
        pl.when(g == H - 1)(lambda: issue_o(1))
        wait_kv(g)
        a_group(g)
        pl.when(g < 4)(lambda: ctx_piece(0, g))
        pl.when((g >= 4) & (g < 8))(lambda: ctx_piece(1, g - 4))
        return carry

    lax.fori_loop(0, H, a_body, 0)

    acc_a = jnp.zeros((8, DM), F32)
    acc_b = jnp.zeros((8, DM), F32)
    issue_o(2)
    ob_build()
    acc_a = o_proj(acc_a, oa_v, wo_v, fsems.at[0], 0, 0, 8)
    acc_b = o_proj(acc_b, ob_v, bo_v, fsems.at[1], 0, 0, 8)
    issue_o(3)
    for t in (1, 2):
        acc_a = o_proj(acc_a, oa_v, wo_v, fsems.at[2 * t], t, 0, 8)
        acc_b = o_proj(acc_b, ob_v, bo_v, fsems.at[2 * t + 1], t, 0, 8)
    acc_a = o_proj(acc_a, oa_v, wo_v, fsems.at[6], 3, 0, 8)
    o_ref[:, 0:DM] = acc_a[0:B, :].astype(o_ref.dtype)
    for n, (h0, k) in enumerate(TAIL):
        acc_b = o_proj(acc_b, ob_v, bo_v, fsems.at[7 + n], 3, h0, k)
    o_ref[:, DM:2 * DM] = acc_b[0:B, :].astype(o_ref.dtype)


def _kernel(*refs):
    pl.run_scoped(
        functools.partial(_body, *refs),
        pltpu.SemaphoreType.DMA((3,)),
        pltpu.SemaphoreType.DMA((1,)),
        pltpu.SemaphoreType.DMA((11,)),
    )


@jax.jit
def pallas_concat_heads__sliding_block_cached__compressed_kv_cla__decode_kernel(
    A_x: jax.Array,
    A_k_cache: jax.Array,
    A_v_cache: jax.Array,
    A_wq: jax.Array,
    A_wo: jax.Array,
    B_x: jax.Array,
    B_c_kv: jax.Array,
    B_w_q: jax.Array,
    B_w_uk: jax.Array,
    B_w_uv: jax.Array,
    B_w_o: jax.Array,
):
    w3_shape = (4, 4096, DH)
    hbm = pl.BlockSpec(memory_space=pl.ANY)
    vmem = pltpu.VMEM
    out = pl.pallas_call(
        _kernel,
        out_shape=jax.ShapeDtypeStruct((B, 2 * DM), BF16),
        in_specs=[hbm] * 11,
        out_specs=pl.BlockSpec(memory_space=pltpu.VMEM),
        scratch_shapes=[
            vmem((B, DM), BF16),
            vmem((B, DM), BF16),
            vmem((3, 2, B, W, DH), BF16),
            vmem((8, 64, H * DH), BF16),
            vmem((4, 1024, DM), BF16),
            vmem((16, 1024, DM), BF16),
            vmem(w3_shape, BF16),
            vmem(w3_shape, BF16),
            vmem(w3_shape, BF16),
            vmem((4, 1024, DM), BF16),
            vmem((128, 2048), BF16),
            vmem((2048, 128), BF16),
            vmem((64, 8192), BF16),
            vmem((128, DH), BF16),
            vmem((B, H, DM), BF16),
            vmem((B, H, 1), F32),
            vmem((B, H, 1), F32),
            vmem((B, H, DM), F32),
            vmem((8, 64, 128), BF16),
            vmem((2, 64, DH), F32),
            vmem((H, 8, DH), F32),
            vmem((H, 8, DH), F32),
            vmem((H, 8, DH), F32),
        ],
        compiler_params=pltpu.CompilerParams(vmem_limit_bytes=100 * 1024 * 1024),
        name="fused_decode",
    )(
        A_x.reshape(B, DM),
        A_k_cache.reshape(B * H, SK, DH),
        A_v_cache.reshape(B * H, SK, DH),
        A_wq.reshape(8, 64, H * DH),
        A_wo.reshape(4, 1024, DM),
        B_x.reshape(B, DM),
        B_c_kv.reshape(16, 1024, DM),
        B_w_q.reshape(w3_shape),
        B_w_uk.reshape(w3_shape),
        B_w_uv.reshape(w3_shape),
        B_w_o.reshape(4, 1024, DM),
    )
    return out.reshape(B, 1, 2 * DM)
```

```python
import functools

import jax
import jax.numpy as jnp
from jax import lax
import jax.experimental.pallas as pl
import jax.experimental.pallas.tpu as pltpu

F32 = jnp.float32
BF16 = jnp.bfloat16

B = 4
H = 32
DH = 128
DM = 512
SK = 4096
W = 1024
SCALE = DH ** -0.5

NP = 32
NT = (((1,), (1,)), ((), ()))


def _iota(shape, d):
    return lax.broadcasted_iota(jnp.int32, shape, d)


def _dot(a, b):
    return jnp.dot(a, b, preferred_element_type=F32)


def _dot_nt(a, b):
    return lax.dot_general(a, b, NT, preferred_element_type=F32)


def _body(
    xa_hbm, k_hbm, v_hbm, wq_hbm, wo_hbm,
    xb_hbm, c_hbm, bq_hbm, buk_hbm, buv_hbm, bo_hbm,
    o_ref,
    xa_v, xb_v, kv_v, wq_v, wo_v, c_v, bq_v, buk_v, buv_v, bo_v,
    e_v, et_v, x2_v, qb_v, qabs_v, m_v, l_v, acc_v, cn_v, ctx_v,
    qa_v, oa_v, ob_v,
    sems, xsem, fsems,
):
    def start(src, dst, sem, prio):
        pltpu.make_async_copy(src, dst, sem).start(priority=prio)

    def wait(dst, sem):
        pltpu.make_async_copy(dst, dst, sem).wait()

    def edge(k, n, size, shift):
        return 0 if k == 0 else (n * size if k == n else k * size + shift)

    def w3_idx(p0, np_, k0, k1):
        r0, r1 = edge(k0, 32, 128, 8), edge(k1, 32, 128, 8)
        return (pl.ds(p0, np_), pl.ds(r0, r1 - r0), slice(None))

    def c_idx(p0, np_, k0, k1):
        return (pl.ds(p0, np_), pl.ds(k0 * 32, (k1 - k0) * 32), slice(None))

    def start2(src, dst, idx, sem, prio):
        start(src.at[idx], dst.at[idx], sem, prio)

    def start_w3(src, dst, p, k, sem, prio):
        start2(src, dst, w3_idx(p, 1, k, k + 1), sem, prio)

    def start_c(p, k, sem, prio):
        start2(c_hbm, c_v, c_idx(p, 1, k, k + 1), sem, prio)

    def issue_s0(t, j0, j1):
        sem = sems.at[t % 3]
        for j in range(j0, j1):
            k, n = t * 8 + j // 4, j % 4
            for u in range(2):
                prio = 1 if (t == 0 and j < 16) else u
                if n == 0:
                    start_w3(buk_hbm, buk_v, 2 + u, k, sem, prio)
                elif n < 3:
                    start_w3(bq_hbm, bq_v, (n - 1) * 2 + u, k, sem, prio)
                else:
                    start_c(u, k, sem, prio)

    def wait_s0(t):
        sem = sems.at[t % 3]
        wait(buk_v.at[w3_idx(2, 2, t * 8, t * 8 + 8)], sem)
        wait(bq_v.at[w3_idx(0, 4, t * 8, t * 8 + 8)], sem)
        wait(c_v.at[c_idx(0, 2, t * 8, t * 8 + 8)], sem)

    def issue_s1(t, j0, j1):
        sem = sems.at[(4 + t) % 3]
        for j in range(j0, j1):
            k, n = t * 8 + j // 4, j % 4
            for u in range(2):
                if n == 0:
                    start_w3(buv_hbm, buv_v, 2 + u, k, sem, u)
                elif n == 2:
                    start_w3(buk_hbm, buk_v, u, k, sem, u)
                else:
                    kq = k % 16
                    cols = pl.ds(0, 1920) if kq % 2 == 0 else pl.ds(1920, 2176)
                    idx = ((t // 2) * 4 + n - 1 + u, pl.ds((kq // 2) * 8, 8), cols)
                    start2(wq_hbm, wq_v, idx, sem, u)

    def wait_s1(t):
        sem = sems.at[(4 + t) % 3]
        wait(buv_v.at[w3_idx(2, 2, t * 8, t * 8 + 8)], sem)
        wait(buk_v.at[w3_idx(0, 2, t * 8, t * 8 + 8)], sem)
        wait(wq_v.at[pl.ds((t // 2) * 4, 4), pl.ds((t % 2) * 32, 32), :], sem)

    def issue_c(i, j0, j1):
        sem = sems.at[(8 + i) % 3]
        for j in range(j0, j1):
            k, n = (i % 4) * 8 + j // 4, j % 4
            for u in range(2):
                if i < 4:
                    start_c(2 + n * 2 + u, k, sem, u)
                elif n < 3:
                    start_c(10 + n * 2 + u, k, sem, u)
                else:
                    start_w3(buv_hbm, buv_v, u, k, sem, u)

    def wait_c(i):
        sem = sems.at[(8 + i) % 3]
        rows = pl.ds(pl.multiple_of((i % 4) * 256, 256), 256)
        wait(c_v.at[pl.ds(2 + (i // 4) * 8, 6), rows, :], sem)
        pl.when(i < 4)(lambda: wait(c_v.at[pl.ds(8, 2), rows, :], sem))
        for t in range(4):
            pl.when(i == 4 + t)(functools.partial(wait, buv_v.at[w3_idx(0, 2, t * 8, t * 8 + 8)], sem))

    def kv_heads(g):
        return [(((g & 1) << 5) + (g >> 1) + (d + 2)) & 127 for d in (0, 16, 64, 80)]

    def issue_kv(g, j0, j1):
        slot = (16 + g) % 3
        sem = sems.at[slot]
        fs = kv_heads(g)
        for j in range(j0, j1):
            k, n = j // 4, j % 4
            r0, r1 = edge(k, 8, 128, -8), edge(k + 1, 8, 128, -8)
            for u, src in enumerate((k_hbm, v_hbm)):
                start(src.at[fs[n], pl.ds(SK - W + r0, r1 - r0), :],
                      kv_v.at[slot, u, n, pl.ds(r0, r1 - r0), :], sem, u)

    def wait_kv(g):
        slot = (16 + g) % 3
        wait(kv_v.at[slot], sems.at[slot])

    def o_heads(t):
        return [(p, (t ^ (p & 2)) * 256 + hb * 128) for hb in range(2) for p in range(4)]

    def o_chunks(heads):
        return [(p, pl.ds(r0 + r, 32), slice(None)) for r in range(0, 128, 32) for p, r0 in heads]

    def o_order(t, groups):
        heads = o_heads(t)
        return [(n, idx) for n, (h0, k) in enumerate(groups) for idx in o_chunks(heads[h0:h0 + k])]

    HALVES = ((0, 4), (4, 4))
    TAIL = ((0, 4), (4, 2), (6, 1), (7, 1))

    def issue_o(t):
        for (_, ia), (n, ib) in zip(o_order(t, HALVES), o_order(t, HALVES if t < 3 else TAIL)):
            start2(wo_hbm, wo_v, ia, fsems.at[2 * t], 0)
            start2(bo_hbm, bo_v, ib, fsems.at[2 * t + 1 + (n if t == 3 else 0)], 1)

    def diag_mask():
        return (_iota((64, 2048), 1) & 15) == (_iota((64, 2048), 0) & 15)

    def w3(ref, k, hf):
        return ref[k].reshape(128, 2, 16, DH)[:, hf].reshape(2048, DH)

    def build_consts():
        e_v[...] = jnp.where(_iota((128, 2048), 0) == (_iota((128, 2048), 1) >> 4), 1.0, 0.0).astype(BF16)
        et_v[...] = jnp.where(_iota((2048, 128), 1) == (_iota((2048, 128), 0) >> 4), 1.0, 0.0).astype(BF16)
        m_v[...] = jnp.full(m_v.shape, -jnp.inf, F32)
        l_v[...] = jnp.zeros(l_v.shape, F32)
        acc_v[...] = jnp.zeros(acc_v.shape, F32)
        oa_v[...] = jnp.zeros(oa_v.shape, F32)

    def build_x2():
        x = xb_v[...].astype(F32)
        xrep = jnp.concatenate(
            [jnp.broadcast_to(x[b:b + 1, :], (16, DM)) for b in range(B)], axis=0).astype(BF16)
        for k in range(4):
            xe = _dot(xrep[:, k * 128:(k + 1) * 128], e_v[...])
            x2_v[:, k * 2048:(k + 1) * 2048] = jnp.where(diag_mask(), xe, 0.0).astype(BF16)

    def qb_half(hf):
        acc = None
        for k in range(4):
            r = _dot(x2_v[:, k * 2048:(k + 1) * 2048], w3(bq_v, k, hf))
            acc = r if acc is None else acc + r
        qb_v[hf * 64:(hf + 1) * 64, :] = acc.astype(BF16)

    def qabs_piece(hf, k):
        r = _dot_nt(qb_v[hf * 64:(hf + 1) * 64, :], w3(buk_v, k, hf))
        r = jnp.where(diag_mask(), r, 0.0).astype(BF16)
        z = _dot(r, et_v[...]).astype(BF16)
        for b in range(B):
            qabs_v[b, hf * 16:(hf + 1) * 16, k * 128:(k + 1) * 128] = z[b * 16:(b + 1) * 16, :]

    def qa_proj():
        x = xa_v[...].astype(F32)
        x8 = jnp.concatenate([x, x], axis=0).astype(BF16)
        acc = None
        for k in range(4):
            r = _dot(x8[:, k * 128:(k + 1) * 128], wq_v[2 * k:2 * k + 2].reshape(128, H * DH))
            acc = r if acc is None else acc + r
        for h in range(H):
            qa_v[h] = acc[:, h * DH:(h + 1) * DH]

    def b_attn(i, u):
        rows = pl.ds(pl.multiple_of((i % 4) * 256, 256), 256)
        p0s = [(2 + (i // 4) * 8 + u * 4 + n * 2) % 16 for n in range(2)]
        bs = [p0 // 4 for p0 in p0s]
        cs = [c_v[pl.ds(p0, 2), rows, :].reshape(512, DM) for p0 in p0s]
        ss = [_dot_nt(qabs_v[b], c) * SCALE for b, c in zip(bs, cs)]
        ps, alphas = [], []
        for b, s in zip(bs, ss):
            m_old = m_v[b]
            m_new = jnp.maximum(m_old, jnp.max(s, axis=1, keepdims=True))
            alpha = jnp.exp(m_old - m_new)
            p = jnp.exp(s - m_new)
            l_v[b] = alpha * l_v[b] + jnp.sum(p, axis=1, keepdims=True)
            m_v[b] = m_new
            ps.append(p.astype(BF16))
            alphas.append(alpha)
        for b, p, c, alpha in zip(bs, ps, cs, alphas):
            acc_v[b] = alpha * acc_v[b] + _dot(p, c)

    def b_norm():
        for b in range(B):
            cn = (acc_v[b] / l_v[b]).astype(BF16)
            for hf in range(2):
                for k in range(4):
                    cn_v[hf * 4 + k, b * 16:(b + 1) * 16, :] = (
                        cn[hf * 16:(hf + 1) * 16, k * 128:(k + 1) * 128])
        ctx_v[...] = jnp.zeros(ctx_v.shape, F32)

    def ctx_piece(hf, k):
        xe = _dot(cn_v[hf * 4 + k], e_v[...])
        xe = jnp.where(diag_mask(), xe, 0.0).astype(BF16)
        ctx_v[hf] += _dot(xe, w3(buv_v, k, hf))

    def ob_build():
        ro = _iota((256, 128), 0)
        ri = _iota((256, 128), 1)
        src = ((ro >> 7) << 6) + ((ro & 7) << 4) + ((ro >> 3) & 15)
        perm = jnp.where(((ro & 7) < 4) & (ri == src), 1.0, 0.0).astype(BF16)
        ctx = ctx_v[...].reshape(128, DH).astype(BF16)
        ob_v[...] = _dot(perm, ctx).reshape(H, 8, DH)

    def a_group(g):
        slot = (16 + g) % 3
        fs = kv_heads(g)
        ss = [_dot_nt(qa_v[f & 31].astype(BF16), kv_v[slot, 0, j]) * SCALE for j, f in enumerate(fs)]
        ps = [jnp.exp(s - jnp.max(s, axis=1, keepdims=True)) for s in ss]
        ls = [jnp.sum(p, axis=1, keepdims=True) for p in ps]
        outs = [_dot(p.astype(BF16), kv_v[slot, 1, j]) / l for j, (p, l) in enumerate(zip(ps, ls))]
        for f, o in zip(fs, outs):
            oa_v[f & 31] = jnp.where(_iota((8, DH), 0) == (f >> 5), o, oa_v[f & 31])

    def o_proj(acc, o_v, w_v, sem, t, h0, n):
        heads = o_heads(t)[h0:h0 + n]
        for p, r0 in heads:
            wait(w_v.at[p, pl.ds(r0, 128), :], sem)
        for p, r0 in heads:
            acc += _dot(o_v[p * 8 + r0 // 128].astype(BF16), w_v[p, r0:r0 + 128, :])
        return acc

    issue_s0(0, 0, 2)
    start(xa_hbm, xa_v, xsem.at[0], 0)
    start(xb_hbm, xb_v, xsem.at[0], 0)
    issue_s0(0, 2, NP)
    issue_s0(1, 0, NP)

    issue_s0(2, 0, NP)
    wait_s0(0)
    wait(xa_v, xsem.at[0])
    wait(xb_v, xsem.at[0])
    build_consts()

    issue_s0(3, 0, NP)
    wait_s0(1)
    build_x2()

    issue_s1(0, 0, NP)
    wait_s0(2)

    issue_s1(1, 0, 16)
    wait_s0(3)
    qb_half(0)
    issue_s1(1, 16, NP)
    qb_half(1)

    for hf in range(2):
        issue_s1(2 + hf, 0, NP)
        wait_s1(hf)
        qabs_piece(hf, 2)
        qabs_piece(hf, 3)

    issue_c(0, 0, NP)
    wait_s1(2)

    issue_c(1, 0, 16)
    wait_s1(3)
    qabs_piece(0, 0)
    qabs_piece(0, 1)
    issue_c(1, 16, 24)
    qabs_piece(1, 0)
    qabs_piece(1, 1)
    issue_c(1, 24, NP)
    qa_proj()

    def b_body(i, carry):
        for u in range(2):
            j0, j1 = u * 16, (u + 1) * 16
            for n in range(8):
                nxt = (functools.partial(issue_c, n + 2) if n < 6 else functools.partial(issue_kv, n - 6))
                pl.when(i == n)(functools.partial(nxt, j0, j1))
            if u == 0:
                wait_c(i)
            b_attn(i, u)
        return carry

    lax.fori_loop(0, 8, b_body, 0)
    b_norm()

    def a_body(g, carry):
        pl.when(g < H - 2)(lambda: issue_kv(g + 2, 0, NP))
        pl.when(g == H - 2)(lambda: issue_o(0))
        pl.when(g == H - 1)(lambda: issue_o(1))
        wait_kv(g)
        a_group(g)
        pl.when(g < 4)(lambda: ctx_piece(0, g))
        pl.when((g >= 4) & (g < 8))(lambda: ctx_piece(1, g - 4))
        return carry

    lax.fori_loop(0, H, a_body, 0)

    acc_a = jnp.zeros((8, DM), F32)
    acc_b = jnp.zeros((8, DM), F32)
    issue_o(2)
    ob_build()
    acc_a = o_proj(acc_a, oa_v, wo_v, fsems.at[0], 0, 0, 8)
    acc_b = o_proj(acc_b, ob_v, bo_v, fsems.at[1], 0, 0, 8)
    issue_o(3)
    for t in (1, 2):
        acc_a = o_proj(acc_a, oa_v, wo_v, fsems.at[2 * t], t, 0, 8)
        acc_b = o_proj(acc_b, ob_v, bo_v, fsems.at[2 * t + 1], t, 0, 8)
    acc_a = o_proj(acc_a, oa_v, wo_v, fsems.at[6], 3, 0, 8)
    o_ref[:, 0:DM] = acc_a[0:B, :].astype(o_ref.dtype)
    for n, (h0, k) in enumerate(TAIL):
        acc_b = o_proj(acc_b, ob_v, bo_v, fsems.at[7 + n], 3, h0, k)
    o_ref[:, DM:2 * DM] = acc_b[0:B, :].astype(o_ref.dtype)


def _kernel(*refs):
    pl.run_scoped(
        functools.partial(_body, *refs),
        pltpu.SemaphoreType.DMA((3,)),
        pltpu.SemaphoreType.DMA((1,)),
        pltpu.SemaphoreType.DMA((11,)),
    )


@jax.jit
def pallas_concat_heads__sliding_block_cached__compressed_kv_cla__decode_kernel(
    A_x: jax.Array,
    A_k_cache: jax.Array,
    A_v_cache: jax.Array,
    A_wq: jax.Array,
    A_wo: jax.Array,
    B_x: jax.Array,
    B_c_kv: jax.Array,
    B_w_q: jax.Array,
    B_w_uk: jax.Array,
    B_w_uv: jax.Array,
    B_w_o: jax.Array,
):
    w3_shape = (4, 4096, DH)
    hbm = pl.BlockSpec(memory_space=pl.ANY)
    vmem = pltpu.VMEM
    out = pl.pallas_call(
        _kernel,
        out_shape=jax.ShapeDtypeStruct((B, 2 * DM), BF16),
        in_specs=[hbm] * 11,
        out_specs=pl.BlockSpec(memory_space=pltpu.VMEM),
        scratch_shapes=[
            vmem((B, DM), BF16),
            vmem((B, DM), BF16),
            vmem((3, 2, B, W, DH), BF16),
            vmem((8, 64, H * DH), BF16),
            vmem((4, 1024, DM), BF16),
            vmem((16, 1024, DM), BF16),
            vmem(w3_shape, BF16),
            vmem(w3_shape, BF16),
            vmem(w3_shape, BF16),
            vmem((4, 1024, DM), BF16),
            vmem((128, 2048), BF16),
            vmem((2048, 128), BF16),
            vmem((64, 8192), BF16),
            vmem((128, DH), BF16),
            vmem((B, H, DM), BF16),
            vmem((B, H, 1), F32),
            vmem((B, H, 1), F32),
            vmem((B, H, DM), F32),
            vmem((8, 64, 128), BF16),
            vmem((2, 64, DH), F32),
            vmem((H, 8, DH), F32),
            vmem((H, 8, DH), F32),
            vmem((H, 8, DH), F32),
        ],
        compiler_params=pltpu.CompilerParams(vmem_limit_bytes=100 * 1024 * 1024),
        name="fused_decode",
    )(
        A_x.reshape(B, DM),
        A_k_cache.reshape(B * H, SK, DH),
        A_v_cache.reshape(B * H, SK, DH),
        A_wq.reshape(8, 64, H * DH),
        A_wo.reshape(4, 1024, DM),
        B_x.reshape(B, DM),
        B_c_kv.reshape(16, 1024, DM),
        B_w_q.reshape(w3_shape),
        B_w_uk.reshape(w3_shape),
        B_w_uv.reshape(w3_shape),
        B_w_o.reshape(4, 1024, DM),
    )
    return out.reshape(B, 1, 2 * DM)
```

```python
import functools

import jax
import jax.numpy as jnp
from jax import lax
import jax.experimental.pallas as pl
import jax.experimental.pallas.tpu as pltpu

F32 = jnp.float32
BF16 = jnp.bfloat16

B = 4
H = 32
DH = 128
DM = 512
SK = 4096
W = 1024
SCALE = DH ** -0.5

NP = 32
NT = (((1,), (1,)), ((), ()))


def _iota(shape, d):
    return lax.broadcasted_iota(jnp.int32, shape, d)


def _dot(a, b):
    return jnp.dot(a, b, preferred_element_type=F32)


def _dot_nt(a, b):
    return lax.dot_general(a, b, NT, preferred_element_type=F32)


def _body(
    xa_hbm, k_hbm, v_hbm, wq_hbm, wo_hbm,
    xb_hbm, c_hbm, bq_hbm, buk_hbm, buv_hbm, bo_hbm,
    o_ref,
    xa_v, xb_v, kv_v, wq_v, wo_v, c_v, bq_v, buk_v, buv_v, bo_v,
    e_v, et_v, x2_v, qb_v, qabs_v, m_v, l_v, acc_v, cn_v, ctx_v,
    qa_v, oa_v, ob_v,
    sems, xsem, fsems,
):
    def start(src, dst, sem, prio):
        pltpu.make_async_copy(src, dst, sem).start(priority=prio)

    def wait(dst, sem):
        pltpu.make_async_copy(dst, dst, sem).wait()

    def edge(k, n, size, shift):
        return 0 if k == 0 else (n * size if k == n else k * size + shift)

    def w3_idx(p0, np_, k0, k1):
        r0, r1 = edge(k0, 32, 128, 8), edge(k1, 32, 128, 8)
        return (pl.ds(p0, np_), pl.ds(r0, r1 - r0), slice(None))

    def c_idx(p0, np_, k0, k1):
        return (pl.ds(p0, np_), pl.ds(k0 * 32, (k1 - k0) * 32), slice(None))

    def start2(src, dst, idx, sem, prio):
        start(src.at[idx], dst.at[idx], sem, prio)

    def start_w3(src, dst, p, k, sem, prio):
        start2(src, dst, w3_idx(p, 1, k, k + 1), sem, prio)

    def start_c(p, k, sem, prio):
        start2(c_hbm, c_v, c_idx(p, 1, k, k + 1), sem, prio)

    def issue_s0(t, j0, j1):
        sem = sems.at[t % 3]
        for j in range(j0, j1):
            k, n = t * 8 + j // 4, j % 4
            for u in range(2):
                prio = 1 if (t == 0 and j < 16) else u
                if n == 0:
                    start_w3(buk_hbm, buk_v, 2 + u, k, sem, prio)
                elif n < 3:
                    start_w3(bq_hbm, bq_v, (n - 1) * 2 + u, k, sem, prio)
                else:
                    start_c(u, k, sem, prio)

    def wait_s0(t):
        sem = sems.at[t % 3]
        wait(buk_v.at[w3_idx(2, 2, t * 8, t * 8 + 8)], sem)
        wait(bq_v.at[w3_idx(0, 4, t * 8, t * 8 + 8)], sem)
        wait(c_v.at[c_idx(0, 2, t * 8, t * 8 + 8)], sem)

    def issue_s1(t, j0, j1):
        sem = sems.at[(4 + t) % 3]
        for j in range(j0, j1):
            k, n = t * 8 + j // 4, j % 4
            for u in range(2):
                if n == 0:
                    start_w3(buv_hbm, buv_v, 2 + u, k, sem, u)
                elif n == 2:
                    start_w3(buk_hbm, buk_v, u, k, sem, u)
                else:
                    kq = k % 16
                    cols = pl.ds(0, 1920) if kq % 2 == 0 else pl.ds(1920, 2176)
                    idx = ((t // 2) * 4 + n - 1 + u, pl.ds((kq // 2) * 8, 8), cols)
                    start2(wq_hbm, wq_v, idx, sem, u)

    def wait_s1(t):
        sem = sems.at[(4 + t) % 3]
        wait(buv_v.at[w3_idx(2, 2, t * 8, t * 8 + 8)], sem)
        wait(buk_v.at[w3_idx(0, 2, t * 8, t * 8 + 8)], sem)
        wait(wq_v.at[pl.ds((t // 2) * 4, 4), pl.ds((t % 2) * 32, 32), :], sem)

    def issue_c(i, j0, j1):
        sem = sems.at[(8 + i) % 3]
        for j in range(j0, j1):
            k, n = (i % 4) * 8 + j // 4, j % 4
            for u in range(2):
                if i < 4:
                    start_c(2 + n * 2 + u, k, sem, u)
                elif n < 3:
                    start_c(10 + n * 2 + u, k, sem, u)
                else:
                    start_w3(buv_hbm, buv_v, u, k, sem, u)

    def wait_c(i):
        sem = sems.at[(8 + i) % 3]
        rows = pl.ds(pl.multiple_of((i % 4) * 256, 256), 256)
        wait(c_v.at[pl.ds(2 + (i // 4) * 8, 6), rows, :], sem)
        pl.when(i < 4)(lambda: wait(c_v.at[pl.ds(8, 2), rows, :], sem))
        for t in range(4):
            pl.when(i == 4 + t)(functools.partial(wait, buv_v.at[w3_idx(0, 2, t * 8, t * 8 + 8)], sem))

    def kv_heads(g):
        return [(((g & 1) << 5) + (g >> 1) + (d + 2)) & 127 for d in (0, 16, 64, 80)]

    def issue_kv(g, j0, j1):
        slot = (16 + g) % 3
        sem = sems.at[slot]
        fs = kv_heads(g)
        for j in range(j0, j1):
            a, n = (j // 4) % 2, j % 4
            for u in range(2):
                k = j // 8 + 4 * u
                r0, r1 = edge(k, 8, 128, -8), edge(k + 1, 8, 128, -8)
                start((k_hbm, v_hbm)[a].at[fs[n], pl.ds(SK - W + r0, r1 - r0), :],
                      kv_v.at[slot, a, n, pl.ds(r0, r1 - r0), :], sem, u)

    def wait_kv(g):
        slot = (16 + g) % 3
        wait(kv_v.at[slot], sems.at[slot])

    def o_heads(t):
        return [(p, (t ^ (p & 2)) * 256 + hb * 128) for hb in range(2) for p in (0, 2, 1, 3)]

    def o_chunks(heads):
        return [(p, pl.ds(r0 + r, 32), slice(None)) for r in range(0, 128, 32) for p, r0 in heads]

    def o_order(t, groups):
        heads = o_heads(t)
        return [(n, idx) for n, (h0, k) in enumerate(groups) for idx in o_chunks(heads[h0:h0 + k])]

    HALVES = ((0, 4), (4, 4))
    TAIL = ((0, 4), (4, 2), (6, 1), (7, 1))

    def issue_o(t):
        for (_, ia), (n, ib) in zip(o_order(t, HALVES), o_order(t, HALVES if t < 3 else TAIL)):
            start2(wo_hbm, wo_v, ia, fsems.at[2 * t], 0)
            start2(bo_hbm, bo_v, ib, fsems.at[2 * t + 1 + (n if t == 3 else 0)], 1)

    def diag_mask():
        return (_iota((64, 2048), 1) & 15) == (_iota((64, 2048), 0) & 15)

    def w3(ref, k, hf):
        return ref[k].reshape(128, 2, 16, DH)[:, hf].reshape(2048, DH)

    def build_consts():
        e_v[...] = jnp.where(_iota((128, 2048), 0) == (_iota((128, 2048), 1) >> 4), 1.0, 0.0).astype(BF16)
        et_v[...] = jnp.where(_iota((2048, 128), 1) == (_iota((2048, 128), 0) >> 4), 1.0, 0.0).astype(BF16)
        m_v[...] = jnp.full(m_v.shape, -jnp.inf, F32)
        l_v[...] = jnp.zeros(l_v.shape, F32)
        acc_v[...] = jnp.zeros(acc_v.shape, F32)
        oa_v[...] = jnp.zeros(oa_v.shape, F32)

    def build_x2():
        x = xb_v[...].astype(F32)
        xrep = jnp.concatenate(
            [jnp.broadcast_to(x[b:b + 1, :], (16, DM)) for b in range(B)], axis=0).astype(BF16)
        for k in range(4):
            xe = _dot(xrep[:, k * 128:(k + 1) * 128], e_v[...])
            x2_v[:, k * 2048:(k + 1) * 2048] = jnp.where(diag_mask(), xe, 0.0).astype(BF16)

    def qb_half(hf):
        acc = None
        for k in range(4):
            r = _dot(x2_v[:, k * 2048:(k + 1) * 2048], w3(bq_v, k, hf))
            acc = r if acc is None else acc + r
        qb_v[hf * 64:(hf + 1) * 64, :] = acc.astype(BF16)

    def qabs_piece(hf, k):
        r = _dot_nt(qb_v[hf * 64:(hf + 1) * 64, :], w3(buk_v, k, hf))
        r = jnp.where(diag_mask(), r, 0.0).astype(BF16)
        z = _dot(r, et_v[...]).astype(BF16)
        for b in range(B):
            qabs_v[b, hf * 16:(hf + 1) * 16, k * 128:(k + 1) * 128] = z[b * 16:(b + 1) * 16, :]

    def qa_proj():
        x = xa_v[...].astype(F32)
        x8 = jnp.concatenate([x, x], axis=0).astype(BF16)
        acc = None
        for k in range(4):
            r = _dot(x8[:, k * 128:(k + 1) * 128], wq_v[2 * k:2 * k + 2].reshape(128, H * DH))
            acc = r if acc is None else acc + r
        for h in range(H):
            qa_v[h] = acc[:, h * DH:(h + 1) * DH]

    def b_attn(i, u):
        rows = pl.ds(pl.multiple_of((i % 4) * 256, 256), 256)
        p0s = [(2 + (i // 4) * 8 + u * 4 + n * 2) % 16 for n in range(2)]
        bs = [p0 // 4 for p0 in p0s]
        cs = [c_v[pl.ds(p0, 2), rows, :].reshape(512, DM) for p0 in p0s]
        ss = [_dot_nt(qabs_v[b], c) * SCALE for b, c in zip(bs, cs)]
        ps, alphas = [], []
        for b, s in zip(bs, ss):
            m_old = m_v[b]
            m_new = jnp.maximum(m_old, jnp.max(s, axis=1, keepdims=True))
            alpha = jnp.exp(m_old - m_new)
            p = jnp.exp(s - m_new)
            l_v[b] = alpha * l_v[b] + jnp.sum(p, axis=1, keepdims=True)
            m_v[b] = m_new
            ps.append(p.astype(BF16))
            alphas.append(alpha)
        for b, p, c, alpha in zip(bs, ps, cs, alphas):
            acc_v[b] = alpha * acc_v[b] + _dot(p, c)

    def b_norm():
        for b in range(B):
            cn = (acc_v[b] / l_v[b]).astype(BF16)
            for hf in range(2):
                for k in range(4):
                    cn_v[hf * 4 + k, b * 16:(b + 1) * 16, :] = (
                        cn[hf * 16:(hf + 1) * 16, k * 128:(k + 1) * 128])
        ctx_v[...] = jnp.zeros(ctx_v.shape, F32)

    def ctx_piece(hf, k):
        xe = _dot(cn_v[hf * 4 + k], e_v[...])
        xe = jnp.where(diag_mask(), xe, 0.0).astype(BF16)
        ctx_v[hf] += _dot(xe, w3(buv_v, k, hf))

    def ob_build():
        ro = _iota((256, 128), 0)
        ri = _iota((256, 128), 1)
        src = ((ro >> 7) << 6) + ((ro & 7) << 4) + ((ro >> 3) & 15)
        perm = jnp.where(((ro & 7) < 4) & (ri == src), 1.0, 0.0).astype(BF16)
        ctx = ctx_v[...].reshape(128, DH).astype(BF16)
        ob_v[...] = _dot(perm, ctx).reshape(H, 8, DH)

    def a_group(g):
        slot = (16 + g) % 3
        fs = kv_heads(g)
        ss = [_dot_nt(qa_v[f & 31].astype(BF16), kv_v[slot, 0, j]) * SCALE for j, f in enumerate(fs)]
        ps = [jnp.exp(s - jnp.max(s, axis=1, keepdims=True)) for s in ss]
        ls = [jnp.sum(p, axis=1, keepdims=True) for p in ps]
        outs = [_dot(p.astype(BF16), kv_v[slot, 1, j]) / l for j, (p, l) in enumerate(zip(ps, ls))]
        for f, o in zip(fs, outs):
            oa_v[f & 31] = jnp.where(_iota((8, DH), 0) == (f >> 5), o, oa_v[f & 31])

    def o_proj(acc, o_v, w_v, sem, t, h0, n):
        heads = o_heads(t)[h0:h0 + n]
        for p, r0 in heads:
            wait(w_v.at[p, pl.ds(r0, 128), :], sem)
        for p, r0 in heads:
            acc += _dot(o_v[p * 8 + r0 // 128].astype(BF16), w_v[p, r0:r0 + 128, :])
        return acc

    issue_s0(0, 0, 2)
    start(xa_hbm, xa_v, xsem.at[0], 0)
    start(xb_hbm, xb_v, xsem.at[0], 0)
    issue_s0(0, 2, NP)
    issue_s0(1, 0, NP)

    issue_s0(2, 0, NP)
    wait_s0(0)
    wait(xa_v, xsem.at[0])
    wait(xb_v, xsem.at[0])
    build_consts()

    issue_s0(3, 0, NP)
    wait_s0(1)
    build_x2()

    issue_s1(0, 0, NP)
    wait_s0(2)

    issue_s1(1, 0, 16)
    wait_s0(3)
    qb_half(0)
    issue_s1(1, 16, NP)
    qb_half(1)

    for hf in range(2):
        issue_s1(2 + hf, 0, NP)
        wait_s1(hf)
        qabs_piece(hf, 2)
        qabs_piece(hf, 3)

    issue_c(0, 0, NP)
    wait_s1(2)

    issue_c(1, 0, 16)
    wait_s1(3)
    qabs_piece(0, 0)
    qabs_piece(0, 1)
    issue_c(1, 16, 24)
    qabs_piece(1, 0)
    qabs_piece(1, 1)
    issue_c(1, 24, NP)
    qa_proj()

    def b_body(i, carry):
        for u in range(2):
            j0, j1 = u * 16, (u + 1) * 16
            for n in range(8):
                nxt = (functools.partial(issue_c, n + 2) if n < 6 else functools.partial(issue_kv, n - 6))
                pl.when(i == n)(functools.partial(nxt, j0, j1))
            if u == 0:
                wait_c(i)
            b_attn(i, u)
        return carry

    lax.fori_loop(0, 8, b_body, 0)
    b_norm()

    def a_body(g, carry):
        pl.when(g < H - 2)(lambda: issue_kv(g + 2, 0, NP))
        pl.when(g == H - 2)(lambda: issue_o(0))
        pl.when(g == H - 1)(lambda: issue_o(1))
        wait_kv(g)
        a_group(g)
        pl.when(g < 4)(lambda: ctx_piece(0, g))
        pl.when((g >= 4) & (g < 8))(lambda: ctx_piece(1, g - 4))
        return carry

    lax.fori_loop(0, H, a_body, 0)

    acc_a = jnp.zeros((8, DM), F32)
    acc_b = jnp.zeros((8, DM), F32)
    issue_o(2)
    ob_build()
    acc_a = o_proj(acc_a, oa_v, wo_v, fsems.at[0], 0, 0, 8)
    acc_b = o_proj(acc_b, ob_v, bo_v, fsems.at[1], 0, 0, 8)
    issue_o(3)
    for t in (1, 2):
        acc_a = o_proj(acc_a, oa_v, wo_v, fsems.at[2 * t], t, 0, 8)
        acc_b = o_proj(acc_b, ob_v, bo_v, fsems.at[2 * t + 1], t, 0, 8)
    acc_a = o_proj(acc_a, oa_v, wo_v, fsems.at[6], 3, 0, 8)
    o_ref[:, 0:DM] = acc_a[0:B, :].astype(o_ref.dtype)
    for n, (h0, k) in enumerate(TAIL):
        acc_b = o_proj(acc_b, ob_v, bo_v, fsems.at[7 + n], 3, h0, k)
    o_ref[:, DM:2 * DM] = acc_b[0:B, :].astype(o_ref.dtype)


def _kernel(*refs):
    pl.run_scoped(
        functools.partial(_body, *refs),
        pltpu.SemaphoreType.DMA((3,)),
        pltpu.SemaphoreType.DMA((1,)),
        pltpu.SemaphoreType.DMA((11,)),
    )


@jax.jit
def pallas_concat_heads__sliding_block_cached__compressed_kv_cla__decode_kernel(
    A_x: jax.Array,
    A_k_cache: jax.Array,
    A_v_cache: jax.Array,
    A_wq: jax.Array,
    A_wo: jax.Array,
    B_x: jax.Array,
    B_c_kv: jax.Array,
    B_w_q: jax.Array,
    B_w_uk: jax.Array,
    B_w_uv: jax.Array,
    B_w_o: jax.Array,
):
    w3_shape = (4, 4096, DH)
    hbm = pl.BlockSpec(memory_space=pl.ANY)
    vmem = pltpu.VMEM
    out = pl.pallas_call(
        _kernel,
        out_shape=jax.ShapeDtypeStruct((B, 2 * DM), BF16),
        in_specs=[hbm] * 11,
        out_specs=pl.BlockSpec(memory_space=pltpu.VMEM),
        scratch_shapes=[
            vmem((B, DM), BF16),
            vmem((B, DM), BF16),
            vmem((3, 2, B, W, DH), BF16),
            vmem((8, 64, H * DH), BF16),
            vmem((4, 1024, DM), BF16),
            vmem((16, 1024, DM), BF16),
            vmem(w3_shape, BF16),
            vmem(w3_shape, BF16),
            vmem(w3_shape, BF16),
            vmem((4, 1024, DM), BF16),
            vmem((128, 2048), BF16),
            vmem((2048, 128), BF16),
            vmem((64, 8192), BF16),
            vmem((128, DH), BF16),
            vmem((B, H, DM), BF16),
            vmem((B, H, 1), F32),
            vmem((B, H, 1), F32),
            vmem((B, H, DM), F32),
            vmem((8, 64, 128), BF16),
            vmem((2, 64, DH), F32),
            vmem((H, 8, DH), F32),
            vmem((H, 8, DH), F32),
            vmem((H, 8, DH), F32),
        ],
        compiler_params=pltpu.CompilerParams(vmem_limit_bytes=100 * 1024 * 1024),
        name="fused_decode",
    )(
        A_x.reshape(B, DM),
        A_k_cache.reshape(B * H, SK, DH),
        A_v_cache.reshape(B * H, SK, DH),
        A_wq.reshape(8, 64, H * DH),
        A_wo.reshape(4, 1024, DM),
        B_x.reshape(B, DM),
        B_c_kv.reshape(16, 1024, DM),
        B_w_q.reshape(w3_shape),
        B_w_uk.reshape(w3_shape),
        B_w_uv.reshape(w3_shape),
        B_w_o.reshape(4, 1024, DM),
    )
    return out.reshape(B, 1, 2 * DM)
```

```python
import functools

import jax
import jax.numpy as jnp
from jax import lax
import jax.experimental.pallas as pl
import jax.experimental.pallas.tpu as pltpu

F32 = jnp.float32
BF16 = jnp.bfloat16

B = 4
H = 32
DH = 128
DM = 512
SK = 4096
W = 1024
SCALE = DH ** -0.5

NP = 32
NT = (((1,), (1,)), ((), ()))


def _iota(shape, d):
    return lax.broadcasted_iota(jnp.int32, shape, d)


def _dot(a, b):
    return jnp.dot(a, b, preferred_element_type=F32)


def _dot_nt(a, b):
    return lax.dot_general(a, b, NT, preferred_element_type=F32)


def _body(
    xa_hbm, k_hbm, v_hbm, wq_hbm, wo_hbm,
    xb_hbm, c_hbm, bq_hbm, buk_hbm, buv_hbm, bo_hbm,
    o_ref,
    xa_v, xb_v, kv_v, wq_v, wo_v, c_v, bq_v, buk_v, buv_v, bo_v,
    e_v, et_v, x2_v, qb_v, qabs_v, m_v, l_v, acc_v, cn_v, ctx_v,
    qa_v, oa_v, ob_v,
    sems, xsem, fsems,
):
    def start(src, dst, sem, prio):
        pltpu.make_async_copy(src, dst, sem).start(priority=prio)

    def wait(dst, sem):
        pltpu.make_async_copy(dst, dst, sem).wait()

    def edge(k, n, size, shift):
        return 0 if k == 0 else (n * size if k == n else k * size + shift)

    def w3_idx(p0, np_, k0, k1):
        r0, r1 = edge(k0, 32, 128, 8), edge(k1, 32, 128, 8)
        return (pl.ds(p0, np_), pl.ds(r0, r1 - r0), slice(None))

    def start2(src, dst, idx, sem, prio):
        start(src.at[idx], dst.at[idx], sem, prio)

    def start_w3(src, dst, p, k, sem, prio):
        start2(src, dst, w3_idx(p, 1, k, k + 1), sem, prio)

    def start_c(p, k, sem, prio):
        start_w3(c_hbm, c_v, p, k, sem, prio)

    def issue_s0(t, j0, j1):
        sem = sems.at[t % 3]
        for j in range(j0, j1):
            k, n = t * 8 + j // 4, j % 4
            for u in range(2):
                prio = 1 if (t == 0 and j < 16) else u
                if n == 0:
                    start_w3(buk_hbm, buk_v, 2 + u, k, sem, prio)
                elif n < 3:
                    start_w3(bq_hbm, bq_v, (n - 1) * 2 + u, k, sem, prio)
                else:
                    start_c(u, k, sem, prio)

    def wait_s0(t):
        sem = sems.at[t % 3]
        wait(buk_v.at[w3_idx(2, 2, t * 8, t * 8 + 8)], sem)
        wait(bq_v.at[w3_idx(0, 4, t * 8, t * 8 + 8)], sem)
        wait(c_v.at[w3_idx(0, 2, t * 8, t * 8 + 8)], sem)

    def issue_s1(t, j0, j1):
        sem = sems.at[(4 + t) % 3]
        for j in range(j0, j1):
            k, n = t * 8 + j // 4, j % 4
            for u in range(2):
                if n == 0:
                    start_w3(buv_hbm, buv_v, 2 + u, k, sem, u)
                elif n == 2:
                    start_w3(buk_hbm, buk_v, u, k, sem, u)
                else:
                    kq = k % 16
                    cols = pl.ds(0, 1920) if kq % 2 == 0 else pl.ds(1920, 2176)
                    idx = ((t // 2) * 4 + n - 1 + u, pl.ds((kq // 2) * 8, 8), cols)
                    start2(wq_hbm, wq_v, idx, sem, u)

    def wait_s1(t):
        sem = sems.at[(4 + t) % 3]
        wait(buv_v.at[w3_idx(2, 2, t * 8, t * 8 + 8)], sem)
        wait(buk_v.at[w3_idx(0, 2, t * 8, t * 8 + 8)], sem)
        wait(wq_v.at[pl.ds((t // 2) * 4, 4), pl.ds((t % 2) * 32, 32), :], sem)

    def issue_c(i, j0, j1):
        sem = sems.at[(8 + i) % 3]
        for j in range(j0, j1):
            k, n = (i % 4) * 8 + j // 4, j % 4
            for u in range(2):
                if i < 4:
                    start_c(2 + n * 2 + u, k, sem, u)
                elif n < 3:
                    start_c(10 + n * 2 + u, k, sem, u)
                else:
                    start_w3(buv_hbm, buv_v, u, k, sem, u)

    def wait_c(i):
        sem = sems.at[(8 + i) % 3]
        k0 = (i % 4) * 8
        if i < 4:
            wait(c_v.at[w3_idx(2, 8, k0, k0 + 8)], sem)
        else:
            wait(c_v.at[w3_idx(10, 6, k0, k0 + 8)], sem)
            wait(buv_v.at[w3_idx(0, 2, k0, k0 + 8)], sem)

    def kv_heads(g):
        return [(((g & 1) << 5) + (g >> 1) + (d + 2)) & 127 for d in (0, 16, 64, 80)]

    def issue_kv(g, j0, j1):
        slot = (16 + g) % 3
        sem = sems.at[slot]
        fs = kv_heads(g)
        for j in range(j0, j1):
            a, n = (j // 4) % 2, j % 4
            for u in range(2):
                k = j // 8 + 4 * u
                r0, r1 = edge(k, 8, 128, -8), edge(k + 1, 8, 128, -8)
                start((k_hbm, v_hbm)[a].at[fs[n], pl.ds(SK - W + r0, r1 - r0), :],
                      kv_v.at[slot, a, n, pl.ds(r0, r1 - r0), :], sem, u)

    def wait_kv(g):
        slot = (16 + g) % 3
        wait(kv_v.at[slot], sems.at[slot])

    def o_heads(t):
        return [(p, (t ^ (p & 2)) * 2 + hb) for hb in range(2) for p in (0, 2, 1, 3)]

    def o_rows(p, h, k0, k1, shift):
        k0, k1 = k0 + (h % 2) * 4, k1 + (h % 2) * 4
        r0, r1 = edge(k0, 8, 128, shift), edge(k1, 8, 128, shift)
        return (p, pl.ds((h // 2) * 1024 + r0, r1 - r0), slice(None))

    def o_order(t, groups, shift):
        heads = o_heads(t)
        return [(n, o_rows(p, h, k, k + 1, shift))
                for n, (h0, nh) in enumerate(groups) for k in range(4) for p, h in heads[h0:h0 + nh]]

    HALVES = ((0, 4), (4, 4))
    TAIL = ((0, 4), (4, 2), (6, 1), (7, 1))

    def issue_o(t):
        for (_, ia), (n, ib) in zip(o_order(t, HALVES, -8), o_order(t, HALVES if t < 3 else TAIL, 8)):
            start2(wo_hbm, wo_v, ia, fsems.at[2 * t], 0)
            start2(bo_hbm, bo_v, ib, fsems.at[2 * t + 1 + (n if t == 3 else 0)], 1)

    def diag_mask():
        return (_iota((64, 2048), 1) & 15) == (_iota((64, 2048), 0) & 15)

    def w3(ref, k, hf):
        return ref[k].reshape(128, 2, 16, DH)[:, hf].reshape(2048, DH)

    def untile(v):
        n = v.size // DM
        v = v.reshape(n // 8, 4, 8, 128)
        return jnp.concatenate([v[:, k].reshape(n, 128) for k in range(4)], axis=1)

    def build_consts():
        e_v[...] = jnp.where(_iota((128, 2048), 0) == (_iota((128, 2048), 1) >> 4), 1.0, 0.0).astype(BF16)
        et_v[...] = jnp.where(_iota((2048, 128), 1) == (_iota((2048, 128), 0) >> 4), 1.0, 0.0).astype(BF16)
        m_v[...] = jnp.full(m_v.shape, -jnp.inf, F32)
        l_v[...] = jnp.zeros(l_v.shape, F32)
        acc_v[...] = jnp.zeros(acc_v.shape, F32)
        oa_v[...] = jnp.zeros(oa_v.shape, F32)

    def build_x2():
        x = xb_v[...].astype(F32)
        xrep = jnp.concatenate(
            [jnp.broadcast_to(x[b:b + 1, :], (16, DM)) for b in range(B)], axis=0).astype(BF16)
        for k in range(4):
            xe = _dot(xrep[:, k * 128:(k + 1) * 128], e_v[...])
            x2_v[:, k * 2048:(k + 1) * 2048] = jnp.where(diag_mask(), xe, 0.0).astype(BF16)

    def qb_half(hf):
        acc = None
        for k in range(4):
            r = _dot(x2_v[:, k * 2048:(k + 1) * 2048], w3(bq_v, k, hf))
            acc = r if acc is None else acc + r
        qb_v[hf * 64:(hf + 1) * 64, :] = acc.astype(BF16)

    def qabs_piece(hf, k):
        r = _dot_nt(qb_v[hf * 64:(hf + 1) * 64, :], w3(buk_v, k, hf))
        r = jnp.where(diag_mask(), r, 0.0).astype(BF16)
        z = _dot(r, et_v[...]).astype(BF16)
        for b in range(B):
            qabs_v[b, hf * 16:(hf + 1) * 16, k * 128:(k + 1) * 128] = z[b * 16:(b + 1) * 16, :]

    def qa_proj():
        x = xa_v[...].astype(F32)
        x8 = jnp.concatenate([x, x], axis=0).astype(BF16)
        acc = None
        for k in range(4):
            r = _dot(x8[:, k * 128:(k + 1) * 128], wq_v[2 * k:2 * k + 2].reshape(128, H * DH))
            acc = r if acc is None else acc + r
        for h in range(H):
            qa_v[h] = acc[:, h * DH:(h + 1) * DH]

    def b_attn(i, u):
        rows = pl.ds(pl.multiple_of((i % 4) * 1024, 1024), 1024)
        p0s = [(2 + (i // 4) * 8 + u * 4 + n * 2) % 16 for n in range(2)]
        bs = [p0 // 4 for p0 in p0s]
        cs = [untile(c_v[pl.ds(p0, 2), rows, :]) for p0 in p0s]
        ss = [_dot_nt(qabs_v[b], c) * SCALE for b, c in zip(bs, cs)]
        ps, alphas = [], []
        for b, s in zip(bs, ss):
            m_old = m_v[b]
            m_new = jnp.maximum(m_old, jnp.max(s, axis=1, keepdims=True))
            alpha = jnp.exp(m_old - m_new)
            p = jnp.exp(s - m_new)
            l_v[b] = alpha * l_v[b] + jnp.sum(p, axis=1, keepdims=True)
            m_v[b] = m_new
            ps.append(p.astype(BF16))
            alphas.append(alpha)
        for b, p, c, alpha in zip(bs, ps, cs, alphas):
            acc_v[b] = alpha * acc_v[b] + _dot(p, c)

    def b_norm():
        for b in range(B):
            cn = (acc_v[b] / l_v[b]).astype(BF16)
            for hf in range(2):
                for k in range(4):
                    cn_v[hf * 4 + k, b * 16:(b + 1) * 16, :] = (
                        cn[hf * 16:(hf + 1) * 16, k * 128:(k + 1) * 128])
        ctx_v[...] = jnp.zeros(ctx_v.shape, F32)

    def ctx_piece(hf, k):
        xe = _dot(cn_v[hf * 4 + k], e_v[...])
        xe = jnp.where(diag_mask(), xe, 0.0).astype(BF16)
        ctx_v[hf] += _dot(xe, w3(buv_v, k, hf))

    def ob_build():
        ro = _iota((256, 128), 0)
        ri = _iota((256, 128), 1)
        src = ((ro >> 7) << 6) + ((ro & 7) << 4) + ((ro >> 3) & 15)
        perm = jnp.where(((ro & 7) < 4) & (ri == src), 1.0, 0.0).astype(BF16)
        ctx = ctx_v[...].reshape(128, DH).astype(BF16)
        ob_v[...] = _dot(perm, ctx).reshape(H, 8, DH)

    def a_group(g):
        slot = (16 + g) % 3
        fs = kv_heads(g)
        ss = [_dot_nt(qa_v[f & 31].astype(BF16), kv_v[slot, 0, j]) * SCALE for j, f in enumerate(fs)]
        ps = [jnp.exp(s - jnp.max(s, axis=1, keepdims=True)) for s in ss]
        ls = [jnp.sum(p, axis=1, keepdims=True) for p in ps]
        outs = [_dot(p.astype(BF16), kv_v[slot, 1, j]) / l for j, (p, l) in enumerate(zip(ps, ls))]
        for f, o in zip(fs, outs):
            oa_v[f & 31] = jnp.where(_iota((8, DH), 0) == (f >> 5), o, oa_v[f & 31])

    def o_proj(acc, o_v, w_v, shift, sem, t, h0, n):
        heads = o_heads(t)[h0:h0 + n]
        for p, h in heads:
            wait(w_v.at[o_rows(p, h, 0, 4, shift)], sem)
        for p, h in heads:
            acc += _dot(o_v[p * 8 + h].astype(BF16), untile(w_v[p, h * 512:(h + 1) * 512, :]))
        return acc

    issue_s0(0, 0, 2)
    start(xa_hbm, xa_v, xsem.at[0], 0)
    start(xb_hbm, xb_v, xsem.at[0], 0)
    issue_s0(0, 2, NP)
    issue_s0(1, 0, NP)

    issue_s0(2, 0, NP)
    wait_s0(0)
    wait(xa_v, xsem.at[0])
    wait(xb_v, xsem.at[0])
    build_consts()

    issue_s0(3, 0, NP)
    wait_s0(1)
    build_x2()

    issue_s1(0, 0, NP)
    wait_s0(2)

    issue_s1(1, 0, 16)
    wait_s0(3)
    qb_half(0)
    issue_s1(1, 16, NP)
    qb_half(1)

    for hf in range(2):
        issue_s1(2 + hf, 0, NP)
        wait_s1(hf)
        qabs_piece(hf, 2)
        qabs_piece(hf, 3)

    issue_c(0, 0, NP)
    wait_s1(2)

    issue_c(1, 0, 16)
    wait_s1(3)
    qabs_piece(0, 0)
    qabs_piece(0, 1)
    issue_c(1, 16, 24)
    qabs_piece(1, 0)
    qabs_piece(1, 1)
    issue_c(1, 24, NP)
    qa_proj()

    def b_body(i, carry):
        for u in range(2):
            j0, j1 = u * 16, (u + 1) * 16
            for n in range(8):
                nxt = (functools.partial(issue_c, n + 2) if n < 6 else functools.partial(issue_kv, n - 6))
                pl.when(i == n)(functools.partial(nxt, j0, j1))
            if u == 0:
                for n in range(8):
                    pl.when(i == n)(functools.partial(wait_c, n))
            b_attn(i, u)
        return carry

    lax.fori_loop(0, 8, b_body, 0)
    b_norm()

    def a_body(g, carry):
        pl.when(g < H - 2)(lambda: issue_kv(g + 2, 0, NP))
        pl.when(g == H - 2)(lambda: issue_o(0))
        pl.when(g == H - 1)(lambda: issue_o(1))
        wait_kv(g)
        a_group(g)
        pl.when(g < 4)(lambda: ctx_piece(0, g))
        pl.when((g >= 4) & (g < 8))(lambda: ctx_piece(1, g - 4))
        return carry

    lax.fori_loop(0, H, a_body, 0)

    acc_a = jnp.zeros((8, DM), F32)
    acc_b = jnp.zeros((8, DM), F32)
    issue_o(2)
    ob_build()
    acc_a = o_proj(acc_a, oa_v, wo_v, -8, fsems.at[0], 0, 0, 8)
    acc_b = o_proj(acc_b, ob_v, bo_v, 8, fsems.at[1], 0, 0, 8)
    issue_o(3)
    for t in (1, 2):
        acc_a = o_proj(acc_a, oa_v, wo_v, -8, fsems.at[2 * t], t, 0, 8)
        acc_b = o_proj(acc_b, ob_v, bo_v, 8, fsems.at[2 * t + 1], t, 0, 8)
    acc_a = o_proj(acc_a, oa_v, wo_v, -8, fsems.at[6], 3, 0, 8)
    o_ref[:, 0:DM] = acc_a[0:B, :].astype(o_ref.dtype)
    for n, (h0, k) in enumerate(TAIL):
        acc_b = o_proj(acc_b, ob_v, bo_v, 8, fsems.at[7 + n], 3, h0, k)
    o_ref[:, DM:2 * DM] = acc_b[0:B, :].astype(o_ref.dtype)


def _kernel(*refs):
    pl.run_scoped(
        functools.partial(_body, *refs),
        pltpu.SemaphoreType.DMA((3,)),
        pltpu.SemaphoreType.DMA((1,)),
        pltpu.SemaphoreType.DMA((11,)),
    )


@jax.jit
def pallas_concat_heads__sliding_block_cached__compressed_kv_cla__decode_kernel(
    A_x: jax.Array,
    A_k_cache: jax.Array,
    A_v_cache: jax.Array,
    A_wq: jax.Array,
    A_wo: jax.Array,
    B_x: jax.Array,
    B_c_kv: jax.Array,
    B_w_q: jax.Array,
    B_w_uk: jax.Array,
    B_w_uv: jax.Array,
    B_w_o: jax.Array,
):
    w3_shape = (4, 4096, DH)

    def tile_rows(a):
        return a.reshape(-1, 8, 4, 128).transpose(0, 2, 1, 3).reshape(-1, 4096, 128)

    hbm = pl.BlockSpec(memory_space=pl.ANY)
    vmem = pltpu.VMEM
    out = pl.pallas_call(
        _kernel,
        out_shape=jax.ShapeDtypeStruct((B, 2 * DM), BF16),
        in_specs=[hbm] * 11,
        out_specs=pl.BlockSpec(memory_space=pltpu.VMEM),
        scratch_shapes=[
            vmem((B, DM), BF16),
            vmem((B, DM), BF16),
            vmem((3, 2, B, W, DH), BF16),
            vmem((8, 64, H * DH), BF16),
            vmem(w3_shape, BF16),
            vmem((16, 4096, DH), BF16),
            vmem(w3_shape, BF16),
            vmem(w3_shape, BF16),
            vmem(w3_shape, BF16),
            vmem(w3_shape, BF16),
            vmem((128, 2048), BF16),
            vmem((2048, 128), BF16),
            vmem((64, 8192), BF16),
            vmem((128, DH), BF16),
            vmem((B, H, DM), BF16),
            vmem((B, H, 1), F32),
            vmem((B, H, 1), F32),
            vmem((B, H, DM), F32),
            vmem((8, 64, 128), BF16),
            vmem((2, 64, DH), F32),
            vmem((H, 8, DH), F32),
            vmem((H, 8, DH), F32),
            vmem((H, 8, DH), F32),
        ],
        compiler_params=pltpu.CompilerParams(vmem_limit_bytes=100 * 1024 * 1024),
        name="fused_decode",
    )(
        A_x.reshape(B, DM),
        A_k_cache.reshape(B * H, SK, DH),
        A_v_cache.reshape(B * H, SK, DH),
        A_wq.reshape(8, 64, H * DH),
        tile_rows(A_wo),
        B_x.reshape(B, DM),
        tile_rows(B_c_kv),
        B_w_q.reshape(w3_shape),
        B_w_uk.reshape(w3_shape),
        B_w_uv.reshape(w3_shape),
        tile_rows(B_w_o),
    )
    return out.reshape(B, 1, 2 * DM)
```

```python
import functools

import jax
import jax.numpy as jnp
from jax import lax
import jax.experimental.pallas as pl
import jax.experimental.pallas.tpu as pltpu

F32 = jnp.float32
BF16 = jnp.bfloat16

B = 4
H = 32
DH = 128
DM = 512
SK = 4096
W = 1024
SCALE = DH ** -0.5

NP = 32
NT = (((1,), (1,)), ((), ()))


def _iota(shape, d):
    return lax.broadcasted_iota(jnp.int32, shape, d)


def _dot(a, b):
    return jnp.dot(a, b, preferred_element_type=F32)


def _dot_nt(a, b):
    return lax.dot_general(a, b, NT, preferred_element_type=F32)


def _body(
    xa_hbm, k_hbm, v_hbm, wq_hbm, wo_hbm,
    xb_hbm, c_hbm, bq_hbm, buk_hbm, buv_hbm, bo_hbm,
    o_ref,
    xa_v, xb_v, kv_v, wq_v, wo_v, c_v, bq_v, buk_v, buv_v, bo_v,
    e_v, et_v, x2_v, qb_v, qabs_v, m_v, l_v, acc_v, cn_v, ctx_v,
    qa_v, oa_v, ob_v,
    sems, xsem, fsems,
):
    def start(src, dst, sem, prio):
        pltpu.make_async_copy(src, dst, sem).start(priority=prio)

    def wait(dst, sem):
        pltpu.make_async_copy(dst, dst, sem).wait()

    def edge(k, n, size, shift):
        return 0 if k == 0 else (n * size if k == n else k * size + shift)

    def w3_idx(p0, np_, k0, k1):
        r0, r1 = edge(k0, 32, 128, 8), edge(k1, 32, 128, 8)
        return (pl.ds(p0, np_), pl.ds(r0, r1 - r0), slice(None))

    def start2(src, dst, idx, sem, prio):
        start(src.at[idx], dst.at[idx], sem, prio)

    def start_w3(src, dst, p, k, sem, prio):
        start2(src, dst, w3_idx(p, 1, k, k + 1), sem, prio)

    def start_c(p, k, sem, prio):
        start_w3(c_hbm, c_v, p, k, sem, prio)

    def issue_s0(t, j0, j1):
        sem = sems.at[t % 3]
        for j in range(j0, j1):
            k, n = t * 8 + j // 4, j % 4
            for u in range(2):
                prio = 1 if (t == 0 and j < 16) else u
                if n == 0:
                    start_w3(buk_hbm, buk_v, 2 + u, k, sem, prio)
                elif n < 3:
                    start_w3(bq_hbm, bq_v, (n - 1) * 2 + u, k, sem, prio)
                else:
                    start_c(u, k, sem, prio)

    def wait_s0(t):
        sem = sems.at[t % 3]
        wait(buk_v.at[w3_idx(2, 2, t * 8, t * 8 + 8)], sem)
        wait(bq_v.at[w3_idx(0, 4, t * 8, t * 8 + 8)], sem)
        wait(c_v.at[w3_idx(0, 2, t * 8, t * 8 + 8)], sem)

    def wq_idx(t, p0, np_, k0, k1):
        r0, r1 = (edge((t % 2) * 8 + k, 16, 128, -8) for k in (k0, k1))
        return (pl.ds((t // 2) * 4 + p0, np_), pl.ds(r0, r1 - r0), slice(None))

    def issue_s1(t, j0, j1):
        sem = sems.at[(4 + t) % 3]
        for j in range(j0, j1):
            k, n = t * 8 + j // 4, j % 4
            for u in range(2):
                if n == 0:
                    start_w3(buv_hbm, buv_v, 2 + u, k, sem, u)
                elif n == 2:
                    start_w3(buk_hbm, buk_v, u, k, sem, u)
                else:
                    start2(wq_hbm, wq_v, wq_idx(t, n - 1 + u, 1, j // 4, j // 4 + 1), sem, u)

    def wait_s1(t):
        sem = sems.at[(4 + t) % 3]
        wait(buv_v.at[w3_idx(2, 2, t * 8, t * 8 + 8)], sem)
        wait(buk_v.at[w3_idx(0, 2, t * 8, t * 8 + 8)], sem)
        wait(wq_v.at[wq_idx(t, 0, 4, 0, 8)], sem)

    def issue_c(i, j0, j1):
        sem = sems.at[(8 + i) % 3]
        for j in range(j0, j1):
            k, n = (i % 4) * 8 + j // 4, j % 4
            for u in range(2):
                if i < 4:
                    start_c(2 + n * 2 + u, k, sem, u)
                elif n < 3:
                    start_c(10 + n * 2 + u, k, sem, u)
                else:
                    start_w3(buv_hbm, buv_v, u, k, sem, u)

    def wait_c(i):
        sem = sems.at[(8 + i) % 3]
        k0 = (i % 4) * 8
        if i < 4:
            wait(c_v.at[w3_idx(2, 8, k0, k0 + 8)], sem)
        else:
            wait(c_v.at[w3_idx(10, 6, k0, k0 + 8)], sem)
            wait(buv_v.at[w3_idx(0, 2, k0, k0 + 8)], sem)

    def kv_heads(g):
        return [(((g & 1) << 5) + (g >> 1) + (d + 2)) & 127 for d in (0, 16, 64, 80)]

    def issue_kv(g, j0, j1):
        slot = (16 + g) % 3
        sem = sems.at[slot]
        fs = kv_heads(g)
        for j in range(j0, j1):
            a, n = (j // 4) % 2, j % 4
            for u in range(2):
                k = j // 8 + 4 * u
                r0, r1 = edge(k, 8, 128, -8), edge(k + 1, 8, 128, -8)
                start((k_hbm, v_hbm)[a].at[fs[n], pl.ds(SK - W + r0, r1 - r0), :],
                      kv_v.at[slot, a, n, pl.ds(r0, r1 - r0), :], sem, u)

    def wait_kv(g):
        slot = (16 + g) % 3
        wait(kv_v.at[slot], sems.at[slot])

    def o_heads(t):
        return [(p, (t ^ (p & 2)) * 2 + hb) for hb in range(2) for p in (0, 2, 1, 3)]

    def o_rows(p, h, k0, k1, shift):
        k0, k1 = k0 + (h % 2) * 4, k1 + (h % 2) * 4
        r0, r1 = edge(k0, 8, 128, shift), edge(k1, 8, 128, shift)
        return (p, pl.ds((h // 2) * 1024 + r0, r1 - r0), slice(None))

    def o_order(t, groups, shift):
        heads = o_heads(t)
        return [(n, o_rows(p, h, k, k + 1, shift))
                for n, (h0, nh) in enumerate(groups) for k in range(4) for p, h in heads[h0:h0 + nh]]

    HALVES = ((0, 4), (4, 4))
    TAIL = ((0, 4), (4, 2), (6, 1), (7, 1))

    def issue_o(t):
        for (_, ia), (n, ib) in zip(o_order(t, HALVES, -8), o_order(t, HALVES if t < 3 else TAIL, 8)):
            start2(wo_hbm, wo_v, ia, fsems.at[2 * t], 0)
            start2(bo_hbm, bo_v, ib, fsems.at[2 * t + 1 + (n if t == 3 else 0)], 1)

    def diag_mask():
        return (_iota((64, 2048), 1) & 15) == (_iota((64, 2048), 0) & 15)

    def w3(ref, k, hf):
        return ref[k].reshape(128, 2, 16, DH)[:, hf].reshape(2048, DH)

    def untile(v, nt=4):
        n = v.size // (128 * nt)
        v = v.reshape(n // 8, nt, 8, 128)
        return jnp.concatenate([v[:, k].reshape(n, 128) for k in range(nt)], axis=1)

    def build_consts():
        e_v[...] = jnp.where(_iota((128, 2048), 0) == (_iota((128, 2048), 1) >> 4), 1.0, 0.0).astype(BF16)
        et_v[...] = jnp.where(_iota((2048, 128), 1) == (_iota((2048, 128), 0) >> 4), 1.0, 0.0).astype(BF16)
        m_v[...] = jnp.full(m_v.shape, -jnp.inf, F32)
        l_v[...] = jnp.zeros(l_v.shape, F32)
        acc_v[...] = jnp.zeros(acc_v.shape, F32)
        oa_v[...] = jnp.zeros(oa_v.shape, F32)

    def build_x2():
        x = xb_v[...].astype(F32)
        xrep = jnp.concatenate(
            [jnp.broadcast_to(x[b:b + 1, :], (16, DM)) for b in range(B)], axis=0).astype(BF16)
        for k in range(4):
            xe = _dot(xrep[:, k * 128:(k + 1) * 128], e_v[...])
            x2_v[:, k * 2048:(k + 1) * 2048] = jnp.where(diag_mask(), xe, 0.0).astype(BF16)

    def qb_half(hf):
        acc = None
        for k in range(4):
            r = _dot(x2_v[:, k * 2048:(k + 1) * 2048], w3(bq_v, k, hf))
            acc = r if acc is None else acc + r
        qb_v[hf * 64:(hf + 1) * 64, :] = acc.astype(BF16)

    def qabs_piece(hf, k):
        r = _dot_nt(qb_v[hf * 64:(hf + 1) * 64, :], w3(buk_v, k, hf))
        r = jnp.where(diag_mask(), r, 0.0).astype(BF16)
        z = _dot(r, et_v[...]).astype(BF16)
        for b in range(B):
            qabs_v[b, hf * 16:(hf + 1) * 16, k * 128:(k + 1) * 128] = z[b * 16:(b + 1) * 16, :]

    def qa_proj():
        x = xa_v[...].astype(F32)
        x8 = jnp.concatenate([x, x], axis=0).astype(BF16)
        acc = None
        for k in range(4):
            r = _dot(x8[:, k * 128:(k + 1) * 128], untile(wq_v[2 * k:2 * k + 2], H))
            acc = r if acc is None else acc + r
        for h in range(H):
            qa_v[h] = acc[:, h * DH:(h + 1) * DH]

    def b_attn(i, u):
        rows = pl.ds(pl.multiple_of((i % 4) * 1024, 1024), 1024)
        p0s = [(2 + (i // 4) * 8 + u * 4 + n * 2) % 16 for n in range(2)]
        bs = [p0 // 4 for p0 in p0s]
        cs = [untile(c_v[pl.ds(p0, 2), rows, :]) for p0 in p0s]
        ss = [_dot_nt(qabs_v[b], c) * SCALE for b, c in zip(bs, cs)]
        ps, alphas = [], []
        for b, s in zip(bs, ss):
            m_old = m_v[b]
            m_new = jnp.maximum(m_old, jnp.max(s, axis=1, keepdims=True))
            alpha = jnp.exp(m_old - m_new)
            p = jnp.exp(s - m_new)
            l_v[b] = alpha * l_v[b] + jnp.sum(p, axis=1, keepdims=True)
            m_v[b] = m_new
            ps.append(p.astype(BF16))
            alphas.append(alpha)
        for b, p, c, alpha in zip(bs, ps, cs, alphas):
            acc_v[b] = alpha * acc_v[b] + _dot(p, c)

    def b_norm():
        for b in range(B):
            cn = (acc_v[b] / l_v[b]).astype(BF16)
            for hf in range(2):
                for k in range(4):
                    cn_v[hf * 4 + k, b * 16:(b + 1) * 16, :] = (
                        cn[hf * 16:(hf + 1) * 16, k * 128:(k + 1) * 128])
        ctx_v[...] = jnp.zeros(ctx_v.shape, F32)

    def ctx_piece(hf, k):
        xe = _dot(cn_v[hf * 4 + k], e_v[...])
        xe = jnp.where(diag_mask(), xe, 0.0).astype(BF16)
        ctx_v[hf] += _dot(xe, w3(buv_v, k, hf))

    def ob_build():
        ro = _iota((256, 128), 0)
        ri = _iota((256, 128), 1)
        src = ((ro >> 7) << 6) + ((ro & 7) << 4) + ((ro >> 3) & 15)
        perm = jnp.where(((ro & 7) < 4) & (ri == src), 1.0, 0.0).astype(BF16)
        ctx = ctx_v[...].reshape(128, DH).astype(BF16)
        ob_v[...] = _dot(perm, ctx).reshape(H, 8, DH)

    def a_group(g):
        slot = (16 + g) % 3
        fs = kv_heads(g)
        ss = [_dot_nt(qa_v[f & 31].astype(BF16), kv_v[slot, 0, j]) * SCALE for j, f in enumerate(fs)]
        ps = [jnp.exp(s - jnp.max(s, axis=1, keepdims=True)) for s in ss]
        ls = [jnp.sum(p, axis=1, keepdims=True) for p in ps]
        outs = [_dot(p.astype(BF16), kv_v[slot, 1, j]) / l for j, (p, l) in enumerate(zip(ps, ls))]
        for f, o in zip(fs, outs):
            oa_v[f & 31] = jnp.where(_iota((8, DH), 0) == (f >> 5), o, oa_v[f & 31])

    def o_proj(acc, o_v, w_v, shift, sem, t, h0, n):
        heads = o_heads(t)[h0:h0 + n]
        for p, h in heads:
            wait(w_v.at[o_rows(p, h, 0, 4, shift)], sem)
        for p, h in heads:
            acc += _dot(o_v[p * 8 + h].astype(BF16), untile(w_v[p, h * 512:(h + 1) * 512, :]))
        return acc

    issue_s0(0, 0, 2)
    start(xa_hbm, xa_v, xsem.at[0], 0)
    start(xb_hbm, xb_v, xsem.at[0], 0)
    issue_s0(0, 2, NP)
    issue_s0(1, 0, NP)

    issue_s0(2, 0, NP)
    wait_s0(0)
    wait(xa_v, xsem.at[0])
    wait(xb_v, xsem.at[0])
    build_consts()

    issue_s0(3, 0, NP)
    wait_s0(1)
    build_x2()

    issue_s1(0, 0, NP)
    wait_s0(2)

    issue_s1(1, 0, 16)
    wait_s0(3)
    qb_half(0)
    issue_s1(1, 16, NP)
    qb_half(1)

    for hf in range(2):
        issue_s1(2 + hf, 0, NP)
        wait_s1(hf)
        qabs_piece(hf, 2)
        qabs_piece(hf, 3)

    issue_c(0, 0, NP)
    wait_s1(2)

    issue_c(1, 0, 16)
    wait_s1(3)
    qabs_piece(0, 0)
    qabs_piece(0, 1)
    issue_c(1, 16, 24)
    qabs_piece(1, 0)
    qabs_piece(1, 1)
    issue_c(1, 24, NP)
    qa_proj()

    def b_body(i, carry):
        for u in range(2):
            j0, j1 = u * 16, (u + 1) * 16
            for n in range(8):
                nxt = (functools.partial(issue_c, n + 2) if n < 6 else functools.partial(issue_kv, n - 6))
                pl.when(i == n)(functools.partial(nxt, j0, j1))
            if u == 0:
                for n in range(8):
                    pl.when(i == n)(functools.partial(wait_c, n))
            b_attn(i, u)
        return carry

    lax.fori_loop(0, 8, b_body, 0)
    b_norm()

    def a_body(g, carry):
        pl.when(g < H - 2)(lambda: issue_kv(g + 2, 0, NP))
        pl.when(g == H - 2)(lambda: issue_o(0))
        pl.when(g == H - 1)(lambda: issue_o(1))
        wait_kv(g)
        a_group(g)
        pl.when(g < 4)(lambda: ctx_piece(0, g))
        pl.when((g >= 4) & (g < 8))(lambda: ctx_piece(1, g - 4))
        return carry

    lax.fori_loop(0, H, a_body, 0)

    acc_a = jnp.zeros((8, DM), F32)
    acc_b = jnp.zeros((8, DM), F32)
    issue_o(2)
    ob_build()
    acc_a = o_proj(acc_a, oa_v, wo_v, -8, fsems.at[0], 0, 0, 8)
    acc_b = o_proj(acc_b, ob_v, bo_v, 8, fsems.at[1], 0, 0, 8)
    issue_o(3)
    for t in (1, 2):
        acc_a = o_proj(acc_a, oa_v, wo_v, -8, fsems.at[2 * t], t, 0, 8)
        acc_b = o_proj(acc_b, ob_v, bo_v, 8, fsems.at[2 * t + 1], t, 0, 8)
    acc_a = o_proj(acc_a, oa_v, wo_v, -8, fsems.at[6], 3, 0, 8)
    o_ref[:, 0:DM] = acc_a[0:B, :].astype(o_ref.dtype)
    for n, (h0, k) in enumerate(TAIL):
        acc_b = o_proj(acc_b, ob_v, bo_v, 8, fsems.at[7 + n], 3, h0, k)
    o_ref[:, DM:2 * DM] = acc_b[0:B, :].astype(o_ref.dtype)


def _kernel(*refs):
    pl.run_scoped(
        functools.partial(_body, *refs),
        pltpu.SemaphoreType.DMA((3,)),
        pltpu.SemaphoreType.DMA((1,)),
        pltpu.SemaphoreType.DMA((11,)),
    )


@jax.jit
def pallas_concat_heads__sliding_block_cached__compressed_kv_cla__decode_kernel(
    A_x: jax.Array,
    A_k_cache: jax.Array,
    A_v_cache: jax.Array,
    A_wq: jax.Array,
    A_wo: jax.Array,
    B_x: jax.Array,
    B_c_kv: jax.Array,
    B_w_q: jax.Array,
    B_w_uk: jax.Array,
    B_w_uv: jax.Array,
    B_w_o: jax.Array,
):
    w3_shape = (4, 4096, DH)

    def tile_rows(a, rows=4096):
        return a.reshape(-1, 8, a.shape[-1] // 128, 128).transpose(0, 2, 1, 3).reshape(-1, rows, 128)

    hbm = pl.BlockSpec(memory_space=pl.ANY)
    vmem = pltpu.VMEM
    out = pl.pallas_call(
        _kernel,
        out_shape=jax.ShapeDtypeStruct((B, 2 * DM), BF16),
        in_specs=[hbm] * 11,
        out_specs=pl.BlockSpec(memory_space=pltpu.VMEM),
        scratch_shapes=[
            vmem((B, DM), BF16),
            vmem((B, DM), BF16),
            vmem((3, 2, B, W, DH), BF16),
            vmem((8, 2048, DH), BF16),
            vmem(w3_shape, BF16),
            vmem((16, 4096, DH), BF16),
            vmem(w3_shape, BF16),
            vmem(w3_shape, BF16),
            vmem(w3_shape, BF16),
            vmem(w3_shape, BF16),
            vmem((128, 2048), BF16),
            vmem((2048, 128), BF16),
            vmem((64, 8192), BF16),
            vmem((128, DH), BF16),
            vmem((B, H, DM), BF16),
            vmem((B, H, 1), F32),
            vmem((B, H, 1), F32),
            vmem((B, H, DM), F32),
            vmem((8, 64, 128), BF16),
            vmem((2, 64, DH), F32),
            vmem((H, 8, DH), F32),
            vmem((H, 8, DH), F32),
            vmem((H, 8, DH), F32),
        ],
        compiler_params=pltpu.CompilerParams(vmem_limit_bytes=100 * 1024 * 1024),
        name="fused_decode",
    )(
        A_x.reshape(B, DM),
        A_k_cache.reshape(B * H, SK, DH),
        A_v_cache.reshape(B * H, SK, DH),
        tile_rows(A_wq, 2048),
        tile_rows(A_wo),
        B_x.reshape(B, DM),
        tile_rows(B_c_kv),
        B_w_q.reshape(w3_shape),
        B_w_uk.reshape(w3_shape),
        B_w_uv.reshape(w3_shape),
        tile_rows(B_w_o),
    )
    return out.reshape(B, 1, 2 * DM)
```

```python
import functools

import jax
import jax.numpy as jnp
from jax import lax
import jax.experimental.pallas as pl
import jax.experimental.pallas.tpu as pltpu

F32 = jnp.float32
BF16 = jnp.bfloat16

B = 4
H = 32
DH = 128
DM = 512
SK = 4096
W = 1024
SCALE = DH ** -0.5

NP = 32
NT = (((1,), (1,)), ((), ()))


def _iota(shape, d):
    return lax.broadcasted_iota(jnp.int32, shape, d)


def _dot(a, b):
    return jnp.dot(a, b, preferred_element_type=F32)


def _dot_nt(a, b):
    return lax.dot_general(a, b, NT, preferred_element_type=F32)


def _body(
    xa_hbm, k_hbm, v_hbm, wq_hbm, wo_hbm,
    xb_hbm, c_hbm, bq_hbm, buk_hbm, buv_hbm, bo_hbm,
    o_ref,
    xa_v, xb_v, kv_v, wq_v, wo_v, c_v, bq_v, buk_v, buv_v, bo_v,
    e_v, et_v, x2_v, qb_v, qabs_v, m_v, l_v, acc_v, cn_v, ctx_v,
    qa_v, oa_v, ob_v,
    sems, xsem, fsems,
):
    def start(src, dst, sem, prio):
        pltpu.make_async_copy(src, dst, sem).start(priority=prio)

    def wait(dst, sem):
        pltpu.make_async_copy(dst, dst, sem).wait()

    def edge(k, n, size, shift):
        return 0 if k == 0 else (n * size if k == n else k * size + shift)

    def w3_idx(p0, np_, k0, k1):
        r0, r1 = edge(k0, 32, 128, 8), edge(k1, 32, 128, 8)
        return (pl.ds(p0, np_), pl.ds(r0, r1 - r0), slice(None))

    def start2(src, dst, idx, sem, prio):
        start(src.at[idx], dst.at[idx], sem, prio)

    def start_w3(src, dst, p, k, sem, prio):
        start2(src, dst, w3_idx(p, 1, k, k + 1), sem, prio)

    def start_c(p, k, sem, prio):
        start_w3(c_hbm, c_v, p, k, sem, prio)

    def issue_s0(t, j0, j1):
        sem = sems.at[t % 3]
        for j in range(j0, j1):
            k, n = t * 8 + j // 4, j % 4
            for u in range(2):
                prio = 1 if (t == 0 and j < 16) else u
                if n == 0:
                    start_w3(buk_hbm, buk_v, 2 + u, k, sem, prio)
                elif n < 3:
                    start_w3(bq_hbm, bq_v, (n - 1) * 2 + u, k, sem, prio)
                else:
                    start_c(u, k, sem, prio)

    def wait_s0(t):
        sem = sems.at[t % 3]
        wait(buk_v.at[w3_idx(2, 2, t * 8, t * 8 + 8)], sem)
        wait(bq_v.at[w3_idx(0, 4, t * 8, t * 8 + 8)], sem)
        wait(c_v.at[w3_idx(0, 2, t * 8, t * 8 + 8)], sem)

    def wq_idx(t, p0, np_, k0, k1):
        r0, r1 = (edge((t % 2) * 8 + k, 16, 128, -8) for k in (k0, k1))
        return (pl.ds((t // 2) * 4 + p0, np_), pl.ds(r0, r1 - r0), slice(None))

    def issue_s1(t, j0, j1):
        sem = sems.at[(4 + t) % 3]
        for j in range(j0, j1):
            k, n = t * 8 + j // 4, j % 4
            for u in range(2):
                if n == 0:
                    start_w3(buv_hbm, buv_v, 2 + u, k, sem, u)
                elif n == 2:
                    start_w3(buk_hbm, buk_v, u, k, sem, u)
                else:
                    start2(wq_hbm, wq_v, wq_idx(t, n - 1 + u, 1, j // 4, j // 4 + 1), sem, u)

    def wait_s1(t):
        sem = sems.at[(4 + t) % 3]
        wait(buv_v.at[w3_idx(2, 2, t * 8, t * 8 + 8)], sem)
        wait(buk_v.at[w3_idx(0, 2, t * 8, t * 8 + 8)], sem)
        wait(wq_v.at[wq_idx(t, 0, 4, 0, 8)], sem)

    def issue_c(i, j0, j1):
        sem = sems.at[(8 + i) % 3]
        for j in range(j0, j1):
            k, n = (i % 4) * 8 + j // 4, j % 4
            for u in range(2):
                if i < 4:
                    start_c(2 + n * 2 + u, k, sem, u)
                elif n < 3:
                    start_c(10 + n * 2 + u, k, sem, u)
                else:
                    start_w3(buv_hbm, buv_v, u, k, sem, u)

    def wait_c(i):
        sem = sems.at[(8 + i) % 3]
        k0 = (i % 4) * 8
        if i < 4:
            wait(c_v.at[w3_idx(2, 8, k0, k0 + 8)], sem)
        else:
            wait(c_v.at[w3_idx(10, 6, k0, k0 + 8)], sem)
            wait(buv_v.at[w3_idx(0, 2, k0, k0 + 8)], sem)

    def kv_heads(g):
        return [(((g & 1) << 5) + (g >> 1) + (d + 2)) & 127 for d in (0, 16, 64, 80)]

    def issue_kv(g, j0, j1):
        slot = (16 + g) % 3
        sem = sems.at[slot]
        fs = kv_heads(g)
        for j in range(j0, j1):
            a, n = (j // 4) % 2, j % 4
            for u in range(2):
                k = j // 8 + 4 * u
                r0, r1 = edge(k, 8, 128, -8), edge(k + 1, 8, 128, -8)
                start((k_hbm, v_hbm)[a].at[fs[n], pl.ds(SK - W + r0, r1 - r0), :],
                      kv_v.at[slot, a, n, pl.ds(r0, r1 - r0), :], sem, u)

    def wait_kv(g):
        slot = (16 + g) % 3
        wait(kv_v.at[slot], sems.at[slot])

    def o_heads(t):
        return [(p, (t ^ (p & 2)) * 2 + hb) for hb in range(2) for p in (0, 2, 1, 3)]

    def o_rows(p, h, k0, k1, shift):
        k0, k1 = k0 + (h % 2) * 4, k1 + (h % 2) * 4
        r0, r1 = edge(k0, 8, 128, shift), edge(k1, 8, 128, shift)
        return (p, pl.ds((h // 2) * 1024 + r0, r1 - r0), slice(None))

    def o_order(t, groups, shift):
        heads = o_heads(t)
        return [(n, o_rows(p, h, k, k + 1, shift))
                for n, (h0, nh) in enumerate(groups) for k in range(4) for p, h in heads[h0:h0 + nh]]

    HALVES = ((0, 4), (4, 4))
    TAIL = ((0, 4), (4, 2), (6, 1), (7, 1))

    def issue_o(t):
        for (_, ia), (n, ib) in zip(o_order(t, HALVES, -8), o_order(t, HALVES if t < 3 else TAIL, 8)):
            start2(wo_hbm, wo_v, ia, fsems.at[2 * t], 0)
            start2(bo_hbm, bo_v, ib, fsems.at[2 * t + 1 + (n if t == 3 else 0)], 1)

    def diag_mask():
        return (_iota((64, 2048), 1) & 15) == (_iota((64, 2048), 0) & 15)

    def w3(ref, k, hf):
        return ref[k].reshape(128, 2, 16, DH)[:, hf].reshape(2048, DH)

    def untile(v, nt=4):
        n = v.size // (128 * nt)
        v = v.reshape(n // 8, nt, 8, 128)
        return jnp.concatenate([v[:, k].reshape(n, 128) for k in range(nt)], axis=1)

    def build_consts():
        e_v[...] = jnp.where(_iota((128, 2048), 0) == (_iota((128, 2048), 1) >> 4), 1.0, 0.0).astype(BF16)
        et_v[...] = jnp.where(_iota((2048, 128), 1) == (_iota((2048, 128), 0) >> 4), 1.0, 0.0).astype(BF16)
        m_v[...] = jnp.full(m_v.shape, -jnp.inf, F32)
        l_v[...] = jnp.zeros(l_v.shape, F32)
        acc_v[...] = jnp.zeros(acc_v.shape, F32)
        oa_v[...] = jnp.zeros(oa_v.shape, F32)

    def build_x2():
        x = xb_v[...].astype(F32)
        xrep = jnp.concatenate(
            [jnp.broadcast_to(x[b:b + 1, :], (16, DM)) for b in range(B)], axis=0).astype(BF16)
        for k in range(4):
            xe = _dot(xrep[:, k * 128:(k + 1) * 128], e_v[...])
            x2_v[:, k * 2048:(k + 1) * 2048] = jnp.where(diag_mask(), xe, 0.0).astype(BF16)

    def qb_half(hf):
        acc = None
        for k in range(4):
            r = _dot(x2_v[:, k * 2048:(k + 1) * 2048], w3(bq_v, k, hf))
            acc = r if acc is None else acc + r
        qb_v[hf * 64:(hf + 1) * 64, :] = acc.astype(BF16)

    def qabs_piece(hf, k):
        r = _dot_nt(qb_v[hf * 64:(hf + 1) * 64, :], w3(buk_v, k, hf))
        r = jnp.where(diag_mask(), r, 0.0).astype(BF16)
        z = _dot(r, et_v[...]).astype(BF16)
        for b in range(B):
            qabs_v[b, hf * 16:(hf + 1) * 16, k * 128:(k + 1) * 128] = z[b * 16:(b + 1) * 16, :]

    def qa_proj():
        x = xa_v[...].astype(F32)
        x8 = jnp.concatenate([x, x], axis=0).astype(BF16)
        acc = None
        for k in range(4):
            r = _dot(x8[:, k * 128:(k + 1) * 128], untile(wq_v[2 * k:2 * k + 2], H))
            acc = r if acc is None else acc + r
        for h in range(H):
            qa_v[h] = acc[:, h * DH:(h + 1) * DH]

    def b_attn(i, u):
        rows = pl.ds(pl.multiple_of((i % 4) * 1024, 1024), 1024)
        p0s = [(2 + (i // 4) * 8 + u * 4 + n * 2) % 16 for n in range(2)]
        bs = [p0 // 4 for p0 in p0s]
        cs = [untile(c_v[pl.ds(p0, 2), rows, :]) for p0 in p0s]
        ss = [_dot_nt(qabs_v[b], c) * SCALE for b, c in zip(bs, cs)]
        ps, alphas = [], []
        for b, s in zip(bs, ss):
            m_old = m_v[b]
            m_new = jnp.maximum(m_old, jnp.max(s, axis=1, keepdims=True))
            alpha = jnp.exp(m_old - m_new)
            p = jnp.exp(s - m_new)
            l_v[b] = alpha * l_v[b] + jnp.sum(p, axis=1, keepdims=True)
            m_v[b] = m_new
            ps.append(p.astype(BF16))
            alphas.append(alpha)
        for b, p, c, alpha in zip(bs, ps, cs, alphas):
            acc_v[b] = alpha * acc_v[b] + _dot(p, c)

    def b_norm():
        for b in range(B):
            cn = (acc_v[b] / l_v[b]).astype(BF16)
            for hf in range(2):
                for k in range(4):
                    cn_v[hf * 4 + k, b * 16:(b + 1) * 16, :] = (
                        cn[hf * 16:(hf + 1) * 16, k * 128:(k + 1) * 128])
        ctx_v[...] = jnp.zeros(ctx_v.shape, F32)

    def ctx_piece(hf, k):
        xe = _dot(cn_v[hf * 4 + k], e_v[...])
        xe = jnp.where(diag_mask(), xe, 0.0).astype(BF16)
        ctx_v[hf] += _dot(xe, w3(buv_v, k, hf))

    def ob_build():
        ro = _iota((256, 128), 0)
        ri = _iota((256, 128), 1)
        src = ((ro >> 7) << 6) + ((ro & 7) << 4) + ((ro >> 3) & 15)
        perm = jnp.where(((ro & 7) < 4) & (ri == src), 1.0, 0.0).astype(BF16)
        ctx = ctx_v[...].reshape(128, DH).astype(BF16)
        ob_v[...] = _dot(perm, ctx).reshape(H, 8, DH)

    def a_group(g):
        slot = (16 + g) % 3
        fs = kv_heads(g)
        ss = [_dot_nt(qa_v[f & 31].astype(BF16), kv_v[slot, 0, j]) * SCALE for j, f in enumerate(fs)]
        ps = [jnp.exp(s - jnp.max(s, axis=1, keepdims=True)) for s in ss]
        ls = [jnp.sum(p, axis=1, keepdims=True) for p in ps]
        outs = [_dot(p.astype(BF16), kv_v[slot, 1, j]) / l for j, (p, l) in enumerate(zip(ps, ls))]
        for f, o in zip(fs, outs):
            oa_v[f & 31] = jnp.where(_iota((8, DH), 0) == (f >> 5), o, oa_v[f & 31])

    def o_proj(acc, o_v, w_v, shift, sem, t, h0, n):
        heads = o_heads(t)[h0:h0 + n]
        for p, h in heads:
            wait(w_v.at[o_rows(p, h, 0, 4, shift)], sem)
        for p, h in heads:
            acc += _dot(o_v[p * 8 + h].astype(BF16), untile(w_v[p, h * 512:(h + 1) * 512, :]))
        return acc

    issue_s0(0, 0, 2)
    start(xa_hbm, xa_v, xsem.at[0], 0)
    start(xb_hbm, xb_v, xsem.at[0], 0)
    issue_s0(0, 2, NP)
    issue_s0(1, 0, NP)

    issue_s0(2, 0, NP)
    wait_s0(0)
    wait(xa_v, xsem.at[0])
    wait(xb_v, xsem.at[0])
    build_consts()

    issue_s0(3, 0, NP)
    wait_s0(1)
    build_x2()

    issue_s1(0, 0, NP)
    wait_s0(2)

    issue_s1(1, 0, 24)
    wait_s0(3)
    qb_half(0)
    issue_s1(1, 24, NP)
    qb_half(1)

    for hf in range(2):
        issue_s1(2 + hf, 0, NP)
        wait_s1(hf)
        qabs_piece(hf, 2)
        qabs_piece(hf, 3)

    issue_c(0, 0, NP)
    wait_s1(2)

    issue_c(1, 0, 24)
    wait_s1(3)
    qabs_piece(0, 0)
    qabs_piece(0, 1)
    issue_c(1, 24, 28)
    qabs_piece(1, 0)
    qabs_piece(1, 1)
    issue_c(1, 28, NP)
    qa_proj()

    def b_body(i, carry):
        for u in range(2):
            j0, j1 = (0, 24) if u == 0 else (24, NP)
            for n in range(8):
                nxt = (functools.partial(issue_c, n + 2) if n < 6 else functools.partial(issue_kv, n - 6))
                pl.when(i == n)(functools.partial(nxt, j0, j1))
            if u == 0:
                for n in range(8):
                    pl.when(i == n)(functools.partial(wait_c, n))
            b_attn(i, u)
        return carry

    lax.fori_loop(0, 8, b_body, 0)
    b_norm()

    def a_body(g, carry):
        pl.when(g < H - 2)(lambda: issue_kv(g + 2, 0, NP))
        pl.when(g == H - 2)(lambda: issue_o(0))
        pl.when(g == H - 1)(lambda: issue_o(1))
        wait_kv(g)
        a_group(g)
        pl.when(g < 4)(lambda: ctx_piece(0, g))
        pl.when((g >= 4) & (g < 8))(lambda: ctx_piece(1, g - 4))
        return carry

    lax.fori_loop(0, H, a_body, 0)

    acc_a = jnp.zeros((8, DM), F32)
    acc_b = jnp.zeros((8, DM), F32)
    issue_o(2)
    ob_build()
    acc_a = o_proj(acc_a, oa_v, wo_v, -8, fsems.at[0], 0, 0, 8)
    acc_b = o_proj(acc_b, ob_v, bo_v, 8, fsems.at[1], 0, 0, 8)
    issue_o(3)
    for t in (1, 2):
        acc_a = o_proj(acc_a, oa_v, wo_v, -8, fsems.at[2 * t], t, 0, 8)
        acc_b = o_proj(acc_b, ob_v, bo_v, 8, fsems.at[2 * t + 1], t, 0, 8)
    acc_a = o_proj(acc_a, oa_v, wo_v, -8, fsems.at[6], 3, 0, 8)
    o_ref[:, 0:DM] = acc_a[0:B, :].astype(o_ref.dtype)
    for n, (h0, k) in enumerate(TAIL):
        acc_b = o_proj(acc_b, ob_v, bo_v, 8, fsems.at[7 + n], 3, h0, k)
    o_ref[:, DM:2 * DM] = acc_b[0:B, :].astype(o_ref.dtype)


def _kernel(*refs):
    pl.run_scoped(
        functools.partial(_body, *refs),
        pltpu.SemaphoreType.DMA((3,)),
        pltpu.SemaphoreType.DMA((1,)),
        pltpu.SemaphoreType.DMA((11,)),
    )


@jax.jit
def pallas_concat_heads__sliding_block_cached__compressed_kv_cla__decode_kernel(
    A_x: jax.Array,
    A_k_cache: jax.Array,
    A_v_cache: jax.Array,
    A_wq: jax.Array,
    A_wo: jax.Array,
    B_x: jax.Array,
    B_c_kv: jax.Array,
    B_w_q: jax.Array,
    B_w_uk: jax.Array,
    B_w_uv: jax.Array,
    B_w_o: jax.Array,
):
    w3_shape = (4, 4096, DH)

    def tile_rows(a, rows=4096):
        return a.reshape(-1, 8, a.shape[-1] // 128, 128).transpose(0, 2, 1, 3).reshape(-1, rows, 128)

    hbm = pl.BlockSpec(memory_space=pl.ANY)
    vmem = pltpu.VMEM
    out = pl.pallas_call(
        _kernel,
        out_shape=jax.ShapeDtypeStruct((B, 2 * DM), BF16),
        in_specs=[hbm] * 11,
        out_specs=pl.BlockSpec(memory_space=pltpu.VMEM),
        scratch_shapes=[
            vmem((B, DM), BF16),
            vmem((B, DM), BF16),
            vmem((3, 2, B, W, DH), BF16),
            vmem((8, 2048, DH), BF16),
            vmem(w3_shape, BF16),
            vmem((16, 4096, DH), BF16),
            vmem(w3_shape, BF16),
            vmem(w3_shape, BF16),
            vmem(w3_shape, BF16),
            vmem(w3_shape, BF16),
            vmem((128, 2048), BF16),
            vmem((2048, 128), BF16),
            vmem((64, 8192), BF16),
            vmem((128, DH), BF16),
            vmem((B, H, DM), BF16),
            vmem((B, H, 1), F32),
            vmem((B, H, 1), F32),
            vmem((B, H, DM), F32),
            vmem((8, 64, 128), BF16),
            vmem((2, 64, DH), F32),
            vmem((H, 8, DH), F32),
            vmem((H, 8, DH), F32),
            vmem((H, 8, DH), F32),
        ],
        compiler_params=pltpu.CompilerParams(vmem_limit_bytes=100 * 1024 * 1024),
        name="fused_decode",
    )(
        A_x.reshape(B, DM),
        A_k_cache.reshape(B * H, SK, DH),
        A_v_cache.reshape(B * H, SK, DH),
        tile_rows(A_wq, 2048),
        tile_rows(A_wo),
        B_x.reshape(B, DM),
        tile_rows(B_c_kv),
        B_w_q.reshape(w3_shape),
        B_w_uk.reshape(w3_shape),
        B_w_uv.reshape(w3_shape),
        tile_rows(B_w_o),
    )
    return out.reshape(B, 1, 2 * DM)
```
